```python
import jax
import jax.numpy as jnp

def _softmax(x, axis=-1):
    return jax.nn.softmax(x, axis=axis)

def _gelu(x):
    return jax.nn.gelu(x, approximate=True)

def _silu(x):
    return jax.nn.silu(x)

def _sigmoid(x):
    return jax.nn.sigmoid(x)

def _layernorm(x, axis=-1, eps=1e-05):
    m = jnp.mean(x, axis=axis, keepdims=True)
    v = jnp.var(x, axis=axis, keepdims=True)
    return (x - m) / jnp.sqrt(v + eps)

def _scatter_add(tgt, idx, src, axis=0):
    return tgt.at[idx].add(src)

def _segment_sum(src, seg, n):
    return jax.ops.segment_sum(src, seg, n)

class _Rng:

    def __init__(self, key):
        self._k = key

    def _next(self):
        self._k, sub = jax.random.split(self._k)
        return sub

    def normal(self, shape):
        return jax.random.normal(self._next(), shape, dtype=jnp.bfloat16)

    def randint(self, lo, hi, shape):
        return jax.random.randint(self._next(), shape, lo, hi, dtype=jnp.int32)

    def uniform(self, shape, lo=0.0, hi=1.0):
        return jax.random.uniform(self._next(), shape, jnp.bfloat16, lo, hi)

    def permutation(self, n):
        return jax.random.permutation(self._next(), n)
kernel_name = 'sequential_preLN__sliding_local_dilated__mixer_gmlp__prompt'

def setup_inputs():
    _rng = _Rng(jax.random.key(int.from_bytes(__import__("os").urandom(4), "little")))
    _w = lambda a: (lambda t: t.astype(jnp.bfloat16) if jnp.issubdtype(t.dtype, jnp.floating) else t)(jnp.asarray(a))

    def _A_setup():
        B, S, D = (1, 2048, 1024)
        return {'x': _w((lambda *s: _rng.normal(s) * 0.05)(B, S, D)), 'wqkv': _w((lambda *s: _rng.normal(s) * 0.05)(D, 3 * D)), 'wo': _w((lambda *s: _rng.normal(s) * 0.05)(D, D))}
    _A_in = _A_setup()

    def _B_setup():
        B, S, D, F = (1, 2048, 1024, 3584)
        Fh = F // 2
        return {'x': _w((lambda *s: _rng.normal(s) * 0.05)(B, S, D)), 'w_in': _w((lambda *s: _rng.normal(s) * 0.05)(D, 2 * Fh)), 'w_sp': _w(0.01 * (lambda *s: _rng.normal(s) * 0.05)(S, S)), 'b_sp': _w(1.0 + 0.01 * (lambda *s: _rng.normal(s) * 0.05)(S)), 'w_out': _w((lambda *s: _rng.normal(s) * 0.05)(Fh, D))}
    _B_in = _B_setup()
    return {'A_x': _A_in['x'], 'A_wqkv': _A_in['wqkv'], 'A_wo': _A_in['wo'], 'B_x': _B_in['x'], 'B_w_in': _B_in['w_in'], 'B_w_sp': _B_in['w_sp'], 'B_b_sp': _B_in['b_sp'], 'B_w_out': _B_in['w_out']}

def reference(A_x, A_wqkv, A_wo, B_x, B_w_in, B_w_sp, B_b_sp, B_w_out):

    def _A_ref(x, wqkv, wo):
        B, S, D = x.shape
        H = 32
        Dh = D // H
        W, dil = (8, 2)
        qkv = (lambda x, *d: x.transpose(*d))((x @ wqkv).reshape(B, S, 3, H, Dh), 2, 0, 3, 1, 4)
        q, k, v = (qkv[0], qkv[1], qkv[2])
        scale = Dh ** (-0.5)
        pos = jnp.arange(S)
        off = jnp.arange(W) * dil
        idx = pos[:, None] - off[None, :]
        mask = idx >= 0
        idx_c = jnp.where(mask, idx, 0).reshape(-1)
        kg = k[:, :, idx_c, :].reshape(B, H, S, W, Dh)
        vg = v[:, :, idx_c, :].reshape(B, H, S, W, Dh)
        logits = jnp.einsum('bhsd,bhswd->bhsw', q, kg) * scale
        logits = jnp.where(mask[None, None, :, :], logits, -1000000000.0)
        attn = _softmax(logits, axis=-1)
        o = jnp.einsum('bhsw,bhswd->bhsd', attn, vg)
        return (lambda x, *d: x.transpose(*d))(o, 0, 2, 1, 3).reshape(B, S, D) @ wo

    def _B_ref(x, w_in, w_sp, b_sp, w_out):
        B, S, D = x.shape
        F = w_in.shape[-1]
        Fh = F // 2
        z = _gelu(jnp.einsum('bsd,df->bsf', x, w_in))
        z1 = z[..., :Fh].copy()
        z2 = _layernorm(z[..., Fh:], axis=-1)
        g = jnp.einsum('ts,bsf->btf', w_sp, z2) + b_sp[None, :, None]
        return jnp.einsum('bsf,fd->bsd', z1 * g, w_out)
    x = A_x
    h = x + _A_ref(_layernorm(x, axis=-1), A_wqkv, A_wo)
    h2 = h + _B_ref(_layernorm(h, axis=-1), B_w_in, B_w_sp, B_b_sp, B_w_out)
    return h2
```

```python
import functools

import jax
import jax.numpy as jnp
import numpy as np
from jax import lax
from jax.experimental import pallas as pl
from jax.experimental.pallas import tpu as pltpu

S = 2048
D = 1024
FH = 1792
NH = 32
DH = 32
WIN = 8
DIL = 2
HALO = 16
TM = 512
U = 256
HU = U // 2
NT = D // 128
EPS = 1e-5

f32 = jnp.float32
bf16 = jnp.bfloat16
u32 = jnp.uint32

CFG = dict(part='all', tail=0, ties=True, gates=True, lat_short=3, lat_stats=4, lat_perm=4, lat_logit=4, lat_soft=4, tmp=True, lat_pv=3, lat_wsp=2, flags=None, qkv=True, wo=True, win=True, sp=True, out=True, unroll1=False, unroll2=False)


def _pack(v):
    return pltpu.bitcast(v.astype(bf16), u32)


def _as_bf16(v):
    return pltpu.bitcast(v, bf16)


def _unpack(v):
    return pltpu.bitcast(v, bf16).astype(f32)


def _dot(a, b):
    return jnp.dot(a, b, preferred_element_type=f32)


def _run(tasks):
    for t in tasks:
        t[0]()


def _gelu(v):
    c = float(np.sqrt(2.0 / np.pi))
    t = jnp.tanh(v * (c + (c * 0.044715) * (v * v)))
    hv = 0.5 * v
    return hv + hv * t


def _a_shape(k, fast):
    return (7, HU // 2, k // 2) if fast else (U // 2, k)


def _b_shape(k, n, fast):
    return (7, k // 4, n // 2) if fast else (k // 2, n)


def _put_a(buf, fast, r, nr, c, a11, a12, a21, a22):
    w = a11.shape[1]
    rows = slice(r // 2, (r + nr) // 2)
    if fast:
        ops = (a11 + a22, a21 + a22, a11, a22, a11 + a12, a21 - a11, a12 - a22)
        for i, op in enumerate(ops):
            buf.at[i][rows, c:c + w] = _pack(op)
        return buf, r // 2, c
    kh = buf.shape[1] // 2
    rows2 = slice((HU + r) // 2, (HU + r + nr) // 2)
    buf[rows, c:c + w] = _pack(a11)
    buf[rows, kh + c:kh + c + w] = _pack(a12)
    buf[rows2, c:c + w] = _pack(a21)
    buf[rows2, kh + c:kh + c + w] = _pack(a22)
    return buf, r // 2, c


def _put_b(buf, pr, b11, b12, b21, b22, c=0):
    ops = (b11 + b22, b11, b12 - b22, b21 - b11, b22, b11 + b12, b21 + b22)
    for i, op in enumerate(ops):
        buf.at[i][pr:pr + 8, c:c + op.shape[1]] = _pack(op)
    return buf, pr, c


def _matmul_tasks(a_buf, b_get, fast, nhalf, cw, emit, put=None, tmp=None):
    def gen():
        tie = yield
        for c in range(0, nhalf, cw):
            if fast and put is not None and tmp is not None:
                def dot(i):
                    return _dot(_as_bf16(a_buf.at[i][...]), _as_bf16(tie(b_get(i, c, cw))))
                t1, t2, t3, t4, t5 = [t.at[:, 0:cw] for t in tmp]
                m = dot(0)
                t1[...] = m
                tie = yield m
                m = dot(3)
                t4[...] = m
                tie = yield m
                m = dot(1)
                t2[...] = m
                put(1, 0, c, m + t4[...])
                tie = yield m
                m = dot(2)
                t3[...] = m
                tie = yield m
                m = dot(5)
                put(1, 1, c, (t1[...] - t2[...] + t3[...]) + m)
                tie = yield m
                m = dot(4)
                t5[...] = m
                put(0, 1, c, m + t3[...])
                tie = yield m
                m = dot(6)
                put(0, 0, c, (t1[...] + t4[...] - t5[...]) + m)
                tie = yield m
            elif fast:
                m = {}
                for i in (0, 3, 1, 2, 4, 6, 5):
                    m[i] = _dot(_as_bf16(a_buf.at[i][...]), _as_bf16(tie(b_get(i, c, cw))))
                    if i != 5:
                        tie = yield m[i]
                emit(c, m[0] + m[3] - m[4] + m[6], m[2] + m[4], m[1] + m[3],
                     m[0] - m[1] + m[2] + m[5])
                tie = yield m[5]
            else:
                left = _dot(_as_bf16(a_buf[...]), _as_bf16(tie(b_get(None, c, cw))))
                tie = yield left
                right = _dot(_as_bf16(a_buf[...]), _as_bf16(tie(b_get(None, nhalf + c, cw))))
                emit(c, left[:HU], right[:HU], left[HU:], right[HU:])
                tie = yield right
    return (nhalf // cw) * (7 if fast else 2), gen()


def _permute_cols(tiles):
    lane = lax.broadcasted_iota(jnp.int32, tiles[0].shape, 1)
    r = [t if j == 0 else pltpu.roll(t, 4 * j, 1) for j, t in enumerate(tiles)]
    w = [r[(-j) % NT] for j in range(NT)]
    for b in range(3):
        m = (lane & (4 << b)) != 0
        w = [jnp.where(m, w[(j - (1 << b)) % NT], w[j]) for j in range(NT)]
    return [t if j == 0 else pltpu.roll(t, 128 - 4 * j, 1) for j, t in enumerate(w)]


def _pair_transpose(v):
    sub = lax.broadcasted_iota(jnp.int32, v[0].shape, 0)
    v = list(v)
    for b in range(2):
        s = 1 << b
        m = (sub & (2 * s)) != 0
        nv = list(v)
        for j in range(4):
            if j & s:
                continue
            lo, hi = v[j], v[j + s]
            nv[j] = jnp.where(m, pltpu.roll(hi, 2 * s, 0), lo)
            nv[j + s] = jnp.where(m, hi, pltpu.roll(lo, 8 - 2 * s, 0))
        v = nv
    return v


def _kernel(cfg,
            x_hbm, wqkv_hbm, wo_hbm, win_hbm, wsp_hbm, bsp_hbm, wout_hbm, out_hbm,
            x_s, wq_raw, wk_raw, wv_raw, wo_raw, wz1_raw, wz2_raw, wsp_raw, bsp_raw, wout_raw,
            wq_p, wk_p, wv_p, wo_t, wo_p, wz1_p, wz2_p, wout_p, z2n_p,
            h_s, z1_s, bias_s,
            xa0, xa1, oa0, oa1, ha0, ha1, sa0, sa1, ya0, ya1,
            q_s, k0_s, k1_s, v0_s, v1_s, p0_s, p1_s, z20_s, z21_s,
            stx0, stx1, sth0, sth1, stz0, stz1,
            t1_s, t2_s, t3_s, t4_s, t5_s, l0_s, l1_s, e0_s, e1_s,
            sem, osem):
    nstep = S // TM
    zero = []

    def spot(ref, row, col):
        n = 8 * (4 // ref.dtype.itemsize)
        ref = ref if len(ref.shape) == 2 else ref.at[zero[0]]
        return ref.at[pl.ds(pl.multiple_of(row + zero[0] * n, n), n),
                      pl.ds(pl.multiple_of(col + zero[0] * 128, 128), 128)]

    def gate(ref, row):
        def go(v):
            spot(ref, row, 0)[...] = pltpu.bitcast(v[0:8, 0:128], ref.dtype)
        return go

    def done(ref, row, col):
        v = spot(ref, row, col)[...]
        return v if v.dtype == u32 else pltpu.bitcast(v, u32)

    def tied(toks):
        def tie(b):
            if not toks:
                return b
            tok = functools.reduce(lambda p, q: p | q, toks)
            tok = jnp.concatenate([tok] * (b.shape[1] // 128), axis=1)
            always = lax.broadcasted_iota(jnp.int32, tok.shape, 0) >= zero[0]
            parts = []
            for r in range(0, b.shape[0], 64):
                parts += [b[r:r + 56], jnp.where(always, b[r + 56:r + 64], tok)]
            return jnp.concatenate(parts, axis=0)
        return tie

    def il(main, *sides):
        n, gen = main
        next(gen)
        pos = [0] * len(sides)
        due = [[] for _ in range(n)]
        for i in range(n):
            res = gen.send(tied(due[i]))
            gates, run = {}, []
            for s, side in enumerate(sides):
                if not side:
                    continue
                span = max(1, n - max(t[2] for t in side) - cfg["tail"])
                end = min(len(side), (len(side) * (i + 1) + span - 1) // span)
                run += side[pos[s]:end]
                pos[s] = end
            for t in run:
                gates.update(t[1])
            if cfg["gates"]:
                for g in gates.values():
                    g(res)
            for fn, _, lat in run:
                where = fn()
                if where is not None and cfg["ties"] and i + lat < n:
                    due[i + lat].append(done(*where))
    st_x, st_h, st_z = (stx0, stx1), (sth0, sth1), (stz0, stz1)
    k_s, v_s, p_s, z2_s = (k0_s, k1_s), (v0_s, v1_s), (p0_s, p1_s), (z20_s, z21_s)
    tmp = (t1_s, t2_s, t3_s, t4_s, t5_s)
    l_s, e_s = (l0_s, l1_s), (e0_s, e1_s)
    wqkv_raw, win_raw = (wq_raw, wk_raw, wv_raw), (wz1_raw, wz2_raw)
    xa, oa, ha, sa, ya = (xa0, xa1), (oa0, oa1), (ha0, ha1), (sa0, sa1), (ya0, ya1)

    def cp(src, dst, j):
        return pltpu.make_async_copy(src, dst, sem.at[j])

    dma = dict(
        x0=cp(x_hbm.at[0, 0:TM], x_s.at[0:TM], 0),
        wq=cp(wqkv_hbm.at[:, 0:D], wqkv_raw[0].at[0:D], 1),
        wk=cp(wqkv_hbm.at[:, D:2 * D], wqkv_raw[1].at[0:D], 2),
        wv=cp(wqkv_hbm.at[:, 2 * D:3 * D], wqkv_raw[2].at[0:D], 3),
        wo=cp(wo_hbm, wo_raw.at[0:D], 4),
        wz2=cp(win_hbm.at[:, FH:2 * FH], win_raw[1].at[0:D], 5),
        wz1=cp(win_hbm.at[:, 0:FH], win_raw[0].at[0:D], 6),
        xr=cp(x_hbm.at[0, TM:S], x_s.at[TM:S], 7),
        b=cp(bsp_hbm, bsp_raw, 8),
        wout=cp(wout_hbm, wout_raw.at[0:FH], 9),
        wsp=cp(wsp_hbm, wsp_raw.at[0:S], 10),
    )

    def tasks(fn, args, gates, lat):
        return [(functools.partial(fn, *a), gates, lat) for a in args]

    def prep_qkv_tasks(j, buf):
        raw = wqkv_raw[j]

        def perm(r):
            w = pltpu.bitcast(raw[r:r + 16, :], u32)
            return jnp.concatenate(
                _permute_cols([w[:, t * 128:(t + 1) * 128] for t in range(NT)]), axis=1)

        def task(r):
            top, bot = perm(r), perm(D // 2 + r)
            if cfg["qkv"]:
                top, bot = _unpack(top), _unpack(bot)
                return _put_b(buf, r // 2,
                              top[:, :D // 2], top[:, D // 2:], bot[:, :D // 2], bot[:, D // 2:])
            buf[r // 2:r // 2 + 8, :] = top
            buf[D // 4 + r // 2:D // 4 + r // 2 + 8, :] = bot
            return buf, r // 2, 0
        return tasks(task, [(r,) for r in range(0, D // 2, 16)], {"wqkv%d" % j: gate(raw, D)},
                     cfg["lat_perm"])

    def prep_wo_tasks():
        dst = wo_t if cfg["wo"] else wo_p

        def perm(t2, hh, d4):
            src = [((t2 * 4 + j) * 4 + hh) * 32 + d4 * 16 for j in range(4)]
            v = _pair_transpose([pltpu.bitcast(wo_raw[s:s + 16, :], u32) for s in src])
            for j in range(4):
                r = ((d4 * 4 + j) * 4 + hh) * 32 + t2 * 16
                dst[r // 2:r // 2 + 8, :] = v[j]
            return dst, r // 2, 0

        def comb(r):
            top = _unpack(wo_t[r // 2:r // 2 + 8, :])
            bot = _unpack(wo_t[D // 4 + r // 2:D // 4 + r // 2 + 8, :])
            return _put_b(wo_p, r // 2,
                          top[:, :D // 2], top[:, D // 2:], bot[:, :D // 2], bot[:, D // 2:])
        out = tasks(perm, [(t2, hh, d4) for hh in range(4) for d4 in range(2) for t2 in range(2)],
                    {"wo": gate(wo_raw, D)}, cfg["lat_short"])
        if cfg["wo"]:
            out += tasks(comb, [(r,) for r in range(0, D // 2, 16)], {"wot": gate(wo_t, D // 2)},
                         cfg["lat_short"])
        return out

    def prep_plain_tasks(raw, k, buf, fast):
        if not fast:
            return []
        n = raw.shape[1]

        def task(r, c, w):
            q = [raw[rr:rr + 16, cc:cc + w].astype(f32)
                 for rr in (r, k // 2 + r) for cc in (c, n // 2 + c)]
            return _put_b(buf, r // 2, *q, c)
        return tasks(task, [(r, c, min(512, n // 2 - c))
                            for r in range(0, k // 2, 16) for c in range(0, n // 2, 512)],
                     {"plain": gate(raw, k)}, cfg["lat_short"])

    def prep_bias_tasks():
        def task():
            b = bsp_raw[...].astype(f32).reshape(1, S)
            for j in range(S // 128):
                bias_s[j * 128:(j + 1) * 128, :] = jnp.broadcast_to(
                    b[:, j * 128:(j + 1) * 128], (128, 128)).T
        return [(task, {}, 1)]

    def getter(buf, fast, raw=None):
        def get(i, c, cw):
            if fast:
                return buf.at[i][:, c:c + cw]
            if raw is not None:
                return pltpu.bitcast(raw[0:raw.shape[0] - 16, c:c + cw], u32)
            return buf[:, c:c + cw]
        return get

    def ln_tasks(src, src_gate, r0, st, kw, put):
        n = src.shape[1]

        def shift(r):
            v = src[r0 + r:r0 + r + 64, 0:128].astype(f32)
            st.at[0][r:r + 64, :] = jnp.broadcast_to(v[:, 0:1], (64, 128))
            return st, r, 0

        def stats(r):
            sh = st.at[0][r:r + 16, :]
            s1 = s2 = None
            for c in range(0, n, 256):
                v = src[r0 + r:r0 + r + 16, c:c + 256].astype(f32)
                for d in (v[:, :128] - sh, v[:, 128:] - sh):
                    s1 = d if s1 is None else s1 + d
                    s2 = d * d if s2 is None else s2 + d * d
            m = jnp.sum(s1, axis=-1, keepdims=True) * (1.0 / n)
            var = jnp.sum(s2, axis=-1, keepdims=True) * (1.0 / n) - m * m
            st.at[1][r:r + 16, :] = sh + m
            st.at[2][r:r + 16, :] = jnp.broadcast_to(jnp.maximum(var, 0.0) + EPS, (16, 128))
            return st, r, 0

        def rstd(r):
            for rr in (r, HU + r):
                st.at[0][rr:rr + 16, :] = lax.rsqrt(st.at[2][rr:rr + 16, :])
            return st, r, 0

        def apply(r, c, w):
            def norm(rr, cc):
                v = src[r0 + rr:r0 + rr + 16, cc:cc + w].astype(f32)
                rep = lambda t: jnp.concatenate([t] * (w // 128), axis=1)
                return (v - rep(st.at[1][rr:rr + 16, :])) * rep(st.at[0][rr:rr + 16, :])
            return put(r, c, norm(r, c), norm(r, n // 2 + c), norm(HU + r, c), norm(HU + r, n // 2 + c))
        st_gate = {"st": gate(st, U)}
        out = tasks(shift, [(r,) for r in range(0, U, 64)], src_gate, cfg["lat_stats"])
        out += tasks(stats, [(h * HU + r,) for r in range(0, HU, 16) for h in range(2)],
                     src_gate, cfg["lat_stats"])
        for r in range(0, HU, 16):
            if r == 0:
                out += tasks(rstd, [(0,)], st_gate, cfg["lat_short"])
            if r + 16 < HU:
                out += tasks(rstd, [(r + 16,)], st_gate, cfg["lat_short"])
            out += tasks(apply, [(r, c, min(kw, n // 2 - c)) for c in range(0, n // 2, kw)],
                         src_gate, cfg["lat_short"])
        return out

    def ln_a_tasks(src, src_gate, r0, st, buf, fast):
        return ln_tasks(src, src_gate, r0, st, 256,
                        lambda r, c, *q: _put_a(buf, fast, r, 16, c, *q))

    g_x = {"x": gate(x_s, S)}
    g_h = {"h": gate(h_s, S)}

    def take(v, idx):
        return jnp.take_along_axis(v, idx, axis=1)

    def logits_tasks(u, i):
        scale = float(DH) ** -0.5

        def dots(r):
            lane = lax.broadcasted_iota(jnp.int32, (8, 128), 1)
            q = [q_s[u * U + r:u * U + r + 8, t * 128:(t + 1) * 128] for t in range(NT)]
            acc = []
            for w in range(WIN):
                k0 = HALO + r - DIL * w
                a = q[0] * k_s[u][0, k0:k0 + 8, :]
                for t in range(1, NT):
                    a = a + q[t] * k_s[u][t, k0:k0 + 8, :]
                acc.append(a)
            for bit in (1, 2):
                odd = (lane & bit) != 0
                acc = [jnp.where(odd, acc[w ^ bit], acc[w]) for w in range(WIN)]
            for b in range(2):
                lg = acc[4 * b]
                for j in range(1, 4):
                    lg = lg + take(acc[4 * b + j], lane ^ j)
                lg = lg * scale
                if u * U + r < DIL * WIN:
                    pos = i * TM + u * U + r + lax.broadcasted_iota(jnp.int32, (8, 128), 0)
                    lg = jnp.where(pos >= DIL * (4 * b + (lane & 3)), lg, -1e9)
                l_s[u][b, r:r + 8, :] = lg
            return l_s[u], r, 0

        def exps(r):
            lane = lax.broadcasted_iota(jnp.int32, (16, 128), 1)
            lg = [l_s[u][b, r:r + 16, :] for b in range(2)]
            mx = jnp.maximum(lg[0], lg[1])
            mx = functools.reduce(jnp.maximum, [mx] + [take(mx, lane ^ j) for j in range(1, 4)])
            for b in range(2):
                e_s[u][b, r:r + 16, :] = jnp.exp(lg[b] - mx)
            return e_s[u], r, 0

        def probs(r):
            lane = lax.broadcasted_iota(jnp.int32, (16, 128), 1)
            e = [e_s[u][b, r:r + 16, :] for b in range(2)]
            e = {4 * b + j: take(e[b], (lane & -4) | j) for j in range(4) for b in range(2)}
            inv = 1.0 / functools.reduce(lambda p, q: p + q, e.values())
            for w in range(WIN):
                p_s[u][w, r:r + 16, :] = e[w] * inv
            return p_s[u], r, 0
        rows = lambda n: [(h * HU + r,) for r in range(0, HU, n) for h in range(2)]
        return (tasks(dots, rows(8), {"q": gate(q_s, TM), "k%d" % u: gate(k_s[u], HALO + U)},
                      cfg["lat_logit"]),
                tasks(exps, rows(16), {"l%d" % u: gate(l_s[u], U)}, cfg["lat_soft"])
                + tasks(probs, rows(16), {"e%d" % u: gate(e_s[u], U)}, cfg["lat_soft"]))

    def pv_tasks(u):
        def block(r, t):
            lo = hi = None
            for w in range(WIN):
                k0 = HALO + r - DIL * w
                p = p_s[u][w, r:r + 16, :]
                a, b = p * v_s[u][t, k0:k0 + 16, :], p * v_s[u][t + NT // 2, k0:k0 + 16, :]
                lo, hi = (a, b) if lo is None else (lo + a, hi + b)
            return lo, hi

        def task(r, t):
            return _put_a(oa[u], cfg["wo"], r, 16, t * 128, *block(r, t), *block(HU + r, t))
        return tasks(task, [(r, t) for r in range(0, HU, 16) for t in range(NT // 2)],
                     {"p%d" % u: gate(p_s[u], U), "v%d" % u: gate(v_s[u], HALO + U)},
                     cfg["lat_pv"])

    def ln_z2_tasks(u, dst):
        def put(r, c, b11, b12, b21, b22):
            w = b11.shape[1]
            if cfg["sp"]:
                return _put_b(dst, (u * HU + r) // 2, b11, b12, b21, b22, c)
            pr = (u * U + r) // 2
            where = [(slice(p, p + 8), slice(cc, cc + w))
                     for p in (pr, pr + HU // 2) for cc in (c, FH // 2 + c)]
            for idx, v in zip(where, (b11, b12, b21, b22)):
                dst[idx] = _pack(v)
            return dst, pr, c
        return ln_tasks(z2_s[u], {"z%d" % u: gate(z2_s[u], U)}, 0, st_z[u], 256, put)

    def wsp_tasks(src, r0, buf):
        def task(r, j):
            if cfg["sp"]:
                c1, c2, w = j * U, j * U + HU, HU
            else:
                c1, c2, w = j * HU, S // 2 + j * HU, HU
            q = [src[rr:rr + 16, cc:cc + w].astype(f32)
                 for rr in (r0 + r, r0 + HU + r) for cc in (c1, c2)]
            return _put_a(buf, cfg["sp"], r, 16, j * HU, *q)
        return tasks(task, [(r, j) for r in range(0, HU, 16) for j in range(S // U)],
                     {"wsp": gate(wsp_raw, S)}, cfg["lat_wsp"])

    def quad(store, nhalf, r0):
        def emit(c, c11, c12, c21, c22):
            store(r0, c, c11)
            store(r0, nhalf + c, c12)
            store(r0 + HU, c, c21)
            store(r0 + HU, nhalf + c, c22)
        return emit

    def step1(i, first):
        r0 = i * TM if isinstance(i, int) else pl.multiple_of(i * TM, TM)
        nxt = min(i + 1, nstep - 1) if isinstance(i, int) else jnp.minimum(i + 1, nstep - 1)
        rn = nxt * TM if isinstance(i, int) else pl.multiple_of(nxt * TM, TM)
        xt = x_s.at[pl.ds(r0, TM)]
        xn = x_s.at[pl.ds(rn, TM)]
        ht = h_s.at[pl.ds(r0, TM)]
        z1t = z1_s.at[pl.ds(r0 // 2 if isinstance(i, int) else pl.multiple_of(i * (TM // 2), TM // 2), TM // 2)]
        if cfg["sp"]:
            pr0 = i * (TM // 4)
            zt = z2n_p.at[:, pl.ds(pr0 if isinstance(i, int) else pl.multiple_of(pr0, TM // 4), TM // 4)]
        else:
            pr0 = i * (TM // 2)
            zt = z2n_p.at[pl.ds(pr0 if isinstance(i, int) else pl.multiple_of(pr0, TM // 2), TM // 2)]

        def st_q(r, c, v):
            q_s[r:r + HU, c:c + v.shape[1]] = v

        def st_slab(buf):
            def st(r, c, v):
                for j in range(v.shape[1] // 128):
                    t, u, rr = c // 128 + j, r // U, r % U
                    buf[u][t, HALO + rr:HALO + rr + HU, :] = v[:, j * 128:(j + 1) * 128]
                    if u == 0 and rr == HU:
                        buf[1][t, 0:HALO, :] = v[HU - HALO:, j * 128:(j + 1) * 128]
            return st

        def put_h(r, c, v):
            w = v.shape[1]
            ht[r:r + HU, c:c + w] = xt[r:r + HU, c:c + w].astype(f32) + v

        def st_z1(r, c, v):
            z1t[r // 2:(r + HU) // 2, c:c + v.shape[1]] = _pack(_gelu(v))

        def st_z2(r, c, v):
            z2_s[r // U][r % U:r % U + HU, c:c + v.shape[1]] = _gelu(v)

        def mm(a, b, key, st, u, nhalf, cw, raw=None):
            return _matmul_tasks(a[u], getter(b, cfg[key], raw), cfg[key], nhalf, cw,
                                 quad(st, nhalf, u * U),
                                 lambda rh, ch, c, v: st(u * U + rh * HU, ch * nhalf + c, v),
                                 tmp if cfg["tmp"] else None)

        def wait(name, *starts):
            if first:
                if name:
                    dma[name].wait()
                for n in starts:
                    dma[n].start()

        def once(tasks):
            return tasks if first else []

        def halo_init():
            k_s[0][:, 0:HALO, :] = jnp.zeros((NT, HALO, 128), f32)
            v_s[0][:, 0:HALO, :] = jnp.zeros((NT, HALO, 128), f32)

        def halo_copy():
            k_s[0][:, 0:HALO, :] = k_s[1][:, U:U + HALO, :]
            v_s[0][:, 0:HALO, :] = v_s[1][:, U:U + HALO, :]

        cw = 128
        il(mm(xa, wq_p, "qkv", st_q, 0, D // 2, cw), ln_a_tasks(xt, g_x, U, st_x[1], xa[1], cfg["qkv"]),
                    once([(halo_init, {}, 1)]))
        wait("wk", "wv")
        il(mm(xa, wq_p, "qkv", st_q, 1, D // 2, cw), once(prep_qkv_tasks(1, wk_p)))
        wait("wv", "wo", "wz2")
        pv_prep = once(prep_qkv_tasks(2, wv_p))
        il(mm(xa, wk_p, "qkv", st_slab(k_s), 0, D // 2, cw), pv_prep)
        dots0, soft0 = logits_tasks(0, i)
        dots1, soft1 = logits_tasks(1, i)
        il(mm(xa, wk_p, "qkv", st_slab(k_s), 1, D // 2, cw), dots0)
        wait("wo", "wz1")
        po = once(prep_wo_tasks())
        il(mm(xa, wv_p, "qkv", st_slab(v_s), 0, D // 2, cw), dots1, soft0, po[:len(po) // 2])
        il(mm(xa, wv_p, "qkv", st_slab(v_s), 1, D // 2, cw), pv_tasks(0), soft1, po[len(po) // 2:])
        wait("wz2", "xr", "b", "wout")
        pz = once(prep_plain_tasks(win_raw[1], D, wz2_p, cfg["win"]))
        il(mm(oa, wo_p, "wo", put_h, 0, D // 2, cw), pv_tasks(1), pz[:len(pz) // 2])
        il(mm(oa, wo_p, "wo", put_h, 1, D // 2, cw),
           ln_a_tasks(ht, g_h, 0, st_h[0], ha[0], cfg["win"]), pz[len(pz) // 2:],
           [(halo_copy, {}, 1)])
        wait("wz1", "wsp")
        il(mm(ha, wz2_p, "win", st_z2, 0, FH // 2, cw, win_raw[1]),
                    ln_a_tasks(ht, g_h, U, st_h[1], ha[1], cfg["win"]),
                    once(prep_plain_tasks(win_raw[0], D, wz1_p, cfg["win"])))
        wait("xr")
        wait("b")
        wait("wout")
        il(mm(ha, wz2_p, "win", st_z2, 1, FH // 2, cw, win_raw[1]),
                    ln_z2_tasks(0, zt),
                    once(prep_plain_tasks(wout_raw, FH, wout_p, cfg["out"]) + prep_bias_tasks()))
        il(mm(ha, wz1_p, "win", st_z1, 0, FH // 2, cw, win_raw[0]),
                    ln_z2_tasks(1, zt))
        wait("wsp")
        il(mm(ha, wz1_p, "win", st_z1, 1, FH // 2, cw, win_raw[0]),
                    ln_a_tasks(xn, g_x, 0, st_x[0], xa[0], cfg["qkv"]),
                    once(wsp_tasks(wsp_raw, 0, sa[0])))

    def out_copy(j, u):
        r = j * TM + u * U
        if not isinstance(r, int):
            r = pl.multiple_of(r, U)
        return pltpu.make_async_copy(x_s.at[pl.ds(r, U)], out_hbm.at[0, pl.ds(r, U)],
                                     osem.at[2 * j + u])

    def step2(j):
        st = isinstance(j, int)
        r0 = j * TM if st else pl.multiple_of(j * TM, TM)
        nxt = min(j + 1, nstep - 1) if st else jnp.minimum(j + 1, nstep - 1)
        rn = nxt * TM if st else pl.multiple_of(nxt * TM, TM)
        wt = wsp_raw.at[pl.ds(r0, TM)]
        wn = wsp_raw.at[pl.ds(rn, TM)]
        ht = h_s.at[pl.ds(r0, TM)]
        bt = bias_s.at[pl.ds(r0, TM)]
        ot = x_s.at[pl.ds(r0, TM)]
        z1t = z1_s.at[pl.ds(r0 // 2 if st else pl.multiple_of(j * (TM // 2), TM // 2), TM // 2)]

        def gating(u):
            def one(r, c, g):
                w = g.shape[1]
                z1 = _unpack(z1t[r // 2:(r + HU) // 2, c:c + w])
                b = bt[r:r + HU, :]
                return z1 * (g + jnp.concatenate([b] * (w // 128), axis=1))

            def emit(c, c11, c12, c21, c22):
                r = u * U
                _put_a(ya[u], cfg["out"], 0, HU, c,
                       one(r, c, c11), one(r, FH // 2 + c, c12),
                       one(r + HU, c, c21), one(r + HU, FH // 2 + c, c22))
            return emit

        def st_out(r, c, v):
            w = v.shape[1]
            ot[r:r + HU, c:c + w] = (ht[r:r + HU, c:c + w] + v).astype(bf16)

        def gmm(u):
            return _matmul_tasks(sa[u], getter(z2n_p, cfg["sp"]), cfg["sp"], FH // 2, 128, gating(u))

        def omm(u):
            return _matmul_tasks(ya[u], getter(wout_p, cfg["out"], wout_raw), cfg["out"], D // 2,
                                 256, quad(st_out, D // 2, u * U))

        il(gmm(0), wsp_tasks(wt, U, sa[1]))
        il(gmm(1))
        il(omm(0), wsp_tasks(wn, 0, sa[0]))
        out_copy(j, 0).start()
        il(omm(1))
        out_copy(j, 1).start()

    def keep(j):
        r = pl.ds(pl.multiple_of(j * 8, 8), 8)
        v = z1_s[r, 0:128] | pltpu.bitcast(h_s[r, 0:128], u32) | pltpu.bitcast(bias_s[r, 0:128], u32)
        for b in (z2n_p, *xa, *oa, *ha, *sa, *ya, wo_t, wq_p, wk_p, wv_p, wo_p, wz1_p, wz2_p, wout_p):
            v = v | (b[j, 0:8, 0:128] if len(b.shape) == 3 else b[r, 0:128])
        v = v | pltpu.bitcast(sum(b[j % 2, 0:8, :] for b in k_s + v_s + p_s + st_x + st_h + st_z) + sum(t[r, :] for t in tmp) + sum(t[0, r, :] for t in l_s + e_s) + q_s[r, 0:128] + z2_s[0][r, 0:128] + z2_s[1][r, 0:128], u32)
        x_s[0:16, 0:128] = _as_bf16(v)
        c = cp(x_s.at[0:16, 0:128], out_hbm.at[0, 0:16, 0:128], 0)
        c.start()
        c.wait()

    def make_zero():
        bits = pltpu.bitcast(x_s[0:16, 0:128], jnp.int32)
        zero.append(bits[0, 0] ^ pltpu.roll(bits, 1, 1)[0, 1])

    if cfg["part"] in ("s1", "s2"):
        make_zero()
    if cfg["part"] == "s1":
        pl.loop(1, nstep)(lambda i: step1(i, False))
        pl.loop(0, 4)(keep)
        return
    if cfg["part"] == "s2":
        pl.loop(0, nstep)(step2)
        for j in range(nstep):
            for u in range(2):
                out_copy(j, u).wait()
        pl.loop(0, 4)(keep)
        return
    dma["x0"].start()
    dma["wq"].start()
    dma["x0"].wait()
    make_zero()
    _run(ln_a_tasks(x_s, g_x, 0, st_x[0], xa[0], cfg["qkv"]))
    dma["wq"].wait()
    dma["wk"].start()
    _run(prep_qkv_tasks(0, wq_p))
    step1(0, True)
    if cfg["part"] == "first":
        pl.loop(0, 4)(keep)
        return
    if cfg["unroll1"]:
        for i in range(1, nstep):
            step1(i, False)
    else:
        pl.loop(1, nstep)(lambda i: step1(i, False))
    if cfg["unroll2"]:
        for j in range(nstep):
            step2(j)
    else:
        pl.loop(0, nstep)(step2)
    for j in range(nstep):
        for u in range(2):
            out_copy(j, u).wait()


def build(cfg, interpret=False, name="fused_block"):
    dummy = (8, 128)

    def vm(shape, dt):
        return pltpu.VMEM(shape, dt)

    def opt(shape, on):
        return vm(shape if on else dummy, u32)

    scratch = [
        vm((S + 16, D), bf16),
        vm((D + 16, D), bf16), vm((D + 16, D), bf16), vm((D + 16, D), bf16),
        vm((D + 16, D), bf16),
        vm((D + 16, FH), bf16), vm((D + 16, FH), bf16),
        vm((S + 16, S), bf16),
        vm((S,), bf16),
        vm((FH + 16, D), bf16),
        vm(_b_shape(D, D, cfg["qkv"]), u32),
        vm(_b_shape(D, D, cfg["qkv"]), u32),
        vm(_b_shape(D, D, cfg["qkv"]), u32),
        opt((D // 2 + 8, D), cfg["wo"]),
        vm(_b_shape(D, D, cfg["wo"]), u32),
        opt(_b_shape(D, FH, True), cfg["win"]),
        opt(_b_shape(D, FH, True), cfg["win"]),
        opt(_b_shape(FH, D, True), cfg["out"]),
        vm(_b_shape(S, FH, cfg["sp"]), u32),
        vm((S + 8, D), f32),
        vm((S // 2, FH), u32),
        vm((S, 128), f32),
    ]
    for k, key in ((D, "qkv"), (D, "wo"), (D, "win"), (S, "sp"), (FH, "out")):
        scratch += [vm(_a_shape(k, cfg[key]), u32)] * 2
    scratch += [
        vm((TM + 8, D), f32),
        *[vm((NT, HALO + U + 8, 128), f32)] * 4,
        *[vm((WIN, U + 8, 128), f32)] * 2,
        *[vm((U + 8, FH), f32)] * 2,
        *[vm((3, U + 8, 128), f32)] * 6,
        *[vm((HU, 128), f32)] * 5,
        *[vm((2, U + 8, 128), f32)] * 4,
        pltpu.SemaphoreType.DMA((11,)),
        pltpu.SemaphoreType.DMA((2 * (S // TM),)),
    ]
    hbm = pl.BlockSpec(memory_space=pl.ANY)
    return pl.pallas_call(
        functools.partial(_kernel, cfg),
        out_shape=jax.ShapeDtypeStruct((1, S, D), bf16),
        in_specs=[hbm] * 7,
        out_specs=hbm,
        scratch_shapes=scratch,
        compiler_params=pltpu.CompilerParams(vmem_limit_bytes=126 * 1024 * 1024, flags=cfg['flags']),
        interpret=interpret,
        name=name,
    )


@jax.jit
def pallas_sequential_preLN__sliding_local_dilated__mixer_gmlp__prompt_kernel(
    A_x: jax.Array,
    A_wqkv: jax.Array,
    A_wo: jax.Array,
    B_x: jax.Array,
    B_w_in: jax.Array,
    B_w_sp: jax.Array,
    B_b_sp: jax.Array,
    B_w_out: jax.Array,
):
    del B_x
    return build(CFG)(A_x, A_wqkv, A_wo, B_w_in, B_w_sp, B_b_sp, B_w_out)
```

```python
import functools

import jax
import jax.numpy as jnp
import numpy as np
from jax import lax
from jax.experimental import pallas as pl
from jax.experimental.pallas import tpu as pltpu

S = 2048
D = 1024
FH = 1792
DH = 32
WIN = 8
DIL = 2
HALO = 16
U = 256
NU = S // U
NT = D // 128
EPS = 1e-5

f32 = jnp.float32
bf16 = jnp.bfloat16
u32 = jnp.uint32

CFG = dict(part="all", flags=None, qkv=1, wo=1, win=2, sp=2, out=2, slot=32,
           lat_short=320, lat_xlu=448, tail=0, regs=False, cw_wo=128, cut_prep=5, z_over=20, peel=False)

ORDER = (0, 3, 1, 2, 5, 4, 6)
REST = (3, 1, 2, 4)


def _pack(v):
    return pltpu.bitcast(v.astype(bf16), u32)


def _as_bf16(v):
    return pltpu.bitcast(v, bf16)


def _unpack(v):
    return pltpu.bitcast(v, bf16).astype(f32)


_C = float(np.sqrt(2.0 / np.pi))
ALPHA = float((_C * 0.044715) ** (1.0 / 3.0))
GAIN = 2.0 * ALPHA


def _gelu(v):
    return v * (1.0 + jnp.tanh(v * (_C / ALPHA + v * v)))


LEFT = (((1, 0, 0), (1, 1, 1)), ((1, 1, 0), (1, 1, 1)), ((1, 0, 0),), ((1, 1, 1),),
        ((1, 0, 0), (1, 0, 1)), ((1, 1, 0), (-1, 0, 0)), ((1, 0, 1), (-1, 1, 1)))
RIGHT = (((1, 0, 0), (1, 1, 1)), ((1, 0, 0),), ((1, 0, 1), (-1, 1, 1)), ((1, 1, 0), (-1, 0, 0)),
         ((1, 1, 1),), ((1, 0, 0), (1, 0, 1)), ((1, 1, 0), (1, 1, 1)))


def _factor(terms, get):
    v = get(*terms[0][1:])
    for sign, i, j in terms[1:]:
        v = v + get(i, j) if sign > 0 else v - get(i, j)
    return v


def _factors(forms, get):
    blk = {(i, j): get(i, j) for i in range(2) for j in range(2)}
    return [_factor(terms, lambda i, j: blk[i, j]) for terms in forms]


class _Held:
    def __setitem__(self, _, v):
        self.v = v

    def __getitem__(self, _):
        return self.v


def _combiner(tmp, put):
    t1, t2, t3, t4, t5 = tmp

    def feed(i, m):
        if i == 0:
            t1[...] = m
        elif i == 3:
            t4[...] = m
        elif i == 1:
            t2[...] = m
            put(1, 0, m + t4[...])
        elif i == 2:
            t3[...] = m
        elif i == 5:
            put(1, 1, (t1[...] - t2[...] + t3[...]) + m)
        elif i == 4:
            t5[...] = m
            put(0, 1, m + t3[...])
        else:
            put(0, 0, (t1[...] + t4[...] - t5[...]) + m)
    return feed


class _Split:
    def __init__(self, n, level):
        self.level, self.parts = level, 1 << level
        self.width = n // self.parts // 128 * 128
        self.rest = n // 2 - 2 * self.width if level == 2 else 0
        self.half = n // 2

    def start(self, j):
        if self.level == 1:
            return j * self.half
        return (j // 2) * self.half + (j % 2) * self.width

    def rest_start(self, h):
        return h * self.half + 2 * self.width


def _pair_transpose(v):
    sub = lax.broadcasted_iota(jnp.int32, v[0].shape, 0)
    v = list(v)
    for b in range(2):
        s = 1 << b
        m = (sub & (2 * s)) != 0
        nv = list(v)
        for j in range(4):
            if j & s:
                continue
            lo, hi = v[j], v[j + s]
            nv[j] = jnp.where(m, pltpu.roll(hi, 2 * s, 0), lo)
            nv[j + s] = jnp.where(m, hi, pltpu.roll(lo, 8 - 2 * s, 0))
        v = nv
    return v


def _ds(start, size, align):
    return pl.ds(start if isinstance(start, int) else pl.multiple_of(start, align), size)


def _kernel(cfg,
            x_hbm, wqkv_hbm, wo_hbm, win_hbm, wsp_hbm, bsp_hbm, wout_hbm, out_hbm,
            x_s, raw, bsp_raw,
            wq_p, wk_p, wv_p, wo_p, wz1_p, wz1_r, wz2_p, wz2_r, wout_p, wout_r, z2n_p, z2n_r,
            z1_s, bias_s, xa, xb, oa, ha, sa, ya,
            q_s, o_s, k_s, v_s, p_s, l_s, e_s, z_s, zn_s, sp_s, st0, st1, tmp_s,
            sem, osem):
    zero = []

    def spot(ref, row, col):
        n = 8 * (4 // ref.dtype.itemsize)
        ref = ref if len(ref.shape) == 2 else ref.at[zero[0]]
        return ref.at[_ds(row + zero[0] * n, n, n), _ds(col + zero[0] * 128, 128, 128)]

    def gate(ref, v):
        n = 8 * (4 // ref.dtype.itemsize)
        spot(ref, ref.shape[-2] - n, 0)[0:8, :] = v.astype(ref.dtype)

    def done(ref, row, col):
        v = spot(ref, row, col)[...]
        return v if v.dtype == u32 else pltpu.bitcast(v, u32)

    def tied(toks):
        def tie(b):
            if not toks:
                return b
            tok = functools.reduce(lambda p, q: p | q, toks)
            tok = jnp.concatenate([tok] * (b.shape[1] // 128), axis=1)
            always = lax.broadcasted_iota(jnp.int32, tok.shape, 0) >= zero[0]
            parts = []
            for r in range(0, b.shape[0], 64):
                parts += [b[r:r + 56], jnp.where(always, b[r + 56:r + 64], tok)]
            return jnp.concatenate(parts, axis=0)
        return tie

    def overlap(main, *sides):
        n, cyc, gen = main
        per = max(1, cyc // cfg["slot"])
        plan = [[] for _ in range(n * per)]
        for side in sides:
            if not isinstance(side, tuple):
                side = (side, 0, n)
            todo, first, last = side
            if todo and last == n:
                last -= (todo[-1][2] + cfg["tail"]) / cyc
            span = max(1, int((last - first) * per))
            for j, t in enumerate(todo):
                plan[int(first * per) + j * span // len(todo)].append(t)
        next(gen)
        due = [[] for _ in range(n)]
        for i, todo in enumerate(plan):
            if i % per == 0:
                res = gen.send(tied([tok for _, tok in due[i // per]]))
            gated = []
            for _, refs, _ in todo:
                gated += [r for r in refs if not any(r is g for g in gated)]
            row = res.shape[0] * (i % per) // per
            for r in gated:
                gate(r, res[row:row + 8, 0:128])
            for fn, _, lat in todo:
                where = fn()
                j = -(-(i * cyc // per + lat) // cyc)
                if where is not None and j < n:
                    due[j] = [d for d in due[j] if d[0] is not where[0]]
                    due[j].append((where[0], done(*where)))

    def tasks(fn, args, refs, lat):
        return [(functools.partial(fn, *a), refs, cfg[lat]) for a in args]

    def run(todo):
        for t in todo:
            t[0]()

    def left_tasks(ref, key, k, load, refs, rows=None, cols=None, outer=None, rest=True):
        ks = _Split(k, cfg[key])
        h = U // ks.parts

        def put(n, r, c, v):
            ref[_ds(n * h // 2 + r // 2, 8, 8), c:c + 128] = _pack(v)

        def main(r, c, o):
            def get(i, j):
                if ks.level == 1:
                    return load(i * h + r, j, ks.start(j) + c)
                return _factor(LEFT[o], lambda a, b: load((2 * a + i) * h + r, 2 * b + j,
                                                          ks.start(2 * b + j) + c))
            for n, v in enumerate(_factors(LEFT, get)):
                put(7 * o + n, r, c, v)
            return ref, 7 * o * h // 2 + r // 2, c

        def other(r, i):
            vals = _factors(LEFT, lambda a, b: load((2 * a + i) * h + r, None, ks.rest_start(b)))
            for o, v in enumerate(vals):
                put(7 * o + 6 - i, r, ks.width, v)
            return ref, (6 - i) * h // 2 + r // 2, ks.width
        out = []
        for r in range(0, h, 16) if rows is None else rows:
            out += tasks(main, [(r, c, o)
                                for c in (range(0, ks.width, 128) if cols is None else cols)
                                for o in (range(7 ** (ks.level - 1)) if outer is None else outer)],
                         refs, "lat_short")
            out += tasks(other, [(r, 0), (r, 1)] if ks.rest and rest else [], refs, "lat_short")
        return out

    def right_tasks(bufs, key, n, rows, load, refs):
        main_p, rest_p = bufs
        ns = _Split(n, cfg[key])

        def main(prow, r, c, o):
            def get(i, j):
                if ns.level == 1:
                    return load(i, r, ns.start(j) + c)
                return _factor(RIGHT[o], lambda a, b: load(2 * a + i, r, ns.start(2 * b + j) + c))
            for m, v in enumerate(_factors(RIGHT, get)):
                main_p.at[7 * o + m][_ds(prow, 8, 8), c:c + 128] = _pack(v)
            return main_p, prow, c

        def rest(prow, r, o):
            top, bot = [_factor(RIGHT[o], lambda a, b: load(2 * a + i, r, ns.rest_start(b)))
                        for i in range(2)]
            for m, v in enumerate((top, bot, top - bot)):
                rest_p.at[3 * o + m][_ds(prow, 8, 8), :] = _pack(v)
            return rest_p, prow, 0
        out = []
        for prow, r in rows:
            out += tasks(main, [(prow, r, c, o) for c in range(0, ns.width, 128)
                                for o in range(7 ** (ns.level - 1))], refs, "lat_short")
            out += tasks(rest, [(prow, r, o) for o in range(7)] if ns.rest else [], refs,
                         "lat_short")
        return out

    def matmul(ref, bufs, key, k, n, store, cw=128, rest_first=False):
        main_p, rest_p = bufs
        ks, ns = _Split(k, cfg[key]), _Split(n, cfg[key])
        h = U // ks.parts

        def lhs(m, lo, hi):
            return _as_bf16(ref[m * h // 2:(m + 1) * h // 2, lo:hi])

        def dot(a, b):
            return jnp.dot(a, _as_bf16(b), preferred_element_type=f32)

        def temps(slot):
            return [tmp_s.at[(5 * slot + j) * h:(5 * slot + j + 1) * h, 0:cw] for j in range(5)]

        def gen1():
            tie = yield
            for c in range(0, ns.width, cw):
                feed = _combiner(temps(0), lambda i, j, v: store(i * h, ns.start(j) + c, v))
                for m in ORDER:
                    res = dot(lhs(m, 0, ks.width), tie(main_p.at[m][:, c:c + cw]))
                    feed(m, res)
                    tie = yield res

        def inner_temps():
            return [_Held() for _ in range(5)] if cfg["regs"] else temps(4)

        def chunk(c, tie):
            def put(i, j):
                return lambda a, b, v: store((2 * a + i) * h, ns.start(2 * b + j) + c, v)
            outer = {(i, j): _combiner(temps(2 * i + j), put(i, j))
                     for i in range(2) for j in range(2)}
            for o in ORDER:
                def extra(i, j, v):
                    if ks.rest and i != j:
                        v = v + dot(lhs(7 * o + 6 - i, ks.width, ks.width + 128),
                                    rest_p.at[2 * o + j][:, c:c + cw])
                    outer[i, j](o, v)
                feed = _combiner(inner_temps(), extra)
                for m in ORDER:
                    b = main_p.at[7 * o + m][:, c:c + cw]
                    hi = ks.width
                    if ks.rest and m >= 5:
                        b = jnp.concatenate([b, rest_p.at[2 * o + 6 - m][:, c:c + cw]], axis=0)
                        hi += 128
                    res = dot(lhs(7 * o + m, 0, hi), tie(b))
                    feed(m, res)
                    tie = yield res
            return tie

        def rest_chunk(tie):
            def put(i):
                return lambda a, b, v: store((2 * a + i) * h, ns.rest_start(b), v)
            outer = [_combiner(temps(i), put(i)) for i in range(2)]
            for o in ORDER:
                for i, (m0, b0), (m1, b1) in ((1, (3, 2), (1, 0)), (0, (2, 2), (4, 1))):
                    first = dot(lhs(7 * o + m0, 0, ks.width), tie(rest_p.at[3 * o + b0][...]))
                    tie = yield first
                    res = dot(lhs(7 * o + m1, 0, ks.width), tie(rest_p.at[3 * o + b1][...]))
                    outer[i](o, res - first if i else res + first)
                    tie = yield res
            return tie

        def gen2():
            tie = yield
            if ns.rest and rest_first:
                tie = yield from rest_chunk(tie)
            for c in range(0, ns.width, cw):
                tie = yield from chunk(c, tie)
            if ns.rest and not rest_first:
                tie = yield from rest_chunk(tie)
        cyc = h // 16 * 4 * (ks.width // 128) * (cw // 128)
        if ks.level == 1:
            return 7 * (ns.width // cw), cyc, gen1()
        return 49 * (ns.width // cw) + (28 if ns.rest else 0), cyc, gen2()

    def staged(i):
        return (z_s, zn_s)[i].at[0:D // 4, 0:D]

    def mix_staged(buf, shift):
        def task(r, t):
            def get(i, j):
                tile = j * NT // 2 + t
                v = pltpu.bitcast(staged(i)[r:r + 8, tile * 128:(tile + 1) * 128], u32)
                return _unpack(pltpu.roll(v, 128 - 4 * tile, 1) if shift and tile else v)
            for m, v in enumerate(_factors(RIGHT, get)):
                buf.at[m][r:r + 8, t * 128:(t + 1) * 128] = _pack(v)
            return buf, r, t * 128
        return tasks(task, [(r, t) for r in range(0, D // 4, 8) for t in range(NT // 2)],
                     [z_s, zn_s], "lat_xlu" if shift else "lat_short")

    def prep_qkv(j, buf, rows=range(0, D // 2, 16)):
        def task(i, r):
            w = pltpu.bitcast(raw.at[j][i * D // 2 + r:i * D // 2 + r + 16, :], u32)
            lane = lax.broadcasted_iota(jnp.int32, (8, 128), 1)
            w = [w[:, t * 128:(t + 1) * 128] for t in range(NT)]
            w = [pltpu.roll(v, 4 * t, 1) if t else v for t, v in enumerate(w)]
            w = [w[(-t) % NT] for t in range(NT)]
            for b in range(3):
                m = (lane & (4 << b)) != 0
                w = [jnp.where(m, w[(t - (1 << b)) % NT], w[t]) for t in range(NT)]
            for t in range(NT):
                staged(i)[r // 2:r // 2 + 8, t * 128:(t + 1) * 128] = pltpu.bitcast(w[t], f32)
            return (z_s, zn_s)[i], r // 2, 0
        second = mix_staged(buf, True)
        return (tasks(task, [(i, r) for r in rows for i in range(2)], [raw], "lat_xlu"),
                [second[r // 16 * NT // 2 + t] for r in rows for t in range(NT // 2)])

    def prep_wo():
        def task(d4, t2, hh, c):
            src = [((t2 * 4 + j) * 4 + hh) * 32 + d4 * 16 for j in range(4)]
            v = _pair_transpose([pltpu.bitcast(raw.at[3][s:s + 16, c:c + 256], u32) for s in src])
            for j in range(4):
                r = ((j * 4 + hh) * 32 + t2 * 16) // 2
                staged(d4)[r:r + 8, c:c + 256] = pltpu.bitcast(v[j], f32)
            return (z_s, zn_s)[d4], r, c
        return tasks(task, [(d4, t2, hh, c) for d4 in range(2) for t2 in range(2)
                            for hh in range(4) for c in range(0, D, 256)],
                     [raw], "lat_short") + mix_staged(wo_p, False)

    def prep_win(slab, bufs, first, count):
        ks = _Split(D, cfg["win"])

        def load(i, r, c):
            return raw.at[slab + c // (FH // 2)][
                _ds(ks.start(i) + r, 16, 16), c % (FH // 2):c % (FH // 2) + 128].astype(f32)
        rows = [((first + g) * 8, (first + g) * 16) for g in range(count)]
        return right_tasks(bufs, "win", FH, rows, load, [raw])

    def prep_wout(first, count):
        ks = _Split(FH, cfg["out"])

        def load(i, r, c):
            row = ks.start(i)
            return raw.at[2 + row // (FH // 2)][
                _ds(row % (FH // 2) + r, 16, 16), c:c + 128].astype(f32)
        rows = [((first + g) * 8, (first + g) * 16) for g in range(count)]
        return right_tasks((wout_p, None), "out", D, rows, load, [raw])

    def prep_wout_rest(first, count):
        ks, ns = _Split(FH, cfg["out"]), _Split(D, cfg["out"])

        def task(g, j, c):
            def get(a, b):
                col = ns.start(2 * b + j) + c
                return raw.at[2 + a][_ds(2 * ks.width + (first + g) * 16, 16, 16),
                                     col:col + 128].astype(f32)
            for o, v in enumerate(_factors(RIGHT, get)):
                wout_r.at[2 * o + j][_ds((first + g) * 8, 8, 8), c:c + 128] = _pack(v)
            return wout_r, (first + g) * 8, c
        if not ks.rest:
            return []
        return tasks(task, [(g, j, c) for g in range(count) for j in range(2)
                            for c in range(0, ns.width, 128)], [raw], "lat_short")

    def prep_bias():
        def task(j):
            b = bsp_raw[...].astype(f32).reshape(1, S) * (1.0 / GAIN)
            bias_s[j * 128:(j + 1) * 128, :] = jnp.broadcast_to(
                b[:, j * 128:(j + 1) * 128], (128, 128)).T
            return bias_s, j * 128, 0
        return tasks(task, [(j,) for j in range(S // 128)], [], "lat_xlu")

    def norm_tasks(base, src, st, eps=EPS, scale=None, rows=range(0, U, 16)):
        n = src.shape[1]

        def shift(r):
            v = src[_ds(r, 16, 16), 0:128].astype(f32)
            st.at[0][_ds(r, 16, 16), :] = jnp.broadcast_to(v[:, 0:1], (16, 128))
            return st, r, 0

        def stats(r):
            sh = st.at[0][_ds(r, 8, 8), :]
            s1 = s2 = None
            for c in range(0, n, 256):
                v = src[_ds(r, 8, 8), c:c + 256].astype(f32)
                for d in (v[:, :128] - sh, v[:, 128:] - sh):
                    s1 = d if s1 is None else s1 + d
                    s2 = d * d if s2 is None else s2 + d * d
            m = jnp.sum(s1, axis=-1, keepdims=True) * (1.0 / n)
            var = jnp.sum(s2, axis=-1, keepdims=True) * (1.0 / n) - m * m
            st.at[1][_ds(r, 8, 8), :] = sh + m
            st.at[2][_ds(r, 8, 8), :] = jnp.broadcast_to(jnp.maximum(var, 0.0) + eps, (8, 128))
            return st, r, 0

        def rstd(r):
            v = lax.rsqrt(st.at[2][_ds(r, 16, 16), :])
            st.at[0][_ds(r, 16, 16), :] = v if scale is None else v * scale
            return st, r, 0

        def load(r, c, h=16, w=128):
            v = src[_ds(r, h, h), c:c + w].astype(f32)
            mean, inv = [jnp.concatenate([st.at[j][_ds(r, h, h), :]] * (w // 128), axis=1)
                         for j in (1, 0)]
            return (v - mean) * inv

        def write(dst):
            def task(r, c, w):
                dst[_ds(r, 8, 8), c:c + w] = load(r, c, 8, w)
                return dst, r, c
            return tasks(task, [(r + j, c, min(1024, n - c)) for r in rows for j in (0, 8)
                                for c in range(0, n, 1024)], [base], "lat_short")
        out = tasks(shift, [(r,) for r in rows], [base], "lat_xlu")
        out += tasks(stats, [(r + j,) for r in rows for j in (0, 8)], [base], "lat_xlu")
        out += tasks(rstd, [(r,) for r in rows], [st], "lat_short")
        return out, load, write

    def norm_x(u, buf):
        out, load, _ = norm_tasks(x_s, unit(x_s, u), st0)
        return out + left_tasks(buf, "qkv", D, lambda r, j, c: load(r, c), [x_s])

    def norm_h(u, spare, **kw):
        out, _, write = norm_tasks(x_s, unit(x_s, u), st1, scale=ALPHA, **kw)
        return out + write(spare)

    def left_h(spare, **kw):
        return left_tasks(ha, "win", D, lambda r, j, c: spare[_ds(r, 16, 16), c:c + 128], [spare],
                          **kw)

    def take(v, idx):
        return jnp.take_along_axis(v, idx, axis=1)

    def logit_tasks(first):
        def task(r, b):
            lane = lax.broadcasted_iota(jnp.int32, (8, 128), 1)
            acc = [None] * 4
            for t in range(NT):
                q = q_s[r:r + 8, t * 128:(t + 1) * 128]
                for j in range(4):
                    k0 = HALO + r - DIL * (4 * b + j)
                    term = q * k_s[t, k0:k0 + 8, :]
                    acc[j] = term if t == 0 else acc[j] + term
            for bit in (1, 2):
                odd = (lane & bit) != 0
                acc = [jnp.where(odd, acc[j ^ bit], acc[j]) for j in range(4)]
            lg = acc[0]
            for j in range(1, 4):
                lg = lg + take(acc[j], lane ^ j)
            lg = lg * float(DH) ** -0.5
            if first and r < DIL * WIN:
                pos = r + lax.broadcasted_iota(jnp.int32, (8, 128), 0)
                lg = jnp.where(pos >= DIL * (4 * b + (lane & 3)), lg, -1e9)
            l_s[b, r:r + 8, :] = lg
            return l_s, r, 0
        return tasks(task, [(r, b) for r in range(0, U, 8) for b in range(2)], [q_s, k_s],
                     "lat_xlu")

    def softmax_tasks():
        def exps(r):
            lane = lax.broadcasted_iota(jnp.int32, (16, 128), 1)
            lg = [l_s[b, r:r + 16, :] for b in range(2)]
            mx = jnp.maximum(lg[0], lg[1])
            mx = functools.reduce(jnp.maximum, [mx] + [take(mx, lane ^ j) for j in range(1, 4)])
            for b in range(2):
                e_s[b, r:r + 16, :] = jnp.exp(lg[b] - mx)
            return e_s, r, 0

        def probs(r):
            lane = lax.broadcasted_iota(jnp.int32, (8, 128), 1)
            e = [e_s[b, r:r + 8, :] for b in range(2)]
            e = {4 * b + j: take(e[b], (lane & -4) | j) for j in range(4) for b in range(2)}
            inv = 1.0 / functools.reduce(lambda p, q: p + q, e.values())
            for w in range(WIN):
                p_s[w, r:r + 8, :] = e[w] * inv
            return p_s, r, 0
        return (tasks(exps, [(r,) for r in range(0, U, 16)], [l_s], "lat_xlu")
                + tasks(probs, [(r,) for r in range(0, U, 8)], [e_s], "lat_xlu"))

    def value_tasks():
        def task(r, t0):
            acc = [None] * 4
            for w in range(WIN):
                k0 = HALO + r - DIL * w
                p = p_s[w, r:r + 8, :]
                for j in range(4):
                    term = p * v_s[t0 + j, k0:k0 + 8, :]
                    acc[j] = term if w == 0 else acc[j] + term
            for j in range(4):
                o_s[r:r + 8, (t0 + j) * 128:(t0 + j + 1) * 128] = acc[j]
            return o_s, r, t0 * 128
        out = []
        for g in range(0, U // 2 + 16, 16):
            if g < U // 2:
                out += tasks(task, [(g + b + j, t0) for b in (0, U // 2) for j in (0, 8)
                                    for t0 in (0, 4)], [p_s, v_s], "lat_short")
            if g:
                out += left_tasks(oa, "wo", D, lambda r, j, c: o_s[r:r + 16, c:c + 128], [o_s],
                                  rows=[g - 16])
        return out

    def set_halo(buf, first):
        buf[:, 0:HALO, :] = jnp.zeros((NT, HALO, 128), f32) if first else buf[:, U:U + HALO, :]

    def copies(name):
        half = FH // 2
        early = share(0, NU - 1, _Split(D, cfg["win"]).width // 16)[1] * 16

        def win_rows(lo, hi):
            return [(win_hbm.at[r + lo:r + hi, j * half:(j + 1) * half],
                     raw.at[4 + j, r + lo:r + hi, 0:half])
                    for r in range(0, D, D // 4) for j in range(4)]
        pairs = dict(
            x0=[(x_hbm.at[0, 0:U], x_s.at[0:U])],
            wq=[(wqkv_hbm.at[:, 0:D], raw.at[0, 0:D])],
            wk=[(wqkv_hbm.at[:, D:2 * D], raw.at[1, 0:D])],
            wv=[(wqkv_hbm.at[:, 2 * D:3 * D], raw.at[2, 0:D])],
            wo=[(wo_hbm, raw.at[3, 0:D]), (x_hbm.at[0, U:2 * U], x_s.at[U:2 * U])],
            rest0=[(x_hbm.at[0, 2 * U:3 * U], x_s.at[2 * U:3 * U])] + win_rows(0, early),
            rest1=[(x_hbm.at[0, 3 * U:S], x_s.at[3 * U:S])] + win_rows(early, D // 4),
            rest2=[(wsp_hbm.at[0:D, j * D:(j + 1) * D], raw.at[j, 0:D]) for j in range(2)]
            + [(wout_hbm.at[j * half:(j + 1) * half], raw.at[2 + j, 0:half]) for j in range(2)]
            + [(bsp_hbm, bsp_raw)],
            rest3=[(wsp_hbm.at[D:S, j * D:(j + 1) * D], raw.at[4 + j, 0:D]) for j in range(2)],
        )
        j = list(pairs).index(name)
        return [pltpu.make_async_copy(a, b, sem.at[j]) for a, b in pairs[name]]

    def start(name):
        for c in copies(name):
            c.start()

    def wait(name):
        for c in copies(name):
            c.wait()

    def out_copy(u):
        rows = _ds(u * U, U, U)
        return pltpu.make_async_copy(x_s.at[rows], out_hbm.at[0, rows], osem.at[u])

    def unit(ref, u, n=U):
        return ref.at[_ds(u * n, n, n)]

    def clip(v, lo, hi):
        return min(max(v, lo), hi) if isinstance(v, int) else jnp.clip(v, lo, hi)

    def share(step, steps, total):
        count = -(-total // steps)
        return clip(step * count, 0, total - count), count

    def add_into(u):
        def store(r, c, v):
            idx = (slice(r, r + v.shape[0]), slice(c, c + v.shape[1]))
            dst = unit(x_s, u)
            dst[idx] = (dst[idx].astype(f32) + v).astype(bf16)
        return store

    def put_q(r, c, v):
        q_s[r:r + v.shape[0], c:c + 128] = v

    def put_slab(buf):
        def store(r, c, v):
            buf[c // 128, HALO + r:HALO + r + v.shape[0], :] = v
        return store

    def qkv(src, w, store):
        return matmul(src, (w, None), "qkv", D, D, store)

    def project(u):
        return matmul(oa, (wo_p, None), "wo", D, D, add_into(u), cfg["cw_wo"])

    def first_attention():
        set_halo(k_s, True)
        set_halo(v_s, True)
        start("wv")
        wait("wk")
        overlap(qkv(xb, wq_p, put_q), sum(prep_qkv(1, wk_p), []))
        start("wo")
        wait("wv")
        overlap(qkv(xb, wk_p, put_slab(k_s)), sum(prep_qkv(2, wv_p), []))
        start("rest0")
        wait("wo")
        overlap(qkv(xb, wv_p, put_slab(v_s)), logit_tasks(True), prep_wo() + norm_x(1, xa))

    def step_attention(u):
        if cfg["part"] != "s1":
            @pl.when(u == 2)
            def _():
                wait("rest1")
                start("rest2")
        begin, count = share(u - 1, NU - 1, _Split(D, cfg["win"]).width // 16)
        prep = (prep_win(6, (wz2_p, wz2_r), begin, count)
                + prep_win(4, (wz1_p, wz1_r), begin, count))
        cut = len(prep) * cfg["cut_prep"] // 8
        g = clip(u - 2, 0, U // 64 - 1) * 16
        head = norm_h(0, z_s, rows=[g + b for b in range(0, U, 64)]) + left_h(z_s, rows=[g])
        logits = logit_tasks(False)
        set_halo(k_s, False)
        overlap(qkv(xa, wq_p, put_q), softmax_tasks(), prep[:cut])
        overlap(qkv(xa, wk_p, put_slab(k_s)), value_tasks())
        set_halo(v_s, False)
        overlap(qkv(xa, wv_p, put_slab(v_s)), logits, head)
        overlap(project(u - 1), norm_x(clip(u + 1, 0, NU - 1), xa), prep[cut:])

    def spatial_left(u, rows=range(0, U // 4, 16)):
        per = D // U

        def regroup(r, m):
            lane = lax.broadcasted_iota(jnp.int32, (8, 128), 1)
            col = 2 * U * m
            w = pltpu.bitcast(raw.at[u // per * 4 + col // D][
                _ds(u % per * U + r, 16, 16), col % D:col % D + 2 * U], u32)
            for a in range(2):
                one, two = w[:, a * 128:(a + 1) * 128], w[:, U + a * 128:U + (a + 1) * 128]
                mid = pltpu.roll(jnp.where(lane < 64, two, one), 64, 1)
                for j, v in ((2 * a, jnp.where(lane < 64, one, mid)),
                             (2 * a + 1, jnp.where(lane < 64, mid, two))):
                    sp_s[_ds(r // 2, 8, 8), j * 512 + m * 128:j * 512 + (m + 1) * 128] = v
            return sp_s, r // 2, m * 128
        return tasks(regroup, [(b + r, m) for r in rows for b in range(0, U, U // 4)
                               for m in range(NU // 2)], [raw], "lat_xlu") + left_tasks(
            sa, "sp", S, lambda r, j, c: _unpack(sp_s[_ds(r // 2, 8, 8), c:c + 128]), [sp_s],
            rows=rows)

    def step_input(u):
        z1t = unit(z1_s, u, U // 2)
        h = U // 4
        lag = 1 if cfg['peel'] else 0

        def put_z1(r, c, v):
            z1t[r // 2:(r + v.shape[0]) // 2, c:c + 128] = _pack(_gelu(v))

        def put_z2(r, c, v):
            z_s[r:r + v.shape[0], c:c + 128] = _gelu(v)
        stats, _, write = norm_tasks(z_s, z_s, st0, EPS * GAIN * GAIN, 1.0 / GAIN)
        factors = right_tasks((z2n_p, z2n_r), "sp", FH,
                              [(u * (h // 2) + r // 2, r) for r in range(0, h, 16)],
                              lambda b, r, c: zn_s[b * h + r:b * h + r + 16, c:c + 128], [zn_s])
        gate_in = matmul(ha, (wz2_p, wz2_r), "win", D, FH, put_z2)
        upcoming = norm_h(clip(u + 1, 0, NU - 1), q_s)
        if isinstance(u, int):
            overlap(gate_in, softmax_tasks() + value_tasks())
            overlap(project(NU - 1), upcoming, prep_bias())
        else:
            prep = (prep_wout(*share(u - lag, NU - lag, _Split(FH, cfg["out"]).width // 16))
                    + prep_wout_rest(*share(u - lag, NU - lag, 8))
                    + spatial_left(0, [share(u - lag, NU - lag, h // 16)[0] * 16]))
            overlap(gate_in, upcoming, prep)
        main = matmul(ha, (wz1_p, wz1_r), "win", D, FH, put_z1, rest_first=True)
        last = main[0] - 49
        overlap(main, (stats + write(zn_s) + factors, 0, last + cfg["z_over"]),
                *[(left_h(q_s, outer=[o]), last + 7 * j + 6, last + 7 * j + 12)
                  for j, o in enumerate(ORDER[:-1])])
        run(left_h(q_s, outer=ORDER[-1:]))

    def step_output(u):
        bt, z1t = unit(bias_s, u), unit(z1_s, u, U // 2)

        def put_y(r, c, g):
            n = g.shape[0]
            z_s[r:r + n, c:c + 128] = _unpack(z1t[r // 2:(r + n) // 2, c:c + 128]) * (
                g + bt[r:r + n, :])

        def gated(**kw):
            return left_tasks(ya, "out", FH, lambda r, j, c: z_s[r:r + 16, c:c + 128], [z_s], **kw)
        overlap(matmul(sa, (z2n_p, z2n_r), "sp", S, FH, put_y),
                *[(gated(cols=[128 * j], rest=False), 49 * j + 49, 49 * j + 49 + 20)
                  for j in range(3)])
        run(gated(cols=[]))
        overlap(matmul(ya, (wout_p, wout_r), "out", FH, D, add_into(u), 256),
                spatial_left(clip(u + 1, 0, NU - 1)))
        out_copy(u).start()

    def make_zero():
        bits = pltpu.bitcast(x_s[0:16, 0:128], jnp.int32)
        zero.append(bits[0, 0] ^ pltpu.roll(bits, 1, 1)[0, 1])

    def keep(j):
        v = None
        for b in (wq_p, wk_p, wv_p, wo_p, wz1_p, wz1_r, wz2_p, wz2_r, wout_p, wout_r, z2n_p,
                  z2n_r, z1_s, bias_s, xa, xb, oa, ha, sa, ya, q_s, o_s, k_s, v_s, p_s, l_s, e_s,
                  z_s, zn_s, sp_s, st0, st1, tmp_s):
            v = done(b, 0, 0) if v is None else v | done(b, 0, 0)
        x_s[0:16, 0:128] = _as_bf16(v)
        c = pltpu.make_async_copy(x_s.at[0:16, 0:128], out_hbm.at[0, 0:16, 0:128], sem.at[0])
        c.start()
        c.wait()

    if cfg["part"] in ("s1", "s2", "s3", "mid"):
        make_zero()
        if cfg["part"] == "mid":
            step_input(0)
        else:
            pl.loop(1, NU)({"s1": step_attention, "s2": step_input, "s3": step_output}[cfg["part"]])
        if cfg["part"] == "s3":
            for u in range(1, NU):
                out_copy(u).wait()
        pl.loop(0, 2)(keep)
        return
    start("x0")
    start("wq")
    wait("x0")
    make_zero()
    run(norm_x(0, xb))
    start("wk")
    wait("wq")
    run(sum(prep_qkv(0, wq_p), []))
    first_attention()
    wait("rest0")
    if cfg["part"] == "first":
        pl.loop(0, 2)(keep)
        return
    start("rest1")
    pl.loop(1, NU)(step_attention)
    start("rest3")
    wait("rest2")
    if cfg["part"] == "a":
        wait("rest3")
        pl.loop(0, 2)(keep)
        return
    if cfg["peel"]:
        step_input(0)
        pl.loop(1, NU)(step_input)
    else:
        run(softmax_tasks() + value_tasks())
        overlap(project(NU - 1), prep_bias())
        pl.loop(0, NU)(step_input)
    wait("rest3")
    pl.loop(0, NU)(step_output)
    for u in range(NU):
        out_copy(u).wait()


def build(cfg, interpret=False, name="fused_block"):
    vm = pltpu.VMEM

    def right(key, k, n):
        ks, ns = _Split(k, cfg[key]), _Split(n, cfg[key])
        main = vm((7 ** ks.level, ks.width // 2, ns.width), u32)
        if ns.rest:
            return [main, vm((21, ks.width // 2, 128), u32)]
        if ks.rest:
            return [main, vm((14, 64, ns.width), u32)]
        return [main]

    def left(key, k):
        ks = _Split(k, cfg[key])
        return vm((7 ** ks.level * U // ks.parts // 2, ks.width + ks.rest), u32)
    scratch = [
        vm((S + 16, D), bf16),
        vm((8, D + 16, D), bf16),
        vm((S,), bf16),
        *right("qkv", D, D) * 3, *right("wo", D, D),
        *right("win", D, FH), *right("win", D, FH), *right("out", FH, D), *right("sp", S, FH),
        vm((S // 2, FH), u32),
        vm((S, 128), f32),
        left("qkv", D), left("qkv", D), left("wo", D), left("win", D), left("sp", S),
        left("out", FH),
        *[vm((U + 8, D), f32)] * 2,
        *[vm((NT, HALO + U + 8, 128), f32)] * 2,
        vm((WIN, U + 8, 128), f32),
        *[vm((2, U + 8, 128), f32)] * 2,
        *[vm((U + 8, FH), f32)] * 2,
        vm((U // 2 + 8, S), u32),
        *[vm((3, U + 8, 128), f32)] * 2,
        vm((25 * U // 4, 256), f32),
        pltpu.SemaphoreType.DMA((9,)),
        pltpu.SemaphoreType.DMA((NU,)),
    ]
    hbm = pl.BlockSpec(memory_space=pl.ANY)
    return pl.pallas_call(
        functools.partial(_kernel, cfg),
        out_shape=jax.ShapeDtypeStruct((1, S, D), bf16),
        in_specs=[hbm] * 7,
        out_specs=hbm,
        scratch_shapes=scratch,
        compiler_params=pltpu.CompilerParams(vmem_limit_bytes=127 * 1024 * 1024,
                                             flags=cfg["flags"]),
        interpret=interpret,
        name=name,
    )


@jax.jit
def pallas_sequential_preLN__sliding_local_dilated__mixer_gmlp__prompt_kernel(
    A_x: jax.Array,
    A_wqkv: jax.Array,
    A_wo: jax.Array,
    B_x: jax.Array,
    B_w_in: jax.Array,
    B_w_sp: jax.Array,
    B_b_sp: jax.Array,
    B_w_out: jax.Array,
):
    del B_x
    return build(CFG)(A_x, A_wqkv, A_wo, B_w_in, B_w_sp, B_b_sp, B_w_out)
```

```python
import functools

import jax
import jax.numpy as jnp
import numpy as np
from jax import lax
from jax.experimental import pallas as pl
from jax.experimental.pallas import tpu as pltpu

S = 2048
D = 1024
FH = 1792
DH = 32
WIN = 8
DIL = 2
HALO = 16
U = 256
NU = S // U
NT = D // 128
EPS = 1e-5

f32 = jnp.float32
bf16 = jnp.bfloat16
u32 = jnp.uint32

CFG = dict(part="all", flags=None, qkv=1, wo=1, win=2, sp=2, out=2, slot=32,
           lat_short=320, lat_xlu=448, tail=0, regs=False, cw_wo=128, cut_prep=6, z_over=35, z_left=5, peel=True, wq_parts=4, depth=6, soft_end=76, prof=False)

ORDER = (0, 3, 1, 2, 5, 4, 6)
REST = (3, 1, 2, 4)


def _pack(v):
    return pltpu.bitcast(v.astype(bf16), u32)


def _as_bf16(v):
    return pltpu.bitcast(v, bf16)


def _unpack(v):
    return pltpu.bitcast(v, bf16).astype(f32)


_C = float(np.sqrt(2.0 / np.pi))
ALPHA = float((_C * 0.044715) ** (1.0 / 3.0))
GAIN = 2.0 * ALPHA


def _gelu(v):
    return v * (1.0 + jnp.tanh(v * (_C / ALPHA + v * v)))


LEFT = (((1, 0, 0), (1, 1, 1)), ((1, 1, 0), (1, 1, 1)), ((1, 0, 0),), ((1, 1, 1),),
        ((1, 0, 0), (1, 0, 1)), ((1, 1, 0), (-1, 0, 0)), ((1, 0, 1), (-1, 1, 1)))
RIGHT = (((1, 0, 0), (1, 1, 1)), ((1, 0, 0),), ((1, 0, 1), (-1, 1, 1)), ((1, 1, 0), (-1, 0, 0)),
         ((1, 1, 1),), ((1, 0, 0), (1, 0, 1)), ((1, 1, 0), (1, 1, 1)))


def _factor(terms, get):
    v = get(*terms[0][1:])
    for sign, i, j in terms[1:]:
        v = v + get(i, j) if sign > 0 else v - get(i, j)
    return v


def _factors(forms, get):
    blk = {(i, j): get(i, j) for i in range(2) for j in range(2)}
    return [_factor(terms, lambda i, j: blk[i, j]) for terms in forms]


class _Held:
    def __setitem__(self, _, v):
        self.v = v

    def __getitem__(self, _):
        return self.v


def _combiner(tmp, put):
    t1, t2, t3, t4, t5 = tmp

    def feed(i, m):
        if i == 0:
            t1[...] = m
        elif i == 3:
            t4[...] = m
        elif i == 1:
            t2[...] = m
            put(1, 0, m + t4[...])
        elif i == 2:
            t3[...] = m
        elif i == 5:
            put(1, 1, (t1[...] - t2[...] + t3[...]) + m)
        elif i == 4:
            t5[...] = m
            put(0, 1, m + t3[...])
        else:
            put(0, 0, (t1[...] + t4[...] - t5[...]) + m)
    return feed


class _Split:
    def __init__(self, n, level):
        self.level, self.parts = level, 1 << level
        self.width = n // self.parts // 128 * 128
        self.rest = n // 2 - 2 * self.width if level == 2 else 0
        self.half = n // 2

    def start(self, j):
        if self.level == 1:
            return j * self.half
        return (j // 2) * self.half + (j % 2) * self.width

    def rest_start(self, h):
        return h * self.half + 2 * self.width


def _pair_transpose(v):
    sub = lax.broadcasted_iota(jnp.int32, v[0].shape, 0)
    v = list(v)
    for b in range(2):
        s = 1 << b
        m = (sub & (2 * s)) != 0
        nv = list(v)
        for j in range(4):
            if j & s:
                continue
            lo, hi = v[j], v[j + s]
            nv[j] = jnp.where(m, pltpu.roll(hi, 2 * s, 0), lo)
            nv[j + s] = jnp.where(m, hi, pltpu.roll(lo, 8 - 2 * s, 0))
        v = nv
    return v


def _ds(start, size, align):
    return pl.ds(start if isinstance(start, int) else pl.multiple_of(start, align), size)


def _kernel(cfg,
            x_hbm, wqkv_hbm, wo_hbm, win_hbm, wsp_hbm, bsp_hbm, wout_hbm, out_hbm,
            x_s, raw, bsp_raw,
            wq_p, wk_p, wv_p, wo_p, wz1_p, wz1_r, wz2_p, wz2_r, wout_p, wout_r, z2n_p, z2n_r,
            z1_s, bias_s, xa, xb, oa, ha, sa, ya,
            q_s, o_s, k_s, v_s, kv_s, p_s, l_s, e_s, z_s, zn_s, sp_s, st0, st1, tmp_s,
            sem, osem):
    zero = []

    def spot(ref, row, col):
        n = 8 * (4 // ref.dtype.itemsize)
        ref = ref if len(ref.shape) == 2 else ref.at[zero[0]]
        return ref.at[_ds(row + zero[0] * n, n, n), _ds(col + zero[0] * 128, 128, 128)]

    def gate(ref, v):
        n = 8 * (4 // ref.dtype.itemsize)
        spot(ref, ref.shape[-2] - n, 0)[0:8, :] = v.astype(ref.dtype)

    def done(ref, row, col):
        v = spot(ref, row, col)[...]
        return v if v.dtype == u32 else pltpu.bitcast(v, u32)

    def tied(toks):
        def tie(b):
            if not toks:
                return b
            tok = functools.reduce(lambda p, q: p | q, toks)
            tok = jnp.concatenate([tok] * (b.shape[1] // 128), axis=1)
            always = lax.broadcasted_iota(jnp.int32, tok.shape, 0) >= zero[0]
            parts = []
            for r in range(0, b.shape[0], 64):
                parts += [b[r:r + 56], jnp.where(always, b[r + 56:r + 64], tok)]
            return jnp.concatenate(parts, axis=0)
        return tie

    def overlap(main, *sides):
        n, cyc, gen = main
        per = max(1, cyc // cfg["slot"])
        plan = [[] for _ in range(n * per)]
        for side in sides:
            if not isinstance(side, tuple):
                side = (side, 0, n)
            todo, first, last = side
            if todo and last == n:
                last -= (todo[-1][2] + cfg["tail"]) / cyc
            span = max(1, int((last - first) * per))
            total, spent = sum(t[3] for t in todo), 0
            for t in todo:
                plan[int(first * per) + spent * span // total].append(t)
                spent += t[3]
        next(gen)
        due = [[] for _ in range(n)]
        for i, todo in enumerate(plan):
            if i % per == 0:
                res = gen.send(tied([tok for _, tok in due[i // per]]))
            gated = []
            for _, refs, _, _ in todo:
                gated += [r for r in refs if not any(r is g for g in gated)]
            row = res.shape[0] * (i % per) // per
            for r in gated:
                gate(r, res[row:row + 8, 0:128])
            for fn, _, lat, _ in todo:
                where = fn()
                j = -(-(i * cyc // per + lat) // cyc)
                if where is not None and j < n:
                    due[j] = [d for d in due[j] if d[0] is not where[0]]
                    due[j].append((where[0], done(*where)))

    def tasks(fn, args, refs, lat, cost):
        return [(functools.partial(fn, *a), refs, cfg[lat], cost) for a in args]

    def run(todo):
        for t in todo:
            t[0]()

    def left_tasks(ref, key, k, load, refs, rows=None, cols=None, outer=None, rest=True):
        ks = _Split(k, cfg[key])
        h = U // ks.parts

        def put(n, r, c, v):
            ref[_ds(n * h // 2 + r // 2, 8, 8), c:c + 128] = _pack(v)

        def main(r, c, o):
            def get(i, j):
                if ks.level == 1:
                    return load(i * h + r, j, ks.start(j) + c)
                return _factor(LEFT[o], lambda a, b: load((2 * a + i) * h + r, 2 * b + j,
                                                          ks.start(2 * b + j) + c))
            for n, v in enumerate(_factors(LEFT, get)):
                put(7 * o + n, r, c, v)
            return ref, 7 * o * h // 2 + r // 2, c

        def other(r, i):
            vals = _factors(LEFT, lambda a, b: load((2 * a + i) * h + r, None, ks.rest_start(b)))
            for o, v in enumerate(vals):
                put(7 * o + 6 - i, r, ks.width, v)
            return ref, (6 - i) * h // 2 + r // 2, ks.width
        out = []
        for r in range(0, h, 16) if rows is None else rows:
            out += tasks(main, [(r, c, o)
                                for c in (range(0, ks.width, 128) if cols is None else cols)
                                for o in (range(7 ** (ks.level - 1)) if outer is None else outer)],
                         refs, "lat_short", 30)
            out += tasks(other, [(r, 0), (r, 1)] if ks.rest and rest else [], refs, "lat_short", 30)
        return out

    def right_tasks(bufs, key, n, rows, load, refs):
        main_p, rest_p = bufs
        ns = _Split(n, cfg[key])

        def main(prow, r, c, o):
            def get(i, j):
                if ns.level == 1:
                    return load(i, r, ns.start(j) + c)
                return _factor(RIGHT[o], lambda a, b: load(2 * a + i, r, ns.start(2 * b + j) + c))
            for m, v in enumerate(_factors(RIGHT, get)):
                main_p.at[7 * o + m][_ds(prow, 8, 8), c:c + 128] = _pack(v)
            return main_p, prow, c

        def rest(prow, r, o):
            top, bot = [_factor(RIGHT[o], lambda a, b: load(2 * a + i, r, ns.rest_start(b)))
                        for i in range(2)]
            for m, v in enumerate((top, bot, top - bot)):
                rest_p.at[3 * o + m][_ds(prow, 8, 8), :] = _pack(v)
            return rest_p, prow, 0
        out = []
        for prow, r in rows:
            out += tasks(main, [(prow, r, c, o) for c in range(0, ns.width, 128)
                                for o in range(7 ** (ns.level - 1))], refs, "lat_short", 32)
            out += tasks(rest, [(prow, r, o) for o in range(7)] if ns.rest else [], refs,
                         "lat_short", 16)
        return out

    def matmul(ref, bufs, key, k, n, store, cw=128, rest_first=False):
        main_p, rest_p = bufs
        ks, ns = _Split(k, cfg[key]), _Split(n, cfg[key])
        h = U // ks.parts

        def lhs(m, lo, hi):
            return _as_bf16(ref[m * h // 2:(m + 1) * h // 2, lo:hi])

        def dot(a, b):
            return jnp.dot(a, _as_bf16(b), preferred_element_type=f32)

        def temps(slot):
            return [tmp_s.at[(5 * slot + j) * h:(5 * slot + j + 1) * h, 0:cw] for j in range(5)]

        def gen1():
            tie = yield
            for c in range(0, ns.width, cw):
                feed = _combiner(temps(0), lambda i, j, v: store(i * h, ns.start(j) + c, v))
                for m in ORDER:
                    res = dot(lhs(m, 0, ks.width), tie(main_p.at[m][:, c:c + cw]))
                    feed(m, res)
                    tie = yield res

        def inner_temps():
            return [_Held() for _ in range(5)] if cfg["regs"] else temps(4)

        def chunk(c, tie):
            def put(i, j):
                return lambda a, b, v: store((2 * a + i) * h, ns.start(2 * b + j) + c, v)
            outer = {(i, j): _combiner(temps(2 * i + j), put(i, j))
                     for i in range(2) for j in range(2)}
            for o in ORDER:
                def extra(i, j, v):
                    if ks.rest and i != j:
                        v = v + dot(lhs(7 * o + 6 - i, ks.width, ks.width + 128),
                                    rest_p.at[2 * o + j][:, c:c + cw])
                    outer[i, j](o, v)
                feed = _combiner(inner_temps(), extra)
                for m in ORDER:
                    b = main_p.at[7 * o + m][:, c:c + cw]
                    hi = ks.width
                    if ks.rest and m >= 5:
                        b = jnp.concatenate([b, rest_p.at[2 * o + 6 - m][:, c:c + cw]], axis=0)
                        hi += 128
                    res = dot(lhs(7 * o + m, 0, hi), tie(b))
                    feed(m, res)
                    tie = yield res
            return tie

        def rest_chunk(tie):
            def put(i):
                return lambda a, b, v: store((2 * a + i) * h, ns.rest_start(b), v)
            outer = [_combiner(temps(i), put(i)) for i in range(2)]
            for o in ORDER:
                for i, (m0, b0), (m1, b1) in ((1, (3, 2), (1, 0)), (0, (2, 2), (4, 1))):
                    first = dot(lhs(7 * o + m0, 0, ks.width), tie(rest_p.at[3 * o + b0][...]))
                    tie = yield first
                    res = dot(lhs(7 * o + m1, 0, ks.width), tie(rest_p.at[3 * o + b1][...]))
                    outer[i](o, res - first if i else res + first)
                    tie = yield res
            return tie

        def gen2():
            tie = yield
            if ns.rest and rest_first:
                tie = yield from rest_chunk(tie)
            for c in range(0, ns.width, cw):
                tie = yield from chunk(c, tie)
            if ns.rest and not rest_first:
                tie = yield from rest_chunk(tie)
        cyc = h // 16 * 4 * (ks.width // 128) * (cw // 128)
        if ks.level == 1:
            return 7 * (ns.width // cw), cyc, gen1()
        return 49 * (ns.width // cw) + (28 if ns.rest else 0), cyc, gen2()

    def staged(i):
        return (z_s, zn_s)[i].at[0:D // 4, 0:D]

    def mix_staged(buf, shift):
        def task(r, t):
            def get(i, j):
                tile = j * NT // 2 + t
                v = pltpu.bitcast(staged(i)[r:r + 8, tile * 128:(tile + 1) * 128], u32)
                return _unpack(pltpu.roll(v, 128 - 4 * tile, 1) if shift and tile else v)
            for m, v in enumerate(_factors(RIGHT, get)):
                buf.at[m][r:r + 8, t * 128:(t + 1) * 128] = _pack(v)
            return buf, r, t * 128
        return tasks(task, [(r, t) for r in range(0, D // 4, 8) for t in range(NT // 2)],
                     [z_s, zn_s], "lat_xlu" if shift else "lat_short", 30)

    def prep_qkv(j, buf, rows=range(0, D // 2, 16)):
        def task(i, r):
            w = pltpu.bitcast(raw.at[j][i * D // 2 + r:i * D // 2 + r + 16, :], u32)
            lane = lax.broadcasted_iota(jnp.int32, (8, 128), 1)
            w = [w[:, t * 128:(t + 1) * 128] for t in range(NT)]
            w = [pltpu.roll(v, 4 * t, 1) if t else v for t, v in enumerate(w)]
            w = [w[(-t) % NT] for t in range(NT)]
            for b in range(3):
                m = (lane & (4 << b)) != 0
                w = [jnp.where(m, w[(t - (1 << b)) % NT], w[t]) for t in range(NT)]
            for t in range(NT):
                staged(i)[r // 2:r // 2 + 8, t * 128:(t + 1) * 128] = pltpu.bitcast(w[t], f32)
            return (z_s, zn_s)[i], r // 2, 0
        second = mix_staged(buf, True)
        return (tasks(task, [(i, r) for r in rows for i in range(2)], [raw], "lat_xlu", 45),
                [second[r // 16 * NT // 2 + t] for r in rows for t in range(NT // 2)])

    def prep_wo():
        def task(d4, t2, hh, c):
            src = [((t2 * 4 + j) * 4 + hh) * 32 + d4 * 16 for j in range(4)]
            v = _pair_transpose([pltpu.bitcast(raw.at[3][s:s + 16, c:c + 256], u32) for s in src])
            for j in range(4):
                r = ((j * 4 + hh) * 32 + t2 * 16) // 2
                staged(d4)[r:r + 8, c:c + 256] = pltpu.bitcast(v[j], f32)
            return (z_s, zn_s)[d4], r, c
        return tasks(task, [(d4, t2, hh, c) for d4 in range(2) for t2 in range(2)
                            for hh in range(4) for c in range(0, D, 256)],
                     [raw], "lat_short", 40) + mix_staged(wo_p, False)

    def prep_win(slab, bufs, first, count):
        ks = _Split(D, cfg["win"])

        def load(i, r, c):
            return raw.at[slab + c // (FH // 2)][
                _ds(ks.start(i) + r, 16, 16), c % (FH // 2):c % (FH // 2) + 128].astype(f32)
        rows = [((first + g) * 8, (first + g) * 16) for g in range(count)]
        return right_tasks(bufs, "win", FH, rows, load, [raw])

    def prep_wout(first, count):
        ks = _Split(FH, cfg["out"])

        def load(i, r, c):
            row = ks.start(i)
            return raw.at[2 + row // (FH // 2)][
                _ds(row % (FH // 2) + r, 16, 16), c:c + 128].astype(f32)
        rows = [((first + g) * 8, (first + g) * 16) for g in range(count)]
        return right_tasks((wout_p, None), "out", D, rows, load, [raw])

    def prep_wout_rest(first, count):
        ks, ns = _Split(FH, cfg["out"]), _Split(D, cfg["out"])

        def task(g, j, c):
            def get(a, b):
                col = ns.start(2 * b + j) + c
                return raw.at[2 + a][_ds(2 * ks.width + (first + g) * 16, 16, 16),
                                     col:col + 128].astype(f32)
            for o, v in enumerate(_factors(RIGHT, get)):
                wout_r.at[2 * o + j][_ds((first + g) * 8, 8, 8), c:c + 128] = _pack(v)
            return wout_r, (first + g) * 8, c
        if not ks.rest:
            return []
        return tasks(task, [(g, j, c) for g in range(count) for j in range(2)
                            for c in range(0, ns.width, 128)], [raw], "lat_short", 28)

    def prep_bias():
        def task(j):
            b = bsp_raw[...].astype(f32).reshape(1, S) * (1.0 / GAIN)
            bias_s[j * 128:(j + 1) * 128, :] = jnp.broadcast_to(
                b[:, j * 128:(j + 1) * 128], (128, 128)).T
            return bias_s, j * 128, 0
        return tasks(task, [(j,) for j in range(S // 128)], [], "lat_xlu", 50)

    def norm_tasks(base, src, st, eps=EPS, scale=None, rows=range(0, U, 16)):
        n = src.shape[1]

        def shift(r):
            v = src[_ds(r, 16, 16), 0:128].astype(f32)
            st.at[0][_ds(r, 16, 16), :] = jnp.broadcast_to(v[:, 0:1], (16, 128))
            return st, r, 0

        def stats(r):
            sh = st.at[0][_ds(r, 8, 8), :]
            s1 = s2 = None
            for c in range(0, n, 256):
                v = src[_ds(r, 8, 8), c:c + 256].astype(f32)
                for d in (v[:, :128] - sh, v[:, 128:] - sh):
                    s1 = d if s1 is None else s1 + d
                    s2 = d * d if s2 is None else s2 + d * d
            m = jnp.sum(s1, axis=-1, keepdims=True) * (1.0 / n)
            var = jnp.sum(s2, axis=-1, keepdims=True) * (1.0 / n) - m * m
            st.at[1][_ds(r, 8, 8), :] = sh + m
            st.at[2][_ds(r, 8, 8), :] = jnp.broadcast_to(jnp.maximum(var, 0.0) + eps, (8, 128))
            return st, r, 0

        def rstd(r):
            v = lax.rsqrt(st.at[2][_ds(r, 16, 16), :])
            st.at[0][_ds(r, 16, 16), :] = v if scale is None else v * scale
            return st, r, 0

        def load(r, c, h=16, w=128):
            v = src[_ds(r, h, h), c:c + w].astype(f32)
            mean, inv = [jnp.concatenate([st.at[j][_ds(r, h, h), :]] * (w // 128), axis=1)
                         for j in (1, 0)]
            return (v - mean) * inv

        def write(dst):
            def task(r, c, w):
                dst[_ds(r, 8, 8), c:c + w] = load(r, c, 8, w)
                return dst, r, c
            return tasks(task, [(r + j, c, min(1024, n - c)) for r in rows for j in (0, 8)
                                for c in range(0, n, 1024)], [base], "lat_short", 22)
        out = tasks(shift, [(r,) for r in rows], [base], "lat_xlu", 10)
        out += tasks(stats, [(r + j,) for r in rows for j in (0, 8)], [base], "lat_xlu",
                     n // 28 + 8)
        out += tasks(rstd, [(r,) for r in rows], [st], "lat_short", 22)
        return out, load, write

    def norm_x(u, buf):
        out, load, _ = norm_tasks(x_s, unit(x_s, u), st0)
        return out + left_tasks(buf, "qkv", D, lambda r, j, c: load(r, c), [x_s])

    def norm_h(u, spare, **kw):
        out, _, write = norm_tasks(x_s, unit(x_s, u), st1, scale=ALPHA, **kw)
        return out + write(spare)

    def left_h(spare, **kw):
        return left_tasks(ha, "win", D, lambda r, j, c: spare[_ds(r, 16, 16), c:c + 128], [spare],
                          **kw)

    def take(v, idx):
        return jnp.take_along_axis(v, idx, axis=1)

    def logit_tasks(first, q_s=q_s, k_s=k_s):
        def task(r, b):
            lane = lax.broadcasted_iota(jnp.int32, (8, 128), 1)
            acc = [None] * 4
            for t in range(NT):
                q = q_s[r:r + 8, t * 128:(t + 1) * 128]
                for j in range(4):
                    k0 = HALO + r - DIL * (4 * b + j)
                    term = q * k_s[t, k0:k0 + 8, :]
                    acc[j] = term if t == 0 else acc[j] + term
            for bit in (1, 2):
                odd = (lane & bit) != 0
                acc = [jnp.where(odd, acc[j ^ bit], acc[j]) for j in range(4)]
            lg = acc[0]
            for j in range(1, 4):
                lg = lg + take(acc[j], lane ^ j)
            lg = lg * float(DH) ** -0.5
            if first and r < DIL * WIN:
                pos = r + lax.broadcasted_iota(jnp.int32, (8, 128), 0)
                lg = jnp.where(pos >= DIL * (4 * b + (lane & 3)), lg, -1e9)
            l_s[b, r:r + 8, :] = lg
            return l_s, r, 0
        return tasks(task, [(r, b) for r in range(0, U, 8) for b in range(2)], [q_s, k_s],
                     "lat_xlu", 75)

    def softmax_tasks():
        def exps(r):
            lane = lax.broadcasted_iota(jnp.int32, (16, 128), 1)
            lg = [l_s[b, r:r + 16, :] for b in range(2)]
            mx = jnp.maximum(lg[0], lg[1])
            mx = functools.reduce(jnp.maximum, [mx] + [take(mx, lane ^ j) for j in range(1, 4)])
            for b in range(2):
                e_s[b, r:r + 16, :] = jnp.exp(lg[b] - mx)
            return e_s, r, 0

        def probs(r):
            lane = lax.broadcasted_iota(jnp.int32, (8, 128), 1)
            e = [e_s[b, r:r + 8, :] for b in range(2)]
            e = {4 * b + j: take(e[b], (lane & -4) | j) for j in range(4) for b in range(2)}
            inv = 1.0 / functools.reduce(lambda p, q: p + q, e.values())
            for w in range(WIN):
                p_s[w, r:r + 8, :] = e[w] * inv
            return p_s, r, 0
        return (tasks(exps, [(r,) for r in range(0, U, 16)], [l_s], "lat_xlu", 40)
                + tasks(probs, [(r,) for r in range(0, U, 8)], [e_s], "lat_xlu", 40))

    def value_tasks(v_s=v_s):
        def task(r, t0):
            acc = [None] * 4
            for w in range(WIN):
                k0 = HALO + r - DIL * w
                p = p_s[w, r:r + 8, :]
                for j in range(4):
                    term = p * v_s[t0 + j, k0:k0 + 8, :]
                    acc[j] = term if w == 0 else acc[j] + term
            for j in range(4):
                o_s[r:r + 8, (t0 + j) * 128:(t0 + j + 1) * 128] = acc[j]
            return o_s, r, t0 * 128
        out = []
        for g in range(0, U // 2 + 16, 16):
            if g < U // 2:
                out += tasks(task, [(g + b + j, t0) for b in (0, U // 2) for j in (0, 8)
                                    for t0 in (0, 4)], [p_s, v_s], "lat_short", 62)
            if g:
                out += left_tasks(oa, "wo", D, lambda r, j, c: o_s[r:r + 16, c:c + 128], [o_s],
                                  rows=[g - 16])
        return out

    def set_halo(buf, src):
        buf[:, 0:HALO, :] = (jnp.zeros((NT, HALO, 128), f32) if src is None
                             else src[:, U:U + HALO, :])

    def copies(name):
        half = FH // 2
        early = share(0, NU - 2, _Split(D, cfg["win"]).width // 16)[1] * 16
        part = D // 2 // cfg["wq_parts"]

        def win_rows(lo, hi):
            return [(win_hbm.at[r + lo:r + hi, j * half:(j + 1) * half],
                     raw.at[4 + j, r + lo:r + hi, 0:half])
                    for r in range(0, D, D // 4) for j in range(4)]

        def units(lo, hi):
            return [(x_hbm.at[0, lo * U:hi * U], x_s.at[lo * U:hi * U])]
        pairs = dict(
            x0=units(0, 1),
            x1=units(1, 2),
            wk=[(wqkv_hbm.at[:, D:2 * D], raw.at[1, 0:D])],
            wv=[(wqkv_hbm.at[:, 2 * D:3 * D], raw.at[2, 0:D])],
            wo=[(wo_hbm, raw.at[3, 0:D])] + units(2, 3),
            rest0=units(3, 4) + win_rows(0, early),
            rest1=units(4, 5) + win_rows(early, 2 * early),
            rest1b=units(5, NU) + win_rows(2 * early, D // 4),
            rest2=[(wsp_hbm.at[0:D, j * D:(j + 1) * D], raw.at[j, 0:D]) for j in range(2)]
            + [(wout_hbm.at[j * half:(j + 1) * half], raw.at[2 + j, 0:half]) for j in range(2)]
            + [(bsp_hbm, bsp_raw)],
            rest3=[(wsp_hbm.at[D:S, j * D:(j + 1) * D], raw.at[4 + j, 0:D]) for j in range(2)],
        )
        for j in range(cfg["wq_parts"]):
            pairs["wq%d" % j] = [(wqkv_hbm.at[r:r + part, 0:D], raw.at[0, r:r + part])
                                 for r in (j * part, D // 2 + j * part)]
        j = list(pairs).index(name)
        return [pltpu.make_async_copy(a, b, sem.at[j]) for a, b in pairs[name]]

    def start(name):
        for c in copies(name):
            c.start()

    def wait(name):
        for c in copies(name):
            c.wait()

    def out_copy(u, half):
        rows = _ds(u * U + half * U // 2, U // 2, U // 2)
        return pltpu.make_async_copy(x_s.at[rows], out_hbm.at[0, rows], osem.at[2 * u + half])

    def unit(ref, u, n=U):
        return ref.at[_ds(u * n, n, n)]

    def clip(v, lo, hi):
        return min(max(v, lo), hi) if isinstance(v, int) else jnp.clip(v, lo, hi)

    def share(step, steps, total):
        count = -(-total // steps)
        return clip(step * count, 0, total - count), count

    def add_into(u):
        def store(r, c, v):
            idx = (slice(r, r + v.shape[0]), slice(c, c + v.shape[1]))
            dst = unit(x_s, u)
            dst[idx] = (dst[idx].astype(f32) + v).astype(bf16)
        return store

    def put_rows(buf):
        def store(r, c, v):
            buf[r:r + v.shape[0], c:c + 128] = v
        return store

    def put_slab(buf):
        def store(r, c, v):
            buf[c // 128, HALO + r:HALO + r + v.shape[0], :] = v
        return store

    def qkv(src, w, store):
        return matmul(src, (w, None), "qkv", D, D, store)

    def project(u):
        return matmul(oa, (wo_p, None), "wo", D, D, add_into(u), cfg["cw_wo"])

    def first_attention():
        set_halo(kv_s, None)
        wait("x1")
        overlap(qkv(xb, wq_p, put_rows(o_s)), norm_x(1, xa))
        start("wv")
        wait("wk")
        overlap(qkv(xa, wq_p, put_rows(q_s)), sum(prep_qkv(1, wk_p), []))
        start("wo")
        wait("wv")
        prep, logits, soft = sum(prep_qkv(2, wv_p), []), logit_tasks(False), softmax_tasks()
        overlap(qkv(xb, wk_p, put_slab(kv_s)), prep)
        set_halo(k_s, kv_s)
        overlap(qkv(xa, wk_p, put_slab(k_s)), logit_tasks(True, o_s, kv_s))
        start("rest0")
        wait("wo")
        prep = prep_wo()
        overlap(qkv(xb, wv_p, put_slab(kv_s)), soft, prep)
        set_halo(v_s, kv_s)
        overlap(qkv(xa, wv_p, put_slab(v_s)), value_tasks(kv_s), logits[:24])
        overlap(project(0), (logits[24:], 0, 22), norm_x(2, xa))

    def step_attention(u):
        if cfg["part"] != "s1":
            @pl.when(u == 3)
            def _():
                wait("rest1")
                start("rest1b")

            @pl.when(u == 4)
            def _():
                wait("rest1b")
                start("rest2")
        begin, count = share(u - 2, NU - 2, _Split(D, cfg["win"]).width // 16)
        prep = (prep_win(6, (wz2_p, wz2_r), begin, count)
                + prep_win(4, (wz1_p, wz1_r), begin, count))
        cut = len(prep) * cfg["cut_prep"] // 8
        g = clip(u - 2, 0, U // 64 - 1) * 16
        head = norm_h(0, z_s, rows=[g + b for b in range(0, U, 64)]) + left_h(z_s, rows=[g])
        logits = logit_tasks(False)
        set_halo(k_s, k_s)
        overlap(qkv(xa, wq_p, put_rows(q_s)), softmax_tasks(), prep[:cut])
        overlap(qkv(xa, wk_p, put_slab(k_s)), value_tasks())
        set_halo(v_s, v_s)
        overlap(qkv(xa, wv_p, put_slab(v_s)), logits, head)
        overlap(project(u - 1), norm_x(clip(u + 1, 0, NU - 1), xa), prep[cut:])

    def spatial_left(u, rows=range(0, U // 4, 16)):
        per = D // U

        def regroup(r, m):
            lane = lax.broadcasted_iota(jnp.int32, (8, 128), 1)
            col = 2 * U * m
            w = pltpu.bitcast(raw.at[u // per * 4 + col // D][
                _ds(u % per * U + r, 16, 16), col % D:col % D + 2 * U], u32)
            for a in range(2):
                one, two = w[:, a * 128:(a + 1) * 128], w[:, U + a * 128:U + (a + 1) * 128]
                mid = pltpu.roll(jnp.where(lane < 64, two, one), 64, 1)
                for j, v in ((2 * a, jnp.where(lane < 64, one, mid)),
                             (2 * a + 1, jnp.where(lane < 64, mid, two))):
                    sp_s[_ds(r // 2, 8, 8), j * 512 + m * 128:j * 512 + (m + 1) * 128] = v
            return sp_s, r // 2, m * 128
        return tasks(regroup, [(b + r, m) for r in rows for b in range(0, U, U // 4)
                               for m in range(NU // 2)], [raw], "lat_xlu", 18) + left_tasks(
            sa, "sp", S, lambda r, j, c: _unpack(sp_s[_ds(r // 2, 8, 8), c:c + 128]), [sp_s],
            rows=rows)

    def gate_input():
        def store(r, c, v):
            z_s[r:r + v.shape[0], c:c + 128] = _gelu(v)
        return matmul(ha, (wz2_p, wz2_r), "win", D, FH, store)

    def value_input(u, more):
        z1t = unit(z1_s, u, U // 2)
        h = U // 4

        def store(r, c, v):
            z1t[r // 2:(r + v.shape[0]) // 2, c:c + 128] = _pack(_gelu(v))
        stats, _, write = norm_tasks(z_s, z_s, st0, EPS * GAIN * GAIN, 1.0 / GAIN)
        factors = right_tasks((z2n_p, z2n_r), "sp", FH,
                              [(u * (h // 2) + r // 2, r) for r in range(0, h, 16)],
                              lambda b, r, c: zn_s[b * h + r:b * h + r + 16, c:c + 128], [zn_s])
        main = matmul(ha, (wz1_p, wz1_r), "win", D, FH, store, rest_first=True)
        last = main[0] - 49
        if more:
            overlap(main, (stats + write(zn_s) + factors, 0, last + cfg["z_over"]),
                    *[(left_h(q_s, outer=[o]), last + 7 * j + 6, last + 7 * j + 13)
                      for j, o in enumerate(ORDER[:cfg["z_left"]])])
        else:
            overlap(main, stats + write(zn_s) + factors)

    def last_attention():
        main = gate_input()
        overlap(main, (softmax_tasks(), 0, cfg["soft_end"]),
                (value_tasks(), cfg["soft_end"], main[0]))
        overlap(project(NU - 1), prep_bias() + norm_h(1, q_s))

    def step_input(u):
        value_input(u - 1, True)
        prep = (spatial_left(0, [share(u - 1, NU - 1, U // 64)[0] * 16])
                + prep_wout(*share(u - 1, NU - 1, _Split(FH, cfg["out"]).width // 16))
                + prep_wout_rest(*share(u - 1, NU - 1, 8)))
        late = ORDER[cfg["z_left"]:]
        main = gate_input()
        overlap(main, (left_h(q_s, outer=late[:1]) + left_h(q_s, outer=late[1:]), 0, 7 * len(late)),
                (norm_h(clip(u + 1, 0, NU - 1), q_s), 7 * len(late), main[0]),
                (prep, 7 * len(late), main[0]))

    def step_output(u):
        bt, z1t = unit(bias_s, u), unit(z1_s, u, U // 2)

        def put_y(r, c, g):
            n = g.shape[0]
            z_s[r:r + n, c:c + 128] = _unpack(z1t[r // 2:(r + n) // 2, c:c + 128]) * (
                g + bt[r:r + n, :])

        def gated(**kw):
            return left_tasks(ya, "out", FH, lambda r, j, c: z_s[r:r + 16, c:c + 128], [z_s], **kw)
        overlap(matmul(sa, (z2n_p, z2n_r), "sp", S, FH, put_y),
                *[(gated(cols=[128 * j], rest=False), 49 * j + 49, 49 * j + 49 + 20)
                  for j in range(3)])
        run(gated(cols=[]))
        overlap(matmul(ya, (wout_p, wout_r), "out", FH, D, add_into(u), 256),
                spatial_left(clip(u + 1, 0, NU - 1)),
                ([(out_copy(u, 1).start, [], 0, 1)], 36, 37))
        out_copy(u, 0).start()

    def make_zero():
        bits = pltpu.bitcast(x_s[0:16, 0:128], jnp.int32)
        zero.append(bits[0, 0] ^ pltpu.roll(bits, 1, 1)[0, 1])

    def keep(j):
        v = None
        for b in (wq_p, wk_p, wv_p, wo_p, wz1_p, wz1_r, wz2_p, wz2_r, wout_p, wout_r, z2n_p,
                  z2n_r, z1_s, bias_s, xa, xb, oa, ha, sa, ya, q_s, o_s, k_s, v_s, kv_s, p_s, l_s, e_s,
                  z_s, zn_s, sp_s, st0, st1, tmp_s):
            v = done(b, 0, 0) if v is None else v | done(b, 0, 0)
        x_s[0:16, 0:128] = _as_bf16(v)
        c = pltpu.make_async_copy(x_s.at[0:16, 0:128], out_hbm.at[0, 0:16, 0:128], sem.at[0])
        c.start()
        c.wait()

    if cfg["part"] in ("s1", "s2", "s3", "mid"):
        make_zero()
        if cfg["part"] == "mid":
            last_attention()
            value_input(NU - 1, False)
        else:
            pl.loop(1, NU)({"s1": step_attention, "s2": step_input, "s3": step_output}[cfg["part"]])
        if cfg["part"] == "s3":
            for u in range(1, NU):
                out_copy(u, 0).wait()
                out_copy(u, 1).wait()
        pl.loop(0, 2)(keep)
        return
    import contextlib
    scope = jax.named_scope if cfg["prof"] else (lambda n: contextlib.nullcontext())
    parts = cfg["wq_parts"]
    queue = ["wq%d" % j for j in range(1, parts)] + ["x1", "wk"]
    with scope("p_x0"):
        start("x0")
        start("wq0")
        wait("x0")
    with scope("p_norm"):
        make_zero()
        start(queue[0])
        wait("wq0")
        run(norm_x(0, xb))
    for j in range(parts):
        with scope("p_wq"):
            start(queue[j + 1])
            if j:
                wait("wq%d" % j)
        with scope("p_prepq"):
            run(sum(prep_qkv(0, wq_p, range(j * D // 2 // parts, (j + 1) * D // 2 // parts, 16)), []))
    with scope("p_first"):
        first_attention()
    with scope("p_rest0"):
        wait("rest0")
    if cfg["part"] == "first":
        pl.loop(0, 2)(keep)
        return
    start("rest1")

    def sc(name, fn):
        def g(u):
            with scope(name):
                fn(u)
        return g
    with scope("p_loop1"):
        pl.loop(2, NU)(sc("p_it1", step_attention))
    start("rest3")
    with scope("p_rest2"):
        wait("rest2")
    with scope("p_mid"):
        last_attention()
    with scope("p_loop2"):
        pl.loop(1, NU)(sc("p_it2", step_input))
    with scope("p_mid2"):
        value_input(NU - 1, False)
    wait("rest3")
    with scope("p_loop3"):
        pl.loop(0, NU)(sc("p_it3", step_output))
    with scope("p_out"):
        for u in range(NU):
            out_copy(u, 0).wait()
            out_copy(u, 1).wait()


def build(cfg, interpret=False, name="fused_block"):
    vm = pltpu.VMEM

    def right(key, k, n):
        ks, ns = _Split(k, cfg[key]), _Split(n, cfg[key])
        main = vm((7 ** ks.level, ks.width // 2, ns.width), u32)
        if ns.rest:
            return [main, vm((21, ks.width // 2, 128), u32)]
        if ks.rest:
            return [main, vm((14, 64, ns.width), u32)]
        return [main]

    def left(key, k):
        ks = _Split(k, cfg[key])
        return vm((7 ** ks.level * U // ks.parts // 2, ks.width + ks.rest), u32)
    scratch = [
        vm((S + 16, D), bf16),
        vm((8, D + 16, D), bf16),
        vm((S,), bf16),
        *right("qkv", D, D) * 3, *right("wo", D, D),
        *right("win", D, FH), *right("win", D, FH), *right("out", FH, D), *right("sp", S, FH),
        vm((S // 2, FH), u32),
        vm((S, 128), f32),
        left("qkv", D), left("qkv", D), left("wo", D), left("win", D), left("sp", S),
        left("out", FH),
        *[vm((U + 8, D), f32)] * 2,
        *[vm((NT, HALO + U + 8, 128), f32)] * 3,
        vm((WIN, U + 8, 128), f32),
        *[vm((2, U + 8, 128), f32)] * 2,
        *[vm((U + 8, FH), f32)] * 2,
        vm((U // 2 + 8, S), u32),
        *[vm((3, U + 8, 128), f32)] * 2,
        vm((25 * U // 4, 256), f32),
        pltpu.SemaphoreType.DMA((10 + cfg["wq_parts"],)),
        pltpu.SemaphoreType.DMA((2 * NU,)),
    ]
    hbm = pl.BlockSpec(memory_space=pl.ANY)
    return pl.pallas_call(
        functools.partial(_kernel, cfg),
        out_shape=jax.ShapeDtypeStruct((1, S, D), bf16),
        in_specs=[hbm] * 7,
        out_specs=hbm,
        scratch_shapes=scratch,
        compiler_params=pltpu.CompilerParams(vmem_limit_bytes=127 * 1024 * 1024,
                                             flags=cfg["flags"]),
        interpret=interpret,
        name=name,
    )


@jax.jit
def pallas_sequential_preLN__sliding_local_dilated__mixer_gmlp__prompt_kernel(
    A_x: jax.Array,
    A_wqkv: jax.Array,
    A_wo: jax.Array,
    B_x: jax.Array,
    B_w_in: jax.Array,
    B_w_sp: jax.Array,
    B_b_sp: jax.Array,
    B_w_out: jax.Array,
):
    del B_x
    return build(CFG)(A_x, A_wqkv, A_wo, B_w_in, B_w_sp, B_b_sp, B_w_out)
```

```python
import functools

import jax
import jax.numpy as jnp
import numpy as np
from jax import lax
from jax.experimental import pallas as pl
from jax.experimental.pallas import tpu as pltpu

S = 2048
D = 1024
FH = 1792
DH = 32
WIN = 8
DIL = 2
HALO = 16
U = 256
NU = S // U
NT = D // 128
PARTS = 4
EPS = 1e-5

f32 = jnp.float32
bf16 = jnp.bfloat16
u32 = jnp.uint32

CFG = dict(part="all", flags=None, qkv=1, wo=1, win=2, sp=2, out=2, slot=32,
           lat_short=320, lat_xlu=512, tail=0, regs=False, cw_wo=128, cut_prep=6, z_over=35, z_left=5, f_log=24, f_end=26, gap=100, lag_rstd=6, lag_probs=2, peel=True, wq_parts=4, depth=6, soft_end=84, prof=False)

ORDER = (0, 3, 1, 2, 5, 4, 6)
REST = (3, 1, 2, 4)


def _pack(v):
    return pltpu.bitcast(v.astype(bf16), u32)


def _as_bf16(v):
    return pltpu.bitcast(v, bf16)


def _unpack(v):
    return pltpu.bitcast(v, bf16).astype(f32)


_C = float(np.sqrt(2.0 / np.pi))
ALPHA = float((_C * 0.044715) ** (1.0 / 3.0))
GAIN = 2.0 * ALPHA


def _gelu(v):
    return v * (1.0 + jnp.tanh(v * (_C / ALPHA + v * v)))


LEFT = (((1, 0, 0), (1, 1, 1)), ((1, 1, 0), (1, 1, 1)), ((1, 0, 0),), ((1, 1, 1),),
        ((1, 0, 0), (1, 0, 1)), ((1, 1, 0), (-1, 0, 0)), ((1, 0, 1), (-1, 1, 1)))
RIGHT = (((1, 0, 0), (1, 1, 1)), ((1, 0, 0),), ((1, 0, 1), (-1, 1, 1)), ((1, 1, 0), (-1, 0, 0)),
         ((1, 1, 1),), ((1, 0, 0), (1, 0, 1)), ((1, 1, 0), (1, 1, 1)))


def _factor(terms, get):
    v = get(*terms[0][1:])
    for sign, i, j in terms[1:]:
        v = v + get(i, j) if sign > 0 else v - get(i, j)
    return v


def _factors(forms, get):
    blk = {(i, j): get(i, j) for i in range(2) for j in range(2)}
    return [_factor(terms, lambda i, j: blk[i, j]) for terms in forms]


class _Held:
    def __setitem__(self, _, v):
        self.v = v

    def __getitem__(self, _):
        return self.v


def _combiner(tmp, put):
    t1, t2, t3, t4, t5 = tmp

    def feed(i, m):
        if i == 0:
            t1[...] = m
        elif i == 3:
            t4[...] = m
        elif i == 1:
            t2[...] = m
            put(1, 0, m + t4[...])
        elif i == 2:
            t3[...] = m
        elif i == 5:
            put(1, 1, (t1[...] - t2[...] + t3[...]) + m)
        elif i == 4:
            t5[...] = m
            put(0, 1, m + t3[...])
        else:
            put(0, 0, (t1[...] + t4[...] - t5[...]) + m)
    return feed


class _Split:
    def __init__(self, n, level):
        self.level, self.parts = level, 1 << level
        self.width = n // self.parts // 128 * 128
        self.rest = n // 2 - 2 * self.width if level == 2 else 0
        self.half = n // 2

    def start(self, j):
        if self.level == 1:
            return j * self.half
        return (j // 2) * self.half + (j % 2) * self.width

    def rest_start(self, h):
        return h * self.half + 2 * self.width


def _pair_transpose(v):
    sub = lax.broadcasted_iota(jnp.int32, v[0].shape, 0)
    v = list(v)
    for b in range(2):
        s = 1 << b
        m = (sub & (2 * s)) != 0
        nv = list(v)
        for j in range(4):
            if j & s:
                continue
            lo, hi = v[j], v[j + s]
            nv[j] = jnp.where(m, pltpu.roll(hi, 2 * s, 0), lo)
            nv[j + s] = jnp.where(m, hi, pltpu.roll(lo, 8 - 2 * s, 0))
        v = nv
    return v


def _ds(start, size, align):
    return pl.ds(start if isinstance(start, int) else pl.multiple_of(start, align), size)


def _kernel(cfg,
            x_hbm, wqkv_hbm, wo_hbm, win_hbm, wsp_hbm, bsp_hbm, wout_hbm, out_hbm,
            x_s, raw, bsp_raw,
            wq_p, wk_p, wv_p, wo_p, wz1_p, wz1_r, wz2_p, wz2_r, wout_p, wout_r, z2n_p, z2n_r,
            z1_s, bias_s, xa, xb, oa, ha, sa, ya,
            q_s, o_s, k_s, v_s, kv_s, p_s, l_s, e_s, z_s, zn_s, sp_s, st0_s, st1_s, inv0_s, inv1_s, tmp_s,
            sem, osem):
    st0, st1 = (st0_s, inv0_s), (st1_s, inv1_s)
    zero = []

    def spot(ref, row, col):
        n = 8 * (4 // ref.dtype.itemsize)
        ref = ref if len(ref.shape) == 2 else ref.at[zero[0]]
        return ref.at[_ds(row + zero[0] * n, n, n), _ds(col + zero[0] * 128, 128, 128)]

    def gate(ref, v):
        n = 8 * (4 // ref.dtype.itemsize)
        spot(ref, ref.shape[-2] - n, 0)[0:8, :] = v.astype(ref.dtype)

    def done(ref, row, col):
        v = spot(ref, row, col)[...]
        return v if v.dtype == u32 else pltpu.bitcast(v, u32)

    def tied(toks):
        def tie(b):
            if not toks:
                return b
            tok = functools.reduce(lambda p, q: p | q, toks)
            tok = jnp.concatenate([tok] * (b.shape[1] // 128), axis=1)
            always = lax.broadcasted_iota(jnp.int32, tok.shape, 0) >= zero[0]
            parts = []
            for r in range(0, b.shape[0], 64):
                parts += [b[r:r + 56], jnp.where(always, b[r + 56:r + 64], tok)]
            return jnp.concatenate(parts, axis=0)
        return tie

    def overlap(main, *sides):
        n, cyc, gen = main
        per = max(1, cyc // cfg["slot"])
        plan = [[] for _ in range(n * per)]
        for side in sides:
            if not isinstance(side, tuple):
                side = (side, 0, n)
            todo, first, last = side
            if todo and last == n:
                last -= (todo[-1][2] + cfg["tail"]) / cyc
            span = max(1, int((last - first) * per))
            total, spent = sum(t[3] for t in todo), 0
            for t in todo:
                plan[int(first * per) + spent * span // total].append(t)
                spent += t[3]
        next(gen)
        due = [[] for _ in range(n)]
        for i, todo in enumerate(plan):
            if i % per == 0:
                res = gen.send(tied([tok for _, tok in due[i // per]]))
            gated = []
            for _, refs, _, _ in todo:
                gated += [r for r in refs if not any(r is g for g in gated)]
            row = res.shape[0] * (i % per) // per
            for r in gated:
                gate(r, res[row:row + 8, 0:128])
            for fn, _, lat, _ in todo:
                where = fn()
                j = -(-(i * cyc // per + lat) // cyc)
                if where is not None and j < n:
                    due[j] = [d for d in due[j] if d[0] is not where[0]]
                    due[j].append((where[0], done(*where)))

    def tasks(fn, args, refs, lat, cost):
        return [(functools.partial(fn, *a), refs, cfg[lat], cost) for a in args]

    def staggered(early, late, lag):
        per = len(early) / len(late)
        order = [(j, t) for j, t in enumerate(early)]
        order += [((j + 1) * per + lag - 0.5, t) for j, t in enumerate(late)]
        return [t for _, t in sorted(order, key=lambda p: p[0])]

    gap = [(lambda: None, [], 0, cfg["gap"])]

    def run(todo):
        for t in todo:
            t[0]()

    def left_tasks(ref, key, k, load, refs, rows=None, cols=None, outer=None, rest=True):
        ks = _Split(k, cfg[key])
        h = U // ks.parts

        def put(n, r, c, v):
            ref[_ds(n * h // 2 + r // 2, 8, 8), c:c + 128] = _pack(v)

        def main(r, c, o):
            def get(i, j):
                if ks.level == 1:
                    return load(i * h + r, j, ks.start(j) + c)
                return _factor(LEFT[o], lambda a, b: load((2 * a + i) * h + r, 2 * b + j,
                                                          ks.start(2 * b + j) + c))
            for n, v in enumerate(_factors(LEFT, get)):
                put(7 * o + n, r, c, v)
            return ref, 7 * o * h // 2 + r // 2, c

        def other(r, i):
            vals = _factors(LEFT, lambda a, b: load((2 * a + i) * h + r, None, ks.rest_start(b)))
            for o, v in enumerate(vals):
                put(7 * o + 6 - i, r, ks.width, v)
            return ref, (6 - i) * h // 2 + r // 2, ks.width
        out = []
        for r in range(0, h, 16) if rows is None else rows:
            out += tasks(main, [(r, c, o)
                                for c in (range(0, ks.width, 128) if cols is None else cols)
                                for o in (range(7 ** (ks.level - 1)) if outer is None else outer)],
                         refs, "lat_short", 30)
            out += tasks(other, [(r, 0), (r, 1)] if ks.rest and rest else [], refs, "lat_short", 30)
        return out

    def right_tasks(bufs, key, n, rows, load, refs):
        main_p, rest_p = bufs
        ns = _Split(n, cfg[key])

        def main(prow, r, c, o):
            def get(i, j):
                if ns.level == 1:
                    return load(i, r, ns.start(j) + c)
                return _factor(RIGHT[o], lambda a, b: load(2 * a + i, r, ns.start(2 * b + j) + c))
            for m, v in enumerate(_factors(RIGHT, get)):
                main_p.at[7 * o + m][_ds(prow, 8, 8), c:c + 128] = _pack(v)
            return main_p, prow, c

        def rest(prow, r, o):
            top, bot = [_factor(RIGHT[o], lambda a, b: load(2 * a + i, r, ns.rest_start(b)))
                        for i in range(2)]
            for m, v in enumerate((top, bot, top - bot)):
                rest_p.at[3 * o + m][_ds(prow, 8, 8), :] = _pack(v)
            return rest_p, prow, 0
        out = []
        for prow, r in rows:
            out += tasks(main, [(prow, r, c, o) for c in range(0, ns.width, 128)
                                for o in range(7 ** (ns.level - 1))], refs, "lat_short", 32)
            out += tasks(rest, [(prow, r, o) for o in range(7)] if ns.rest else [], refs,
                         "lat_short", 16)
        return out

    def matmul(ref, bufs, key, k, n, store, cw=128, rest_first=False):
        main_p, rest_p = bufs
        ks, ns = _Split(k, cfg[key]), _Split(n, cfg[key])
        h = U // ks.parts

        def lhs(m, lo, hi):
            return _as_bf16(ref[m * h // 2:(m + 1) * h // 2, lo:hi])

        def dot(a, b):
            return jnp.dot(a, _as_bf16(b), preferred_element_type=f32)

        def temps(slot):
            return [tmp_s.at[(5 * slot + j) * h:(5 * slot + j + 1) * h, 0:cw] for j in range(5)]

        def gen1():
            tie = yield
            for c in range(0, ns.width, cw):
                feed = _combiner(temps(0), lambda i, j, v: store(i * h, ns.start(j) + c, v))
                for m in ORDER:
                    res = dot(lhs(m, 0, ks.width), tie(main_p.at[m][:, c:c + cw]))
                    feed(m, res)
                    tie = yield res

        def inner_temps():
            return [_Held() for _ in range(5)] if cfg["regs"] else temps(4)

        def chunk(c, tie):
            def put(i, j):
                return lambda a, b, v: store((2 * a + i) * h, ns.start(2 * b + j) + c, v)
            outer = {(i, j): _combiner(temps(2 * i + j), put(i, j))
                     for i in range(2) for j in range(2)}
            for o in ORDER:
                def extra(i, j, v):
                    if ks.rest and i != j:
                        v = v + dot(lhs(7 * o + 6 - i, ks.width, ks.width + 128),
                                    rest_p.at[2 * o + j][:, c:c + cw])
                    outer[i, j](o, v)
                feed = _combiner(inner_temps(), extra)
                for m in ORDER:
                    b = main_p.at[7 * o + m][:, c:c + cw]
                    hi = ks.width
                    if ks.rest and m >= 5:
                        b = jnp.concatenate([b, rest_p.at[2 * o + 6 - m][:, c:c + cw]], axis=0)
                        hi += 128
                    res = dot(lhs(7 * o + m, 0, hi), tie(b))
                    feed(m, res)
                    tie = yield res
            return tie

        def rest_chunk(tie):
            def put(i):
                return lambda a, b, v: store((2 * a + i) * h, ns.rest_start(b), v)
            outer = [_combiner(temps(i), put(i)) for i in range(2)]
            for o in ORDER:
                for i, (m0, b0), (m1, b1) in ((1, (3, 2), (1, 0)), (0, (2, 2), (4, 1))):
                    first = dot(lhs(7 * o + m0, 0, ks.width), tie(rest_p.at[3 * o + b0][...]))
                    tie = yield first
                    res = dot(lhs(7 * o + m1, 0, ks.width), tie(rest_p.at[3 * o + b1][...]))
                    outer[i](o, res - first if i else res + first)
                    tie = yield res
            return tie

        def gen2():
            tie = yield
            if ns.rest and rest_first:
                tie = yield from rest_chunk(tie)
            for c in range(0, ns.width, cw):
                tie = yield from chunk(c, tie)
            if ns.rest and not rest_first:
                tie = yield from rest_chunk(tie)
        cyc = h // 16 * 4 * (ks.width // 128) * (cw // 128)
        if ks.level == 1:
            return 7 * (ns.width // cw), cyc, gen1()
        return 49 * (ns.width // cw) + (28 if ns.rest else 0), cyc, gen2()

    def staged(i):
        return (z_s, zn_s)[i].at[0:D // 4, 0:D]

    def mix_staged(buf, shift):
        def task(r, t):
            def get(i, j):
                tile = j * NT // 2 + t
                v = pltpu.bitcast(staged(i)[r:r + 8, tile * 128:(tile + 1) * 128], u32)
                return _unpack(pltpu.roll(v, 128 - 4 * tile, 1) if shift and tile else v)
            for m, v in enumerate(_factors(RIGHT, get)):
                buf.at[m][r:r + 8, t * 128:(t + 1) * 128] = _pack(v)
            return buf, r, t * 128
        return tasks(task, [(r, t) for r in range(0, D // 4, 8) for t in range(NT // 2)],
                     [z_s, zn_s], "lat_xlu" if shift else "lat_short", 30)

    def prep_qkv(j, buf, rows=range(0, D // 2, 16)):
        def task(i, r):
            w = pltpu.bitcast(raw.at[j][i * D // 2 + r:i * D // 2 + r + 16, :], u32)
            lane = lax.broadcasted_iota(jnp.int32, (8, 128), 1)
            w = [w[:, t * 128:(t + 1) * 128] for t in range(NT)]
            w = [pltpu.roll(v, 4 * t, 1) if t else v for t, v in enumerate(w)]
            w = [w[(-t) % NT] for t in range(NT)]
            for b in range(3):
                m = (lane & (4 << b)) != 0
                w = [jnp.where(m, w[(t - (1 << b)) % NT], w[t]) for t in range(NT)]
            for t in range(NT):
                staged(i)[r // 2:r // 2 + 8, t * 128:(t + 1) * 128] = pltpu.bitcast(w[t], f32)
            return (z_s, zn_s)[i], r // 2, 0
        second = mix_staged(buf, True)
        return (tasks(task, [(i, r) for r in rows for i in range(2)], [raw], "lat_xlu", 45) + gap,
                [second[r // 16 * NT // 2 + t] for r in rows for t in range(NT // 2)])

    def prep_wo():
        def task(d4, t2, hh, c):
            src = [((t2 * 4 + j) * 4 + hh) * 32 + d4 * 16 for j in range(4)]
            v = _pair_transpose([pltpu.bitcast(raw.at[3][s:s + 16, c:c + 256], u32) for s in src])
            for j in range(4):
                r = ((j * 4 + hh) * 32 + t2 * 16) // 2
                staged(d4)[r:r + 8, c:c + 256] = pltpu.bitcast(v[j], f32)
            return (z_s, zn_s)[d4], r, c
        return tasks(task, [(d4, t2, hh, c) for d4 in range(2) for t2 in range(2)
                            for hh in range(4) for c in range(0, D, 256)],
                     [raw], "lat_short", 40) + gap + mix_staged(wo_p, False)

    def prep_win(slab, bufs, first, count):
        ks = _Split(D, cfg["win"])

        def load(i, r, c):
            return raw.at[slab + c // (FH // 2)][
                _ds(ks.start(i) + r, 16, 16), c % (FH // 2):c % (FH // 2) + 128].astype(f32)
        rows = [((first + g) * 8, (first + g) * 16) for g in range(count)]
        return right_tasks(bufs, "win", FH, rows, load, [raw])

    def prep_wout(first, count):
        ks = _Split(FH, cfg["out"])

        def load(i, r, c):
            row = ks.start(i)
            return raw.at[2 + row // (FH // 2)][
                _ds(row % (FH // 2) + r, 16, 16), c:c + 128].astype(f32)
        rows = [((first + g) * 8, (first + g) * 16) for g in range(count)]
        return right_tasks((wout_p, None), "out", D, rows, load, [raw])

    def prep_wout_rest(first, count):
        ks, ns = _Split(FH, cfg["out"]), _Split(D, cfg["out"])

        def task(g, j, c):
            def get(a, b):
                col = ns.start(2 * b + j) + c
                return raw.at[2 + a][_ds(2 * ks.width + (first + g) * 16, 16, 16),
                                     col:col + 128].astype(f32)
            for o, v in enumerate(_factors(RIGHT, get)):
                wout_r.at[2 * o + j][_ds((first + g) * 8, 8, 8), c:c + 128] = _pack(v)
            return wout_r, (first + g) * 8, c
        if not ks.rest:
            return []
        return tasks(task, [(g, j, c) for g in range(count) for j in range(2)
                            for c in range(0, ns.width, 128)], [raw], "lat_short", 28)

    def prep_bias():
        def task(j):
            b = bsp_raw[...].astype(f32).reshape(1, S) * (1.0 / GAIN)
            bias_s[j * 128:(j + 1) * 128, :] = jnp.broadcast_to(
                b[:, j * 128:(j + 1) * 128], (128, 128)).T
            return bias_s, j * 128, 0
        return tasks(task, [(j,) for j in range(S // 128)], [], "lat_xlu", 50)

    def norm_tasks(base, src, st, eps=EPS, scale=None, rows=range(0, U, 16)):
        n = src.shape[1]
        st, inv = st

        def shift(r):
            v = src[_ds(r, 16, 16), 0:128].astype(f32)
            st.at[0][_ds(r, 16, 16), :] = jnp.broadcast_to(v[:, 0:1], (16, 128))
            return st, r, 0

        def stats(r):
            sh = st.at[0][_ds(r, 8, 8), :]
            s1 = s2 = None
            for c in range(0, n, 256):
                v = src[_ds(r, 8, 8), c:c + 256].astype(f32)
                for d in (v[:, :128] - sh, v[:, 128:] - sh):
                    s1 = d if s1 is None else s1 + d
                    s2 = d * d if s2 is None else s2 + d * d
            m = jnp.sum(s1, axis=-1, keepdims=True) * (1.0 / n)
            var = jnp.sum(s2, axis=-1, keepdims=True) * (1.0 / n) - m * m
            st.at[1][_ds(r, 8, 8), :] = sh + m
            st.at[2][_ds(r, 8, 8), :] = jnp.broadcast_to(jnp.maximum(var, 0.0) + eps, (8, 128))
            return st, r, 0

        def rstd(r):
            v = lax.rsqrt(st.at[2][_ds(r, 16, 16), :])
            inv[_ds(r, 16, 16), :] = v if scale is None else v * scale
            return inv, r, 0

        def load(r, c, h=16, w=128):
            v = src[_ds(r, h, h), c:c + w].astype(f32)
            mean, mul = [jnp.concatenate([t[_ds(r, h, h), :]] * (w // 128), axis=1)
                         for t in (st.at[1], inv)]
            return (v - mean) * mul

        def write(dst):
            def task(r, c, w):
                dst[_ds(r, 8, 8), c:c + w] = load(r, c, 8, w)
                return dst, r, c
            return tasks(task, [(r + j, c, min(1024, n - c)) for r in rows for j in (0, 8)
                                for c in range(0, n, 1024)], [base], "lat_short", 22)
        out = tasks(shift, [(r,) for r in rows], [base], "lat_xlu", 10)
        out += staggered(tasks(stats, [(r + j,) for r in rows for j in (0, 8)], [base], "lat_xlu",
                               n // 28 + 8),
                         tasks(rstd, [(r,) for r in rows], [], "lat_short", 22), cfg["lag_rstd"])
        return out, load, write

    def norm_x(u, buf):
        out, load, _ = norm_tasks(x_s, unit(x_s, u), st0)
        return out + left_tasks(buf, "qkv", D, lambda r, j, c: load(r, c), [x_s])

    def norm_h(u, spare, **kw):
        out, _, write = norm_tasks(x_s, unit(x_s, u), st1, scale=ALPHA, **kw)
        return out + write(spare)

    def left_h(spare, **kw):
        return left_tasks(ha, "win", D, lambda r, j, c: spare[_ds(r, 16, 16), c:c + 128], [spare],
                          **kw)

    def take(v, idx):
        return jnp.take_along_axis(v, idx, axis=1)

    def logit_tasks(first, q_s=q_s, k_s=k_s):
        def task(r, b):
            lane = lax.broadcasted_iota(jnp.int32, (8, 128), 1)
            acc = [None] * 4
            for t in range(NT):
                q = q_s[r:r + 8, t * 128:(t + 1) * 128]
                for j in range(4):
                    k0 = HALO + r - DIL * (4 * b + j)
                    term = q * k_s[t, k0:k0 + 8, :]
                    acc[j] = term if t == 0 else acc[j] + term
            for bit in (1, 2):
                odd = (lane & bit) != 0
                acc = [jnp.where(odd, acc[j ^ bit], acc[j]) for j in range(4)]
            lg = acc[0]
            for j in range(1, 4):
                lg = lg + take(acc[j], lane ^ j)
            lg = lg * float(DH) ** -0.5
            if first and r < DIL * WIN:
                pos = r + lax.broadcasted_iota(jnp.int32, (8, 128), 0)
                lg = jnp.where(pos >= DIL * (4 * b + (lane & 3)), lg, -1e9)
            l_s[b, r:r + 8, :] = lg
            return l_s, r, 0
        return tasks(task, [(r, b) for r in range(0, U, 8) for b in range(2)], [q_s, k_s],
                     "lat_xlu", 75)

    def softmax_tasks():
        def exps(r):
            lane = lax.broadcasted_iota(jnp.int32, (16, 128), 1)
            lg = [l_s[b, r:r + 16, :] for b in range(2)]
            mx = jnp.maximum(lg[0], lg[1])
            mx = functools.reduce(jnp.maximum, [mx] + [take(mx, lane ^ j) for j in range(1, 4)])
            for b in range(2):
                e_s[b, r:r + 16, :] = jnp.exp(lg[b] - mx)
            return e_s, r, 0

        def probs(r):
            lane = lax.broadcasted_iota(jnp.int32, (8, 128), 1)
            e = [e_s[b, r:r + 8, :] for b in range(2)]
            e = {4 * b + j: take(e[b], (lane & -4) | j) for j in range(4) for b in range(2)}
            inv = 1.0 / functools.reduce(lambda p, q: p + q, e.values())
            for w in range(WIN):
                p_s[w, r:r + 8, :] = e[w] * inv
            return p_s, r, 0
        return staggered(tasks(exps, [(r,) for r in range(0, U, 16)], [l_s], "lat_xlu", 40),
                         tasks(probs, [(r,) for r in range(0, U, 8)], [], "lat_xlu", 40),
                         cfg["lag_probs"])

    def value_tasks(v_s=v_s):
        def task(r, t0):
            acc = [None] * 4
            for w in range(WIN):
                k0 = HALO + r - DIL * w
                p = p_s[w, r:r + 8, :]
                for j in range(4):
                    term = p * v_s[t0 + j, k0:k0 + 8, :]
                    acc[j] = term if w == 0 else acc[j] + term
            for j in range(4):
                o_s[r:r + 8, (t0 + j) * 128:(t0 + j + 1) * 128] = acc[j]
            return o_s, r, t0 * 128
        out = []
        for g in range(0, U // 2 + 16, 16):
            if g < U // 2:
                out += tasks(task, [(g + b + j, t0) for b in (0, U // 2) for j in (0, 8)
                                    for t0 in (0, 4)], [p_s, v_s], "lat_short", 62)
            if g:
                out += left_tasks(oa, "wo", D, lambda r, j, c: o_s[r:r + 16, c:c + 128], [o_s],
                                  rows=[g - 16])
        return out

    def set_halo(buf, src):
        buf[:, 0:HALO, :] = (jnp.zeros((NT, HALO, 128), f32) if src is None
                             else src[:, U:U + HALO, :])

    def copies():
        half, part = FH // 2, D // 2 // PARTS

        def units(lo, hi):
            return [(x_hbm.at[0, lo * U:hi * U], x_s.at[lo * U:hi * U])]

        def weight(j, rows=(0,), n=D):
            return [(wqkv_hbm.at[r:r + n, j * D:(j + 1) * D], raw.at[j, r:r + n]) for r in rows]

        def rows_in(lo, hi):
            return [(win_hbm.at[r + lo:r + hi, j * half:(j + 1) * half],
                     raw.at[4 + j, r + lo:r + hi, 0:half])
                    for r in range(0, D, D // 4) for j in range(4)]
        early = share(0, NU - 2, D // 64)[1] * 16
        pairs = [("x0", units(0, 1))]
        pairs += [("wq%d" % j, weight(0, (j * part, D // 2 + j * part), part))
                  for j in range(PARTS)]
        pairs += [
            ("x1", units(1, 2)), ("wk", weight(1)), ("wv", weight(2)),
            ("wo", [(wo_hbm, raw.at[3, 0:D])] + units(2, 3)),
            ("early", units(3, 4) + rows_in(0, early)),
            ("rest", units(4, NU) + rows_in(early, D // 4) + [(bsp_hbm, bsp_raw)]),
            ("late0", [(wsp_hbm.at[0:D, j * D:(j + 1) * D], raw.at[j, 0:D]) for j in range(2)]
             + [(wout_hbm.at[j * half:(j + 1) * half], raw.at[2 + j, 0:half]) for j in range(2)]),
            ("late1", [(wsp_hbm.at[D:S, j * D:(j + 1) * D], raw.at[4 + j, 0:D])
                       for j in range(2)])]
        return {name: [(a, b, sem.at[j]) for a, b in group]
                for j, (name, group) in enumerate(pairs)}

    def start(*names):
        for name in names:
            for args in copies()[name]:
                pltpu.make_async_copy(*args).start()

    def wait(name):
        for args in copies()[name]:
            pltpu.make_async_copy(*args).wait()

    def out_copy(u, half):
        rows = _ds(u * U + half * U // 2, U // 2, U // 2)
        return pltpu.make_async_copy(x_s.at[rows], out_hbm.at[0, rows], osem.at[2 * u + half])

    def unit(ref, u, n=U):
        return ref.at[_ds(u * n, n, n)]

    def clip(v, lo, hi):
        return min(max(v, lo), hi) if isinstance(v, int) else jnp.clip(v, lo, hi)

    def share(step, steps, total):
        count = -(-total // steps)
        return clip(step * count, 0, total - count), count

    def add_into(u):
        def store(r, c, v):
            idx = (slice(r, r + v.shape[0]), slice(c, c + v.shape[1]))
            dst = unit(x_s, u)
            dst[idx] = (dst[idx].astype(f32) + v).astype(bf16)
        return store

    def put_rows(buf):
        def store(r, c, v):
            buf[r:r + v.shape[0], c:c + 128] = v
        return store

    def put_slab(buf):
        def store(r, c, v):
            buf[c // 128, HALO + r:HALO + r + v.shape[0], :] = v
        return store

    def qkv(src, w, store):
        return matmul(src, (w, None), "qkv", D, D, store)

    def project(u):
        return matmul(oa, (wo_p, None), "wo", D, D, add_into(u), cfg["cw_wo"])

    def first_attention():
        set_halo(kv_s, None)
        wait("x1")
        overlap(qkv(xb, wq_p, put_rows(o_s)), norm_x(1, xa))
        wait("wk")
        overlap(qkv(xa, wq_p, put_rows(q_s)), sum(prep_qkv(1, wk_p), []))
        wait("wv")
        prep, logits, soft = sum(prep_qkv(2, wv_p), []), logit_tasks(False), softmax_tasks()
        overlap(qkv(xb, wk_p, put_slab(kv_s)), prep)
        set_halo(k_s, kv_s)
        overlap(qkv(xa, wk_p, put_slab(k_s)), logit_tasks(True, o_s, kv_s))
        wait("wo")
        prep = prep_wo()
        overlap(qkv(xb, wv_p, put_slab(kv_s)), soft, prep)
        set_halo(v_s, kv_s)
        overlap(qkv(xa, wv_p, put_slab(v_s)), value_tasks(kv_s), logits[:cfg["f_log"]])
        overlap(project(0), (logits[cfg["f_log"]:], 0, cfg["f_end"]), norm_x(2, xa))

    def step_attention(u):
        if cfg["part"] != "s1":
            @pl.when(u == 3)
            def _():
                wait("rest")
        begin, count = share(u - 2, NU - 2, _Split(D, cfg["win"]).width // 16)
        prep = (prep_win(6, (wz2_p, wz2_r), begin, count)
                + prep_win(4, (wz1_p, wz1_r), begin, count))
        cut = len(prep) * cfg["cut_prep"] // 8
        g = clip(u - 2, 0, U // 64 - 1) * 16
        head = norm_h(0, z_s, rows=[g + b for b in range(0, U, 64)]) + left_h(z_s, rows=[g])
        logits = logit_tasks(False)
        set_halo(k_s, k_s)
        overlap(qkv(xa, wq_p, put_rows(q_s)), softmax_tasks(), prep[:cut])
        overlap(qkv(xa, wk_p, put_slab(k_s)), value_tasks())
        set_halo(v_s, v_s)
        overlap(qkv(xa, wv_p, put_slab(v_s)), logits, head)
        overlap(project(u - 1), norm_x(clip(u + 1, 0, NU - 1), xa), prep[cut:])

    def spatial_left(u, rows=range(0, U // 4, 16)):
        per = D // U

        def regroup(r, m):
            lane = lax.broadcasted_iota(jnp.int32, (8, 128), 1)
            col = 2 * U * m
            w = pltpu.bitcast(raw.at[u // per * 4 + col // D][
                _ds(u % per * U + r, 16, 16), col % D:col % D + 2 * U], u32)
            for a in range(2):
                one, two = w[:, a * 128:(a + 1) * 128], w[:, U + a * 128:U + (a + 1) * 128]
                mid = pltpu.roll(jnp.where(lane < 64, two, one), 64, 1)
                for j, v in ((2 * a, jnp.where(lane < 64, one, mid)),
                             (2 * a + 1, jnp.where(lane < 64, mid, two))):
                    sp_s[_ds(r // 2, 8, 8), j * 512 + m * 128:j * 512 + (m + 1) * 128] = v
            return sp_s, r // 2, m * 128
        return tasks(regroup, [(b + r, m) for r in rows for b in range(0, U, U // 4)
                               for m in range(NU // 2)], [raw], "lat_xlu", 18) + left_tasks(
            sa, "sp", S, lambda r, j, c: _unpack(sp_s[_ds(r // 2, 8, 8), c:c + 128]), [sp_s],
            rows=rows)

    def gate_input():
        def store(r, c, v):
            z_s[r:r + v.shape[0], c:c + 128] = _gelu(v)
        return matmul(ha, (wz2_p, wz2_r), "win", D, FH, store)

    def value_input(u, more):
        z1t = unit(z1_s, u, U // 2)
        h = U // 4

        def store(r, c, v):
            z1t[r // 2:(r + v.shape[0]) // 2, c:c + 128] = _pack(_gelu(v))
        stats, _, write = norm_tasks(z_s, z_s, st0, EPS * GAIN * GAIN, 1.0 / GAIN)
        factors = right_tasks((z2n_p, z2n_r), "sp", FH,
                              [(u * (h // 2) + r // 2, r) for r in range(0, h, 16)],
                              lambda b, r, c: zn_s[b * h + r:b * h + r + 16, c:c + 128], [zn_s])
        main = matmul(ha, (wz1_p, wz1_r), "win", D, FH, store, rest_first=True)
        last = main[0] - 49
        if more:
            overlap(main, (stats + write(zn_s) + factors, 0, last + cfg["z_over"]),
                    *[(left_h(q_s, outer=[o]), last + 7 * j + 6, last + 7 * j + 13)
                      for j, o in enumerate(ORDER[:cfg["z_left"]])])
        else:
            overlap(main, stats + write(zn_s) + factors, spatial_left(0, [32, 48]))

    def last_attention():
        main = gate_input()
        overlap(main, (softmax_tasks(), 0, cfg["soft_end"]),
                (value_tasks(), cfg["soft_end"], main[0]))
        overlap(project(NU - 1), prep_bias() + spatial_left(0, [0, 16]) + norm_h(1, q_s))

    def step_input(u):
        value_input(u - 1, True)
        prep = (prep_wout(*share(u - 1, NU - 1, _Split(FH, cfg["out"]).width // 16))
                + prep_wout_rest(*share(u - 1, NU - 1, 8)))
        late = ORDER[cfg["z_left"]:]
        main = gate_input()
        overlap(main, (left_h(q_s, outer=late[:1]) + left_h(q_s, outer=late[1:]), 0, 7 * len(late)),
                (norm_h(clip(u + 1, 0, NU - 1), q_s), 7 * len(late), main[0]),
                (prep, 7 * len(late), main[0]))

    def step_output(u):
        bt, z1t = unit(bias_s, u), unit(z1_s, u, U // 2)

        def put_y(r, c, g):
            n = g.shape[0]
            z_s[r:r + n, c:c + 128] = _unpack(z1t[r // 2:(r + n) // 2, c:c + 128]) * (
                g + bt[r:r + n, :])

        def gated(**kw):
            return left_tasks(ya, "out", FH, lambda r, j, c: z_s[r:r + 16, c:c + 128], [z_s], **kw)
        overlap(matmul(sa, (z2n_p, z2n_r), "sp", S, FH, put_y),
                *[(gated(cols=[128 * j], rest=False), 49 * j + 49, 49 * j + 49 + 20)
                  for j in range(3)])
        run(gated(cols=[]))
        overlap(matmul(ya, (wout_p, wout_r), "out", FH, D, add_into(u), 256),
                spatial_left(clip(u + 1, 0, NU - 1)),
                ([(out_copy(u, 1).start, [], 0, 1)], 36, 37))
        out_copy(u, 0).start()

    def make_zero():
        bits = pltpu.bitcast(x_s[0:16, 0:128], jnp.int32)
        zero.append(bits[0, 0] ^ pltpu.roll(bits, 1, 1)[0, 1])

    def keep(j):
        v = None
        for b in (wq_p, wk_p, wv_p, wo_p, wz1_p, wz1_r, wz2_p, wz2_r, wout_p, wout_r, z2n_p,
                  z2n_r, z1_s, bias_s, xa, xb, oa, ha, sa, ya, q_s, o_s, k_s, v_s, kv_s, p_s, l_s, e_s,
                  z_s, zn_s, sp_s, *st0, *st1, tmp_s):
            v = done(b, 0, 0) if v is None else v | done(b, 0, 0)
        x_s[0:16, 0:128] = _as_bf16(v)
        c = pltpu.make_async_copy(x_s.at[0:16, 0:128], out_hbm.at[0, 0:16, 0:128], sem.at[0])
        c.start()
        c.wait()

    if cfg["part"] in ("s1", "s2", "s3", "mid"):
        make_zero()
        if cfg["part"] == "mid":
            last_attention()
            value_input(NU - 1, False)
        else:
            pl.loop(1, NU)({"s1": step_attention, "s2": step_input, "s3": step_output}[cfg["part"]])
        if cfg["part"] == "s3":
            for u in range(1, NU):
                out_copy(u, 0).wait()
                out_copy(u, 1).wait()
        pl.loop(0, 2)(keep)
        return
    import contextlib
    scope = jax.named_scope if cfg["prof"] else (lambda n: contextlib.nullcontext())
    with scope("p_x0"):
        start(*list(copies())[:-2])
        wait("x0")
    with scope("p_norm"):
        make_zero()
        run(norm_x(0, xb))
    for j in range(PARTS):
        with scope("p_wq"):
            wait("wq%d" % j)
        with scope("p_prepq"):
            part = D // 2 // PARTS
            run(sum(prep_qkv(0, wq_p, range(j * part, (j + 1) * part, 16)), []))
    with scope("p_first"):
        first_attention()
    with scope("p_rest0"):
        wait("early")
    if cfg["part"] == "first":
        wait("rest")
        pl.loop(0, 2)(keep)
        return
    start("late0")

    def sc(name, fn):
        def g(u):
            with scope(name):
                fn(u)
        return g
    with scope("p_loop1"):
        pl.loop(2, NU)(sc("p_it1", step_attention))
    start("late1")
    with scope("p_rest2"):
        wait("late0")
    with scope("p_mid"):
        last_attention()
    with scope("p_loop2"):
        pl.loop(1, NU)(sc("p_it2", step_input))
    with scope("p_mid2"):
        value_input(NU - 1, False)
    wait("late1")
    with scope("p_loop3"):
        pl.loop(0, NU)(sc("p_it3", step_output))
    with scope("p_out"):
        for u in range(NU):
            out_copy(u, 0).wait()
            out_copy(u, 1).wait()


def build(cfg, interpret=False, name="fused_block"):
    vm = pltpu.VMEM

    def right(key, k, n):
        ks, ns = _Split(k, cfg[key]), _Split(n, cfg[key])
        main = vm((7 ** ks.level, ks.width // 2, ns.width), u32)
        if ns.rest:
            return [main, vm((21, ks.width // 2, 128), u32)]
        if ks.rest:
            return [main, vm((14, 64, ns.width), u32)]
        return [main]

    def left(key, k):
        ks = _Split(k, cfg[key])
        return vm((7 ** ks.level * U // ks.parts // 2, ks.width + ks.rest), u32)
    scratch = [
        vm((S + 16, D), bf16),
        vm((8, D + 16, D), bf16),
        vm((S,), bf16),
        *right("qkv", D, D) * 3, *right("wo", D, D),
        *right("win", D, FH), *right("win", D, FH), *right("out", FH, D), *right("sp", S, FH),
        vm((S // 2, FH), u32),
        vm((S, 128), f32),
        left("qkv", D), left("qkv", D), left("wo", D), left("win", D), left("sp", S),
        left("out", FH),
        *[vm((U + 8, D), f32)] * 2,
        *[vm((NT, HALO + U + 8, 128), f32)] * 3,
        vm((WIN, U + 8, 128), f32),
        *[vm((2, U + 8, 128), f32)] * 2,
        *[vm((U + 8, FH), f32)] * 2,
        vm((U // 2 + 8, S), u32),
        *[vm((3, U + 8, 128), f32)] * 2,
        *[vm((U, 128), f32)] * 2,
        vm((25 * U // 4, 256), f32),
        pltpu.SemaphoreType.DMA((9 + PARTS,)),
        pltpu.SemaphoreType.DMA((2 * NU,)),
    ]
    hbm = pl.BlockSpec(memory_space=pl.ANY)
    return pl.pallas_call(
        functools.partial(_kernel, cfg),
        out_shape=jax.ShapeDtypeStruct((1, S, D), bf16),
        in_specs=[hbm] * 7,
        out_specs=hbm,
        scratch_shapes=scratch,
        compiler_params=pltpu.CompilerParams(vmem_limit_bytes=127 * 1024 * 1024,
                                             flags=cfg["flags"]),
        interpret=interpret,
        name=name,
    )


@jax.jit
def pallas_sequential_preLN__sliding_local_dilated__mixer_gmlp__prompt_kernel(
    A_x: jax.Array,
    A_wqkv: jax.Array,
    A_wo: jax.Array,
    B_x: jax.Array,
    B_w_in: jax.Array,
    B_w_sp: jax.Array,
    B_b_sp: jax.Array,
    B_w_out: jax.Array,
):
    del B_x
    return build(CFG)(A_x, A_wqkv, A_wo, B_w_in, B_w_sp, B_b_sp, B_w_out)
```

```python
import functools

import jax
import jax.numpy as jnp
import numpy as np
from jax import lax
from jax.experimental import pallas as pl
from jax.experimental.pallas import tpu as pltpu

S = 2048
D = 1024
FH = 1792
DH = 32
WIN = 8
DIL = 2
HALO = 16
U = 256
NU = S // U
NT = D // 128
PARTS = 4
EPS = 1e-5

f32 = jnp.float32
bf16 = jnp.bfloat16
u32 = jnp.uint32

CFG = dict(part="all", flags=None, qkv=1, wo=1, win=2, sp=2, out=2, slot=32,
           lat_short=320, lat_xlu=512, tail=0, regs=('win', 'sp'), cw_wo=128, cut_prep=6, z_over=21, z_left=3, z_cut=3, fq=2, f_log=24, f_end=26, gap=100, lag_rstd=6, lag_probs=2, peel=True, wq_parts=4, depth=6, soft_end=90, prof=False)

ORDER = (0, 3, 1, 2, 5, 4, 6)
REST = (3, 1, 2, 4)


def _pack(v):
    return pltpu.bitcast(v.astype(bf16), u32)


def _as_bf16(v):
    return pltpu.bitcast(v, bf16)


def _unpack(v):
    return pltpu.bitcast(v, bf16).astype(f32)


_C = float(np.sqrt(2.0 / np.pi))
ALPHA = float((_C * 0.044715) ** (1.0 / 3.0))
GAIN = 2.0 * ALPHA


def _gelu(v):
    return v * (1.0 + jnp.tanh(v * (_C / ALPHA + v * v)))


LEFT = (((1, 0, 0), (1, 1, 1)), ((1, 1, 0), (1, 1, 1)), ((1, 0, 0),), ((1, 1, 1),),
        ((1, 0, 0), (1, 0, 1)), ((1, 1, 0), (-1, 0, 0)), ((1, 0, 1), (-1, 1, 1)))
RIGHT = (((1, 0, 0), (1, 1, 1)), ((1, 0, 0),), ((1, 0, 1), (-1, 1, 1)), ((1, 1, 0), (-1, 0, 0)),
         ((1, 1, 1),), ((1, 0, 0), (1, 0, 1)), ((1, 1, 0), (1, 1, 1)))


def _factor(terms, get):
    v = get(*terms[0][1:])
    for sign, i, j in terms[1:]:
        v = v + get(i, j) if sign > 0 else v - get(i, j)
    return v


def _factors(forms, get):
    blk = {(i, j): get(i, j) for i in range(2) for j in range(2)}
    return [_factor(terms, lambda i, j: blk[i, j]) for terms in forms]


class _Blocks:
    level, parts, rest = 2, 4, 0

    def __init__(self, chunks):
        self.chunks, self.width = chunks, 128 * len(chunks)

    def col(self, j, c):
        return self.chunks[c // 128][j]


Z1_COLS = _Blocks([[c + s for s in (0, 384, 896, 1280)] for c in (0, 128, 256)])
Z2_COLS = _Blocks([[FH + c for c in chunk] for chunk in Z1_COLS.chunks]
                  + [[FH + 768, FH + 1664, 768, 1664]])


class _Held:
    def __setitem__(self, _, v):
        self.v = v

    def __getitem__(self, _):
        return self.v


def _combiner(tmp, put):
    t1, t2, t3, t4, t5 = tmp

    def feed(i, m):
        if i == 0:
            t1[...] = m
        elif i == 3:
            t4[...] = m
        elif i == 1:
            t2[...] = m
            put(1, 0, m + t4[...])
        elif i == 2:
            t3[...] = m
        elif i == 5:
            put(1, 1, (t1[...] - t2[...] + t3[...]) + m)
        elif i == 4:
            t5[...] = m
            put(0, 1, m + t3[...])
        else:
            put(0, 0, (t1[...] + t4[...] - t5[...]) + m)
    return feed


class _Split:
    def __init__(self, n, level):
        self.level, self.parts = level, 1 << level
        self.width = n // self.parts // 128 * 128
        self.rest = n // 2 - 2 * self.width if level == 2 else 0
        self.half = n // 2

    def start(self, j):
        if self.level == 1:
            return j * self.half
        return (j // 2) * self.half + (j % 2) * self.width

    def col(self, j, c):
        return self.start(j) + c

    def rest_start(self, h):
        return h * self.half + 2 * self.width


def _pair_transpose(v):
    sub = lax.broadcasted_iota(jnp.int32, v[0].shape, 0)
    v = list(v)
    for b in range(2):
        s = 1 << b
        m = (sub & (2 * s)) != 0
        nv = list(v)
        for j in range(4):
            if j & s:
                continue
            lo, hi = v[j], v[j + s]
            nv[j] = jnp.where(m, pltpu.roll(hi, 2 * s, 0), lo)
            nv[j + s] = jnp.where(m, hi, pltpu.roll(lo, 8 - 2 * s, 0))
        v = nv
    return v


def _ds(start, size, align):
    return pl.ds(start if isinstance(start, int) else pl.multiple_of(start, align), size)


def _kernel(cfg,
            x_hbm, wqkv_hbm, wo_hbm, win_hbm, wsp_hbm, bsp_hbm, wout_hbm, out_hbm,
            x_s, raw, bsp_raw,
            wq_p, wk_p, wv_p, wo_p, wz1_p, wz2_p, wout_p, wout_r, z2n_p, z2n_r,
            z1_s, bias_s, xa, xb, oa, ha, sa, ya,
            q_s, o_s, k_s, v_s, kv_s, p_s, l_s, e_s, z_s, zn_s, sp_s, st0_s, st1_s, inv0_s, inv1_s, tmp_s,
            sem, osem):
    st0, st1 = (st0_s, inv0_s), (st1_s, inv1_s)
    zero = []

    def spot(ref, row, col):
        n = 8 * (4 // ref.dtype.itemsize)
        ref = ref if len(ref.shape) == 2 else ref.at[zero[0]]
        return ref.at[_ds(row + zero[0] * n, n, n), _ds(col + zero[0] * 128, 128, 128)]

    def gate(ref, v):
        n = 8 * (4 // ref.dtype.itemsize)
        spot(ref, ref.shape[-2] - n, 0)[0:8, :] = v.astype(ref.dtype)

    def done(ref, row, col):
        v = spot(ref, row, col)[...]
        return v if v.dtype == u32 else pltpu.bitcast(v, u32)

    def tied(toks):
        def tie(b):
            if not toks:
                return b
            tok = functools.reduce(lambda p, q: p | q, toks)
            tok = jnp.concatenate([tok] * (b.shape[1] // 128), axis=1)
            always = lax.broadcasted_iota(jnp.int32, tok.shape, 0) >= zero[0]
            parts = []
            for r in range(0, b.shape[0], 64):
                parts += [b[r:r + 56], jnp.where(always, b[r + 56:r + 64], tok)]
            return jnp.concatenate(parts, axis=0)
        return tie

    def overlap(main, *sides):
        n, cyc, gen = main
        per = max(1, cyc // cfg["slot"])
        plan = [[] for _ in range(n * per)]
        for side in sides:
            if not isinstance(side, tuple):
                side = (side, 0, n)
            todo, first, last = side
            if todo and last == n:
                last -= (todo[-1][2] + cfg["tail"]) / cyc
            span = max(1, int((last - first) * per))
            total, spent = sum(t[3] for t in todo), 0
            for t in todo:
                plan[int(first * per) + spent * span // total].append(t)
                spent += t[3]
        next(gen)
        due = [[] for _ in range(n)]
        for i, todo in enumerate(plan):
            if i % per == 0:
                res = gen.send(tied([tok for _, tok in due[i // per]]))
            gated = []
            for _, refs, _, _ in todo:
                gated += [r for r in refs if not any(r is g for g in gated)]
            row = res.shape[0] * (i % per) // per
            for r in gated:
                gate(r, res[row:row + 8, 0:128])
            for fn, _, lat, _ in todo:
                where = fn()
                j = -(-(i * cyc // per + lat) // cyc)
                if where is not None and j < n:
                    due[j] = [d for d in due[j] if d[0] is not where[0]]
                    due[j].append((where[0], done(*where)))

    def tasks(fn, args, refs, lat, cost):
        return [(functools.partial(fn, *a), refs, cfg[lat], cost) for a in args]

    def staggered(early, late, lag):
        per = len(early) / len(late)
        order = [(j, t) for j, t in enumerate(early)]
        order += [((j + 1) * per + lag - 0.5, t) for j, t in enumerate(late)]
        return [t for _, t in sorted(order, key=lambda p: p[0])]

    gap = [(lambda: None, [], 0, cfg["gap"])]

    def run(todo):
        for t in todo:
            t[0]()

    def left_tasks(ref, key, k, load, refs, rows=None, cols=None, outer=None, rest=True):
        ks = _Split(k, cfg[key])
        h = U // ks.parts

        def put(n, r, c, v):
            ref[_ds(n * h // 2 + r // 2, 8, 8), c:c + 128] = _pack(v)

        def main(r, c, o):
            def get(i, j):
                if ks.level == 1:
                    return load(i * h + r, j, ks.start(j) + c)
                return _factor(LEFT[o], lambda a, b: load((2 * a + i) * h + r, 2 * b + j,
                                                          ks.start(2 * b + j) + c))
            for n, v in enumerate(_factors(LEFT, get)):
                put(7 * o + n, r, c, v)
            return ref, 7 * o * h // 2 + r // 2, c

        def other(r, i):
            vals = _factors(LEFT, lambda a, b: load((2 * a + i) * h + r, None, ks.rest_start(b)))
            for o, v in enumerate(vals):
                put(7 * o + 6 - i, r, ks.width, v)
            return ref, (6 - i) * h // 2 + r // 2, ks.width
        out = []
        for r in range(0, h, 16) if rows is None else rows:
            out += tasks(main, [(r, c, o)
                                for c in (range(0, ks.width, 128) if cols is None else cols)
                                for o in (range(7 ** (ks.level - 1)) if outer is None else outer)],
                         refs, "lat_short", 30)
            out += tasks(other, [(r, 0), (r, 1)] if ks.rest and rest else [], refs, "lat_short", 30)
        return out

    def right_tasks(bufs, key, n, rows, load, refs):
        main_p, rest_p = bufs
        ns = n if isinstance(n, _Blocks) else _Split(n, cfg[key])

        def main(prow, r, c, o):
            def get(i, j):
                if ns.level == 1:
                    return load(i, r, ns.start(j) + c)
                return _factor(RIGHT[o], lambda a, b: load(2 * a + i, r, ns.col(2 * b + j, c)))
            for m, v in enumerate(_factors(RIGHT, get)):
                main_p.at[7 * o + m][_ds(prow, 8, 8), c:c + 128] = _pack(v)
            return main_p, prow, c

        def rest(prow, r, o):
            top, bot = [_factor(RIGHT[o], lambda a, b: load(2 * a + i, r, ns.rest_start(b)))
                        for i in range(2)]
            for m, v in enumerate((top, bot, top - bot)):
                rest_p.at[3 * o + m][_ds(prow, 8, 8), :] = _pack(v)
            return rest_p, prow, 0
        out = []
        for prow, r in rows:
            out += tasks(main, [(prow, r, c, o) for c in range(0, ns.width, 128)
                                for o in range(7 ** (ns.level - 1))], refs, "lat_short", 32)
            out += tasks(rest, [(prow, r, o) for o in range(7)] if ns.rest else [], refs,
                         "lat_short", 16)
        return out

    def matmul(ref, bufs, key, k, n, store, cw=128):
        main_p, rest_p = bufs
        ks = _Split(k, cfg[key])
        ns = n if isinstance(n, _Blocks) else _Split(n, cfg[key])
        h = U // ks.parts

        def lhs(m, lo, hi):
            return _as_bf16(ref[m * h // 2:(m + 1) * h // 2, lo:hi])

        def dot(a, b):
            return jnp.dot(a, _as_bf16(b), preferred_element_type=f32)

        def temps(slot):
            return [tmp_s.at[(5 * slot + j) * h:(5 * slot + j + 1) * h, 0:cw] for j in range(5)]

        def gen1():
            tie = yield
            for c in range(0, ns.width, cw):
                feed = _combiner(temps(0), lambda i, j, v: store(i * h, ns.start(j) + c, v))
                for m in ORDER:
                    res = dot(lhs(m, 0, ks.width), tie(main_p.at[m][:, c:c + cw]))
                    feed(m, res)
                    tie = yield res

        def inner_temps():
            return [_Held() for _ in range(5)] if key in cfg["regs"] else temps(4)

        def chunk(c, tie):
            def put(i, j):
                return lambda a, b, v: store((2 * a + i) * h, ns.col(2 * b + j, c), v)
            outer = {(i, j): _combiner(temps(2 * i + j), put(i, j))
                     for i in range(2) for j in range(2)}
            for o in ORDER:
                def extra(i, j, v):
                    if ks.rest and i != j:
                        v = v + dot(lhs(7 * o + 6 - i, ks.width, ks.width + 128),
                                    rest_p.at[2 * o + j][:, c:c + cw])
                    outer[i, j](o, v)
                feed = _combiner(inner_temps(), extra)
                for m in ORDER:
                    b = main_p.at[7 * o + m][:, c:c + cw]
                    hi = ks.width
                    if ks.rest and m >= 5:
                        b = jnp.concatenate([b, rest_p.at[2 * o + 6 - m][:, c:c + cw]], axis=0)
                        hi += 128
                    res = dot(lhs(7 * o + m, 0, hi), tie(b))
                    feed(m, res)
                    tie = yield res
            return tie

        def rest_chunk(tie):
            def put(i):
                return lambda a, b, v: store((2 * a + i) * h, ns.rest_start(b), v)
            outer = [_combiner(temps(i), put(i)) for i in range(2)]
            for o in ORDER:
                for i, (m0, b0), (m1, b1) in ((1, (3, 2), (1, 0)), (0, (2, 2), (4, 1))):
                    first = dot(lhs(7 * o + m0, 0, ks.width), tie(rest_p.at[3 * o + b0][...]))
                    tie = yield first
                    res = dot(lhs(7 * o + m1, 0, ks.width), tie(rest_p.at[3 * o + b1][...]))
                    outer[i](o, res - first if i else res + first)
                    tie = yield res
            return tie

        def gen2():
            tie = yield
            for c in range(0, ns.width, cw):
                tie = yield from chunk(c, tie)
            if ns.rest:
                tie = yield from rest_chunk(tie)
        cyc = h // 16 * 4 * (ks.width // 128) * (cw // 128)
        if ks.level == 1:
            return 7 * (ns.width // cw), cyc, gen1()
        return 49 * (ns.width // cw) + (28 if ns.rest else 0), cyc, gen2()

    def staged(i):
        return (z_s, zn_s)[i].at[0:D // 4, 0:D]

    def mix_staged(buf, shift, plain=None):
        def task(r, t):
            def get(i, j):
                tile = j * NT // 2 + t
                v = pltpu.bitcast(staged(i)[r:r + 8, tile * 128:(tile + 1) * 128], u32)
                v = pltpu.roll(v, 128 - 4 * tile, 1) if shift and tile else v
                if plain is not None and i != j:
                    plain[i * D // 4 + r:i * D // 4 + r + 8, t * 128:(t + 1) * 128] = v
                return _unpack(v)
            for m, v in enumerate(_factors(RIGHT, get)):
                buf.at[m][r:r + 8, t * 128:(t + 1) * 128] = _pack(v)
            return buf, r, t * 128
        return tasks(task, [(r, t) for r in range(0, D // 4, 8) for t in range(NT // 2)],
                     [z_s, zn_s], "lat_xlu" if shift else "lat_short", 30)

    def prep_qkv(j, buf, part, parts, plain=None):
        def task(i, r):
            w = pltpu.bitcast(raw.at[j][i * D // 2 + r:i * D // 2 + r + 16, :], u32)
            lane = lax.broadcasted_iota(jnp.int32, (8, 128), 1)
            w = [w[:, t * 128:(t + 1) * 128] for t in range(NT)]
            w = [pltpu.roll(v, 4 * t, 1) if t else v for t, v in enumerate(w)]
            w = [w[(-t) % NT] for t in range(NT)]
            for b in range(3):
                m = (lane & (4 << b)) != 0
                w = [jnp.where(m, w[(t - (1 << b)) % NT], w[t]) for t in range(NT)]
            for t in range(NT):
                staged(i)[r // 2:r // 2 + 8, t * 128:(t + 1) * 128] = pltpu.bitcast(w[t], f32)
            return (z_s, zn_s)[i], r // 2, 0
        rows = range(part * D // 2 // parts, (part + 1) * D // 2 // parts, 16)
        second = mix_staged(buf, True, plain)
        return (tasks(task, [(i, r) for r in rows for i in range(2)], [raw], "lat_xlu", 45) + gap
                + [second[r // 16 * NT // 2 + t] for r in rows for t in range(NT // 2)])

    def prep_wo():
        def task(d4, t2, hh, c):
            src = [((t2 * 4 + j) * 4 + hh) * 32 + d4 * 16 for j in range(4)]
            v = _pair_transpose([pltpu.bitcast(raw.at[3][s:s + 16, c:c + 256], u32) for s in src])
            for j in range(4):
                r = ((j * 4 + hh) * 32 + t2 * 16) // 2
                staged(d4)[r:r + 8, c:c + 256] = pltpu.bitcast(v[j], f32)
            return (z_s, zn_s)[d4], r, c
        return tasks(task, [(d4, t2, hh, c) for d4 in range(2) for t2 in range(2)
                            for hh in range(4) for c in range(0, D, 256)],
                     [raw], "lat_short", 40) + gap + mix_staged(wo_p, False)

    def prep_win(buf, cols, first, count):
        ks = _Split(D, cfg["win"])

        def load(i, r, c):
            return raw.at[4 + c // (FH // 2)][
                _ds(ks.start(i) + r, 16, 16), c % (FH // 2):c % (FH // 2) + 128].astype(f32)
        rows = [((first + g) * 8, (first + g) * 16) for g in range(count)]
        return right_tasks((buf, None), "win", cols, rows, load, [raw])

    def prep_wout(first, count):
        ks = _Split(FH, cfg["out"])

        def load(i, r, c):
            row = ks.start(i)
            return raw.at[2 + row // (FH // 2)][
                _ds(row % (FH // 2) + r, 16, 16), c:c + 128].astype(f32)
        rows = [((first + g) * 8, (first + g) * 16) for g in range(count)]
        return right_tasks((wout_p, None), "out", D, rows, load, [raw])

    def prep_wout_rest(first, count):
        ks, ns = _Split(FH, cfg["out"]), _Split(D, cfg["out"])

        def task(g, j, c):
            def get(a, b):
                col = ns.start(2 * b + j) + c
                return raw.at[2 + a][_ds(2 * ks.width + (first + g) * 16, 16, 16),
                                     col:col + 128].astype(f32)
            for o, v in enumerate(_factors(RIGHT, get)):
                wout_r.at[2 * o + j][_ds((first + g) * 8, 8, 8), c:c + 128] = _pack(v)
            return wout_r, (first + g) * 8, c
        if not ks.rest:
            return []
        return tasks(task, [(g, j, c) for g in range(count) for j in range(2)
                            for c in range(0, ns.width, 128)], [raw], "lat_short", 28)

    def prep_bias():
        def task(j):
            b = bsp_raw[...].astype(f32).reshape(1, S) * (1.0 / GAIN)
            bias_s[j * 128:(j + 1) * 128, :] = jnp.broadcast_to(
                b[:, j * 128:(j + 1) * 128], (128, 128)).T
            return bias_s, j * 128, 0
        return tasks(task, [(j,) for j in range(S // 128)], [], "lat_xlu", 50)

    def norm_tasks(base, src, st, eps=EPS, scale=None, rows=range(0, U, 16)):
        n = src.shape[1]
        st, inv = st

        def shift(r):
            v = src[_ds(r, 16, 16), 0:128].astype(f32)
            st.at[0][_ds(r, 16, 16), :] = jnp.broadcast_to(v[:, 0:1], (16, 128))
            return st, r, 0

        def stats(r):
            sh = st.at[0][_ds(r, 8, 8), :]
            s1 = s2 = None
            for c in range(0, n, 256):
                v = src[_ds(r, 8, 8), c:c + 256].astype(f32)
                for d in (v[:, :128] - sh, v[:, 128:] - sh):
                    s1 = d if s1 is None else s1 + d
                    s2 = d * d if s2 is None else s2 + d * d
            m = jnp.sum(s1, axis=-1, keepdims=True) * (1.0 / n)
            var = jnp.sum(s2, axis=-1, keepdims=True) * (1.0 / n) - m * m
            st.at[1][_ds(r, 8, 8), :] = sh + m
            st.at[2][_ds(r, 8, 8), :] = jnp.broadcast_to(jnp.maximum(var, 0.0) + eps, (8, 128))
            return st, r, 0

        def rstd(r):
            v = lax.rsqrt(st.at[2][_ds(r, 16, 16), :])
            inv[_ds(r, 16, 16), :] = v if scale is None else v * scale
            return inv, r, 0

        def load(r, c, h=16, w=128):
            v = src[_ds(r, h, h), c:c + w].astype(f32)
            mean, mul = [jnp.concatenate([t[_ds(r, h, h), :]] * (w // 128), axis=1)
                         for t in (st.at[1], inv)]
            return (v - mean) * mul

        def write(dst):
            def task(r, c, w):
                dst[_ds(r, 8, 8), c:c + w] = load(r, c, 8, w)
                return dst, r, c
            return tasks(task, [(r + j, c, min(1024, n - c)) for r in rows for j in (0, 8)
                                for c in range(0, n, 1024)], [base], "lat_short", 22)
        out = tasks(shift, [(r,) for r in rows], [base], "lat_xlu", 10)
        out += staggered(tasks(stats, [(r + j,) for r in rows for j in (0, 8)], [base], "lat_xlu",
                               n // 28 + 8),
                         tasks(rstd, [(r,) for r in rows], [], "lat_short", 22), cfg["lag_rstd"])
        return out, load, write

    def norm_x(u, buf):
        out, load, _ = norm_tasks(x_s, unit(x_s, u), st0)
        return out + left_tasks(buf, "qkv", D, lambda r, j, c: load(r, c), [x_s])

    def norm_h(u, spare, **kw):
        out, _, write = norm_tasks(x_s, unit(x_s, u), st1, scale=ALPHA, **kw)
        return out + write(spare)

    def left_h(spare, **kw):
        return left_tasks(ha, "win", D, lambda r, j, c: spare[_ds(r, 16, 16), c:c + 128], [spare],
                          **kw)

    def take(v, idx):
        return jnp.take_along_axis(v, idx, axis=1)

    def logit_tasks(first, q_s=q_s, k_s=k_s):
        def task(r, b):
            lane = lax.broadcasted_iota(jnp.int32, (8, 128), 1)
            acc = [None] * 4
            for t in range(NT):
                q = q_s[r:r + 8, t * 128:(t + 1) * 128]
                for j in range(4):
                    k0 = HALO + r - DIL * (4 * b + j)
                    term = q * k_s[t, k0:k0 + 8, :]
                    acc[j] = term if t == 0 else acc[j] + term
            for bit in (1, 2):
                odd = (lane & bit) != 0
                acc = [jnp.where(odd, acc[j ^ bit], acc[j]) for j in range(4)]
            lg = acc[0]
            for j in range(1, 4):
                lg = lg + take(acc[j], lane ^ j)
            lg = lg * float(DH) ** -0.5
            if first and r < DIL * WIN:
                pos = r + lax.broadcasted_iota(jnp.int32, (8, 128), 0)
                lg = jnp.where(pos >= DIL * (4 * b + (lane & 3)), lg, -1e9)
            l_s[b, r:r + 8, :] = lg
            return l_s, r, 0
        return tasks(task, [(r, b) for r in range(0, U, 8) for b in range(2)], [q_s, k_s],
                     "lat_xlu", 75)

    def softmax_tasks():
        def exps(r):
            lane = lax.broadcasted_iota(jnp.int32, (16, 128), 1)
            lg = [l_s[b, r:r + 16, :] for b in range(2)]
            mx = jnp.maximum(lg[0], lg[1])
            mx = functools.reduce(jnp.maximum, [mx] + [take(mx, lane ^ j) for j in range(1, 4)])
            for b in range(2):
                e_s[b, r:r + 16, :] = jnp.exp(lg[b] - mx)
            return e_s, r, 0

        def probs(r):
            lane = lax.broadcasted_iota(jnp.int32, (8, 128), 1)
            e = [e_s[b, r:r + 8, :] for b in range(2)]
            e = {4 * b + j: take(e[b], (lane & -4) | j) for j in range(4) for b in range(2)}
            inv = 1.0 / functools.reduce(lambda p, q: p + q, e.values())
            for w in range(WIN):
                p_s[w, r:r + 8, :] = e[w] * inv
            return p_s, r, 0
        return staggered(tasks(exps, [(r,) for r in range(0, U, 16)], [l_s], "lat_xlu", 40),
                         tasks(probs, [(r,) for r in range(0, U, 8)], [], "lat_xlu", 40),
                         cfg["lag_probs"])

    def value_tasks(v_s=v_s):
        def task(r, t0):
            acc = [None] * 4
            for w in range(WIN):
                k0 = HALO + r - DIL * w
                p = p_s[w, r:r + 8, :]
                for j in range(4):
                    term = p * v_s[t0 + j, k0:k0 + 8, :]
                    acc[j] = term if w == 0 else acc[j] + term
            for j in range(4):
                o_s[r:r + 8, (t0 + j) * 128:(t0 + j + 1) * 128] = acc[j]
            return o_s, r, t0 * 128
        out = []
        for g in range(0, U // 2 + 16, 16):
            if g < U // 2:
                out += tasks(task, [(g + b + j, t0) for b in (0, U // 2) for j in (0, 8)
                                    for t0 in (0, 4)], [p_s, v_s], "lat_short", 62)
            if g:
                out += left_tasks(oa, "wo", D, lambda r, j, c: o_s[r:r + 16, c:c + 128], [o_s],
                                  rows=[g - 16])
        return out

    def set_halo(buf, src):
        buf[:, 0:HALO, :] = (jnp.zeros((NT, HALO, 128), f32) if src is None
                             else src[:, U:U + HALO, :])

    def copies():
        half = FH // 2

        def units(lo, hi):
            return [(x_hbm.at[0, lo * U:hi * U], x_s.at[lo * U:hi * U])]

        def weight(j, parts):
            n = D // 2 // parts
            return [("w%d_%d" % (j, p), [(wqkv_hbm.at[r:r + n, j * D:(j + 1) * D],
                                          raw.at[j, r:r + n]) for r in (p * n, D // 2 + p * n)])
                    for p in range(parts)]

        def rows_in(lo, hi):
            return [(win_hbm.at[r + lo:r + hi, j * half:(j + 1) * half],
                     raw.at[4 + j, r + lo:r + hi, 0:half])
                    for r in range(0, D, D // 4) for j in range(4)]
        early = share(0, NU - 2, D // 64)[1] * 16
        pairs = [("x0", units(0, 1))]
        pairs += weight(0, PARTS) + [("x1", units(1, 2))] + weight(1, PARTS) + weight(2, 2)
        pairs += [
            ("wo", [(wo_hbm, raw.at[3, 0:D])] + units(2, 3)),
            ("early", units(3, 4) + rows_in(0, early)),
            ("rest", units(4, NU) + rows_in(early, D // 4) + [(bsp_hbm, bsp_raw)]),
            ("late0", [(wsp_hbm.at[0:D, j * D:(j + 1) * D], raw.at[j, 0:D]) for j in range(2)]
             + [(wout_hbm.at[j * half:(j + 1) * half], raw.at[2 + j, 0:half]) for j in range(2)]),
            ("late1", [(wsp_hbm.at[D:S, j * D:(j + 1) * D], raw.at[4 + j, 0:D])
                       for j in range(2)])]
        return {name: [(a, b, sem.at[j]) for a, b in group]
                for j, (name, group) in enumerate(pairs)}

    def start(*names):
        for name in names:
            for args in copies()[name]:
                pltpu.make_async_copy(*args).start()

    def wait(name):
        for args in copies()[name]:
            pltpu.make_async_copy(*args).wait()

    def out_copy(u, half):
        rows = _ds(u * U + half * U // 2, U // 2, U // 2)
        return pltpu.make_async_copy(x_s.at[rows], out_hbm.at[0, rows], osem.at[2 * u + half])

    def unit(ref, u, n=U):
        return ref.at[_ds(u * n, n, n)]

    def clip(v, lo, hi):
        return min(max(v, lo), hi) if isinstance(v, int) else jnp.clip(v, lo, hi)

    def share(step, steps, total):
        count = -(-total // steps)
        return clip(step * count, 0, total - count), count

    def add_into(u):
        def store(r, c, v):
            idx = (slice(r, r + v.shape[0]), slice(c, c + v.shape[1]))
            dst = unit(x_s, u)
            dst[idx] = (dst[idx].astype(f32) + v).astype(bf16)
        return store

    def put_rows(buf):
        def store(r, c, v):
            buf[r:r + v.shape[0], c:c + 128] = v
        return store

    def put_slab(buf):
        def store(r, c, v):
            buf[c // 128, HALO + r:HALO + r + v.shape[0], :] = v
        return store

    def qkv(src, w, store):
        return matmul(src, (w, None), "qkv", D, D, store)

    def project(u):
        return matmul(oa, (wo_p, None), "wo", D, D, add_into(u), cfg["cw_wo"])

    def first_query(part):
        n = D // 4 // PARTS
        rows, cols, q = slice(part * n, (part + 1) * n), slice(part * 2 * n, (part + 1) * 2 * n), U // 4

        def gen():
            tie = yield
            for j in range(2):
                for c in range(0, D // 2, 128):
                    a = jnp.concatenate([jnp.concatenate([
                        xb[(2 + i) * q:(3 + i) * q, cols] if i == m
                        else sp_s.at[i * q:(i + 1) * q, m * D // 2:(m + 1) * D // 2][:, cols]
                        for m in range(2)], axis=1) for i in range(2)], axis=0)
                    b = jnp.concatenate(
                        [wq_p.at[1 + 3 * i][rows, c:c + 128] if i == j
                         else sa.at[i * D // 4:(i + 1) * D // 4][rows, c:c + 128]
                         for i in range(2)], axis=0)
                    res = jnp.dot(_as_bf16(a), _as_bf16(tie(b)), preferred_element_type=f32)
                    idx = (slice(0, U), slice(j * D // 2 + c, j * D // 2 + c + 128))
                    o_s[idx] = o_s[idx] + res if part else res
                    tie = yield res
        return NT, U // 16 * 4 * 4 * n // 128, gen()

    def arriving(main, j, buf, parts, first=0):
        step = main[0] // (len(parts) + first)
        sides = []
        for i, (part, of) in enumerate(parts, first):
            sides += [([(functools.partial(wait, "w%d_%d" % (j, part)), [], 0, 1)],
                       max(0, i * step - 1), i * step),
                      (prep_qkv(j, buf, part, of), i * step, (i + 1) * step - 2)]
        return sides

    def first_attention():
        wait("x0")
        make_zero()
        stats, load, _ = norm_tasks(x_s, unit(x_s, 0), st0)

        def keeping(r, j, c):
            v = load(r, c)
            if r // (U // 2) != j:
                sp_s[r // 2:r // 2 + 8, c:c + 128] = _pack(v)
            return v
        run(stats + left_tasks(xb, "qkv", D, keeping, [x_s]))
        set_halo(kv_s, None)
        wait("w0_0")
        run(prep_qkv(0, wq_p, 0, PARTS, sa))
        for part in range(1, PARTS):
            wait("w0_%d" % part)
            overlap(first_query(part - 1), (prep_qkv(0, wq_p, part, PARTS, sa), 0, NT - cfg["fq"]))
        wait("x1")
        overlap(first_query(PARTS - 1), (norm_x(1, xa), 0, NT - cfg["fq"]))
        main = qkv(xa, wq_p, put_rows(q_s))
        overlap(main, *arriving(main, 1, wk_p, [(p, PARTS) for p in range(PARTS)]))
        main = qkv(xb, wk_p, put_slab(kv_s))
        overlap(main, *arriving(main, 2, wv_p, [(0, 2)], 1))
        logits, soft = logit_tasks(False), softmax_tasks()
        wait("w2_1")
        set_halo(k_s, kv_s)
        overlap(qkv(xa, wk_p, put_slab(k_s)), prep_qkv(2, wv_p, 1, 2) + logit_tasks(True, o_s, kv_s))
        wait("wo")
        prep = prep_wo()
        overlap(qkv(xb, wv_p, put_slab(kv_s)), soft, prep)
        set_halo(v_s, kv_s)
        overlap(qkv(xa, wv_p, put_slab(v_s)), value_tasks(kv_s), logits[:cfg["f_log"]])
        overlap(project(0), (logits[cfg["f_log"]:], 0, cfg["f_end"]), norm_x(2, xa))

    def step_attention(u):
        if cfg["part"] != "s1":
            @pl.when(u == 3)
            def _():
                wait("rest")
        begin, count = share(u - 2, NU - 2, _Split(D, cfg["win"]).width // 16)
        prep = (prep_win(wz2_p, Z2_COLS, begin, count)
                + prep_win(wz1_p, Z1_COLS, begin, count))
        cut = len(prep) * cfg["cut_prep"] // 8
        g = clip(u - 2, 0, U // 64 - 1) * 16
        head = norm_h(0, z_s, rows=[g + b for b in range(0, U, 64)]) + left_h(z_s, rows=[g])
        logits = logit_tasks(False)
        set_halo(k_s, k_s)
        overlap(qkv(xa, wq_p, put_rows(q_s)), softmax_tasks(), prep[:cut])
        overlap(qkv(xa, wk_p, put_slab(k_s)), value_tasks())
        set_halo(v_s, v_s)
        overlap(qkv(xa, wv_p, put_slab(v_s)), logits, head)
        overlap(project(u - 1), norm_x(clip(u + 1, 0, NU - 1), xa), prep[cut:])

    def spatial_left(u, rows=range(0, U // 4, 16)):
        per = D // U

        def regroup(r, m):
            lane = lax.broadcasted_iota(jnp.int32, (8, 128), 1)
            col = 2 * U * m
            w = pltpu.bitcast(raw.at[u // per * 4 + col // D][
                _ds(u % per * U + r, 16, 16), col % D:col % D + 2 * U], u32)
            for a in range(2):
                one, two = w[:, a * 128:(a + 1) * 128], w[:, U + a * 128:U + (a + 1) * 128]
                mid = pltpu.roll(jnp.where(lane < 64, two, one), 64, 1)
                for j, v in ((2 * a, jnp.where(lane < 64, one, mid)),
                             (2 * a + 1, jnp.where(lane < 64, mid, two))):
                    sp_s[_ds(r // 2, 8, 8), j * 512 + m * 128:j * 512 + (m + 1) * 128] = v
            return sp_s, r // 2, m * 128
        return tasks(regroup, [(b + r, m) for r in rows for b in range(0, U, U // 4)
                               for m in range(NU // 2)], [raw], "lat_xlu", 18) + left_tasks(
            sa, "sp", S, lambda r, j, c: _unpack(sp_s[_ds(r // 2, 8, 8), c:c + 128]), [sp_s],
            rows=rows)

    def input_product(u, w, cols):
        def store(r, c, v):
            n = v.shape[0]
            if c >= FH:
                z_s[r:r + n, c - FH:c - FH + 128] = _gelu(v)
            else:
                unit(z1_s, u, U // 2)[r // 2:(r + n) // 2, c:c + 128] = _pack(_gelu(v))
        return matmul(ha, (w, None), "win", D, cols, store)

    def norm_z2(u):
        h = U // 4
        stats, _, write = norm_tasks(z_s, z_s, st0, EPS * GAIN * GAIN, 1.0 / GAIN)
        return stats + write(zn_s), right_tasks(
            (z2n_p, z2n_r), "sp", FH, [(u * (h // 2) + r // 2, r) for r in range(0, h, 16)],
            lambda b, r, c: zn_s[b * h + r:b * h + r + 16, c:c + 128], [zn_s])

    def last_attention():
        main = input_product(0, wz2_p, Z2_COLS)
        overlap(main, (softmax_tasks(), 0, cfg["soft_end"]),
                (value_tasks(), cfg["soft_end"], main[0]), spatial_left(0, [0]))
        overlap(project(NU - 1), prep_bias() + spatial_left(0, [16, 32]) + norm_h(1, q_s))

    def step_input(u):
        norm, factors = norm_z2(u - 1)
        cut, early = len(factors) * cfg["z_cut"] // 8, cfg["z_left"]
        main = input_product(u - 1, wz1_p, Z1_COLS)
        last = main[0] - 49
        overlap(main, (norm + factors[:cut], 0, last + cfg["z_over"]),
                *[(left_h(q_s, outer=[o]), last + 7 * j + 6, last + 7 * j + 13)
                  for j, o in enumerate(ORDER[:early])])
        prep = (prep_wout(*share(u - 1, NU - 1, _Split(FH, cfg["out"]).width // 16))
                + prep_wout_rest(*share(u - 1, NU - 1, 8)))
        main = input_product(u, wz2_p, Z2_COLS)
        busy = 7 * (7 - early)
        overlap(main, (sum((left_h(q_s, outer=[o]) for o in ORDER[early:]), []), 0, busy),
                (norm_h(clip(u + 1, 0, NU - 1), q_s), busy, main[0]),
                (factors[cut:] + prep, busy, main[0]))

    def last_input():
        overlap(input_product(NU - 1, wz1_p, Z1_COLS), sum(norm_z2(NU - 1), []),
                spatial_left(0, [48]))

    def step_output(u):
        bt, z1t = unit(bias_s, u), unit(z1_s, u, U // 2)

        def put_y(r, c, g):
            n = g.shape[0]
            z_s[r:r + n, c:c + 128] = _unpack(z1t[r // 2:(r + n) // 2, c:c + 128]) * (
                g + bt[r:r + n, :])

        def gated(**kw):
            return left_tasks(ya, "out", FH, lambda r, j, c: z_s[r:r + 16, c:c + 128], [z_s], **kw)
        overlap(matmul(sa, (z2n_p, z2n_r), "sp", S, FH, put_y),
                *[(gated(cols=[128 * j], rest=False), 49 * j + 49, 49 * j + 49 + 20)
                  for j in range(3)])
        run(gated(cols=[]))
        overlap(matmul(ya, (wout_p, wout_r), "out", FH, D, add_into(u), 256),
                spatial_left(clip(u + 1, 0, NU - 1)),
                ([(out_copy(u, 1).start, [], 0, 1)], 36, 37))
        out_copy(u, 0).start()

    def make_zero():
        bits = pltpu.bitcast(x_s[0:16, 0:128], jnp.int32)
        zero.append(bits[0, 0] ^ pltpu.roll(bits, 1, 1)[0, 1])

    def keep(j):
        v = None
        for b in (wq_p, wk_p, wv_p, wo_p, wz1_p, wz2_p, wout_p, wout_r, z2n_p,
                  z2n_r, z1_s, bias_s, xa, xb, oa, ha, sa, ya, q_s, o_s, k_s, v_s, kv_s, p_s, l_s, e_s,
                  z_s, zn_s, sp_s, *st0, *st1, tmp_s):
            v = done(b, 0, 0) if v is None else v | done(b, 0, 0)
        x_s[0:16, 0:128] = _as_bf16(v)
        c = pltpu.make_async_copy(x_s.at[0:16, 0:128], out_hbm.at[0, 0:16, 0:128], sem.at[0])
        c.start()
        c.wait()

    if cfg["part"] in ("s1", "s2", "s3", "mid"):
        make_zero()
        if cfg["part"] == "mid":
            last_attention()
            last_input()
        else:
            pl.loop(1, NU)({"s1": step_attention, "s2": step_input, "s3": step_output}[cfg["part"]])
        if cfg["part"] == "s3":
            for u in range(1, NU):
                out_copy(u, 0).wait()
                out_copy(u, 1).wait()
        pl.loop(0, 2)(keep)
        return
    import contextlib
    scope = jax.named_scope if cfg["prof"] else (lambda n: contextlib.nullcontext())
    start(*list(copies())[:-2])
    with scope("p_first"):
        first_attention()
    with scope("p_rest0"):
        wait("early")
    if cfg["part"] == "first":
        wait("rest")
        pl.loop(0, 2)(keep)
        return
    start("late0")

    def sc(name, fn):
        def g(u):
            with scope(name):
                fn(u)
        return g
    with scope("p_loop1"):
        pl.loop(2, NU)(sc("p_it1", step_attention))
    start("late1")
    with scope("p_rest2"):
        wait("late0")
    with scope("p_mid"):
        last_attention()
    with scope("p_loop2"):
        pl.loop(1, NU)(sc("p_it2", step_input))
    with scope("p_mid2"):
        last_input()
    wait("late1")
    with scope("p_loop3"):
        pl.loop(0, NU)(sc("p_it3", step_output))
    with scope("p_out"):
        for u in range(NU):
            out_copy(u, 0).wait()
            out_copy(u, 1).wait()


def build(cfg, interpret=False, name="fused_block"):
    vm = pltpu.VMEM

    def right(key, k, n):
        ks, ns = _Split(k, cfg[key]), _Split(n, cfg[key])
        main = vm((7 ** ks.level, ks.width // 2, ns.width), u32)
        if ns.rest:
            return [main, vm((21, ks.width // 2, 128), u32)]
        if ks.rest:
            return [main, vm((14, 64, ns.width), u32)]
        return [main]

    def left(key, k):
        ks = _Split(k, cfg[key])
        return vm((7 ** ks.level * U // ks.parts // 2, ks.width + ks.rest), u32)
    scratch = [
        vm((S + 16, D), bf16),
        vm((8, D + 16, D), bf16),
        vm((S,), bf16),
        *right("qkv", D, D) * 3, *right("wo", D, D),
        vm((49, D // 8, 384), u32), vm((49, D // 8, 512), u32), *right("out", FH, D), *right("sp", S, FH),
        vm((S // 2, FH), u32),
        vm((S, 128), f32),
        left("qkv", D), left("qkv", D), left("wo", D), left("win", D), left("sp", S),
        left("out", FH),
        *[vm((U + 8, D), f32)] * 2,
        *[vm((NT, HALO + U + 8, 128), f32)] * 3,
        vm((WIN, U + 8, 128), f32),
        *[vm((2, U + 8, 128), f32)] * 2,
        *[vm((U + 8, FH), f32)] * 2,
        vm((U // 2 + 8, S), u32),
        *[vm((3, U + 8, 128), f32)] * 2,
        *[vm((U, 128), f32)] * 2,
        vm((25 * U // 4, 256), f32),
        pltpu.SemaphoreType.DMA((9 + 2 * PARTS,)),
        pltpu.SemaphoreType.DMA((2 * NU,)),
    ]
    hbm = pl.BlockSpec(memory_space=pl.ANY)
    return pl.pallas_call(
        functools.partial(_kernel, cfg),
        out_shape=jax.ShapeDtypeStruct((1, S, D), bf16),
        in_specs=[hbm] * 7,
        out_specs=hbm,
        scratch_shapes=scratch,
        compiler_params=pltpu.CompilerParams(vmem_limit_bytes=127 * 1024 * 1024,
                                             flags=cfg["flags"]),
        interpret=interpret,
        name=name,
    )


@jax.jit
def pallas_sequential_preLN__sliding_local_dilated__mixer_gmlp__prompt_kernel(
    A_x: jax.Array,
    A_wqkv: jax.Array,
    A_wo: jax.Array,
    B_x: jax.Array,
    B_w_in: jax.Array,
    B_w_sp: jax.Array,
    B_b_sp: jax.Array,
    B_w_out: jax.Array,
):
    del B_x
    return build(CFG)(A_x, A_wqkv, A_wo, B_w_in, B_w_sp, B_b_sp, B_w_out)
```

```python
import functools

import jax
import jax.numpy as jnp
import numpy as np
from jax import lax
from jax.experimental import pallas as pl
from jax.experimental.pallas import tpu as pltpu

S = 2048
D = 1024
FH = 1792
DH = 32
WIN = 8
DIL = 2
HALO = 16
U = 256
NU = S // U
NT = D // 128
PARTS = 4
EPS = 1e-5

f32 = jnp.float32
bf16 = jnp.bfloat16
u32 = jnp.uint32

CFG = dict(part="all", flags=None, qkv=1, wo=2, win=2, sp=2, out=2, slot=32,
           lat_short=320, lat_xlu=512, tail=0, regs=('win', 'sp', 'wo'), cw_wo=128, cut_prep=7, z_over=21, z_left=3, z_cut=3, fq=2, f_log=0, f_cut=5, gap=200, lag_rstd=6, lag_probs=2, peel=True, wq_parts=4, depth=6, soft_end=90, prof=False)

ORDER = (0, 3, 1, 2, 5, 4, 6)
REST = (3, 1, 2, 4)


def _pack(v):
    return pltpu.bitcast(v.astype(bf16), u32)


def _as_bf16(v):
    return pltpu.bitcast(v, bf16)


def _unpack(v):
    return pltpu.bitcast(v, bf16).astype(f32)


_C = float(np.sqrt(2.0 / np.pi))
ALPHA = float((_C * 0.044715) ** (1.0 / 3.0))
GAIN = 2.0 * ALPHA


def _gelu(v):
    return v * (1.0 + jnp.tanh(v * (_C / ALPHA + v * v)))


LEFT = (((1, 0, 0), (1, 1, 1)), ((1, 1, 0), (1, 1, 1)), ((1, 0, 0),), ((1, 1, 1),),
        ((1, 0, 0), (1, 0, 1)), ((1, 1, 0), (-1, 0, 0)), ((1, 0, 1), (-1, 1, 1)))
RIGHT = (((1, 0, 0), (1, 1, 1)), ((1, 0, 0),), ((1, 0, 1), (-1, 1, 1)), ((1, 1, 0), (-1, 0, 0)),
         ((1, 1, 1),), ((1, 0, 0), (1, 0, 1)), ((1, 1, 0), (1, 1, 1)))


def _factor(terms, get):
    v = get(*terms[0][1:])
    for sign, i, j in terms[1:]:
        v = v + get(i, j) if sign > 0 else v - get(i, j)
    return v


def _factors(forms, get):
    blk = {(i, j): get(i, j) for i in range(2) for j in range(2)}
    return [_factor(terms, lambda i, j: blk[i, j]) for terms in forms]


class _Blocks:
    level, parts, rest = 2, 4, 0

    def __init__(self, chunks):
        self.chunks, self.width = chunks, 128 * len(chunks)

    def col(self, j, c):
        return self.chunks[c // 128][j]


Z1_COLS = _Blocks([[c + s for s in (0, 384, 896, 1280)] for c in (0, 128, 256)])
Z2_COLS = _Blocks([[FH + c for c in chunk] for chunk in Z1_COLS.chunks]
                  + [[FH + 768, FH + 1664, 768, 1664]])


class _Held:
    def __setitem__(self, _, v):
        self.v = v

    def __getitem__(self, _):
        return self.v


def _combiner(tmp, put):
    t1, t2, t3, t4, t5 = tmp

    def feed(i, m):
        if i == 0:
            t1[...] = m
        elif i == 3:
            t4[...] = m
        elif i == 1:
            t2[...] = m
            put(1, 0, m + t4[...])
        elif i == 2:
            t3[...] = m
        elif i == 5:
            put(1, 1, (t1[...] - t2[...] + t3[...]) + m)
        elif i == 4:
            t5[...] = m
            put(0, 1, m + t3[...])
        else:
            put(0, 0, (t1[...] + t4[...] - t5[...]) + m)
    return feed


class _Split:
    def __init__(self, n, level):
        self.level, self.parts = level, 1 << level
        self.width = n // self.parts // 128 * 128
        self.rest = n // 2 - 2 * self.width if level == 2 else 0
        self.half = n // 2

    def start(self, j):
        if self.level == 1:
            return j * self.half
        return (j // 2) * self.half + (j % 2) * self.width

    def col(self, j, c):
        return self.start(j) + c

    def rest_start(self, h):
        return h * self.half + 2 * self.width


def _pair_transpose(v):
    sub = lax.broadcasted_iota(jnp.int32, v[0].shape, 0)
    v = list(v)
    for b in range(2):
        s = 1 << b
        m = (sub & (2 * s)) != 0
        nv = list(v)
        for j in range(4):
            if j & s:
                continue
            lo, hi = v[j], v[j + s]
            nv[j] = jnp.where(m, pltpu.roll(hi, 2 * s, 0), lo)
            nv[j + s] = jnp.where(m, hi, pltpu.roll(lo, 8 - 2 * s, 0))
        v = nv
    return v


def _ds(start, size, align):
    return pl.ds(start if isinstance(start, int) else pl.multiple_of(start, align), size)


def _kernel(cfg,
            x_hbm, wqkv_hbm, wo_hbm, win_hbm, wsp_hbm, bsp_hbm, wout_hbm, out_hbm,
            x_s, raw, bsp_raw,
            wq_p, wk_p, wv_p, wo_p, wz1_p, wz2_p, wout_p, wout_r, z2n_p, z2n_r,
            z1_s, bias_s, xa, xb, oa, ha, sa, ya,
            q_s, o_s, k_s, v_s, kv_s, p_s, l_s, e_s, z_s, zn_s, sp_s, st0_s, st1_s, inv0_s, inv1_s, tmp_s,
            sem, osem):
    st0, st1 = (st0_s, inv0_s), (st1_s, inv1_s)
    zero = []

    def spot(ref, row, col):
        n = 8 * (4 // ref.dtype.itemsize)
        ref = ref if len(ref.shape) == 2 else ref.at[zero[0]]
        return ref.at[_ds(row + zero[0] * n, n, n), _ds(col + zero[0] * 128, 128, 128)]

    def gate(ref, v):
        n = 8 * (4 // ref.dtype.itemsize)
        spot(ref, ref.shape[-2] - n, 0)[0:8, :] = v.astype(ref.dtype)

    def done(ref, row, col):
        v = spot(ref, row, col)[...]
        return v if v.dtype == u32 else pltpu.bitcast(v, u32)

    def tied(toks):
        def tie(b):
            if not toks:
                return b
            tok = functools.reduce(lambda p, q: p | q, toks)
            tok = jnp.concatenate([tok] * (b.shape[1] // 128), axis=1)
            always = lax.broadcasted_iota(jnp.int32, tok.shape, 0) >= zero[0]
            parts = []
            for r in range(0, b.shape[0], 64):
                parts += [b[r:r + 56], jnp.where(always, b[r + 56:r + 64], tok)]
            return jnp.concatenate(parts, axis=0)
        return tie

    def overlap(main, *sides):
        n, cyc, gen = main
        per = max(1, cyc // cfg["slot"])
        plan = [[] for _ in range(n * per)]
        for side in sides:
            if not isinstance(side, tuple):
                side = (side, 0, n)
            todo, first, last = side
            if todo and last == n:
                last -= (todo[-1][2] + cfg["tail"]) / cyc
            span = max(1, int((last - first) * per))
            total, spent = sum(t[3] for t in todo), 0
            for t in todo:
                plan[int(first * per) + spent * span // total].append(t)
                spent += t[3]
        next(gen)
        due = [[] for _ in range(n)]
        for i, todo in enumerate(plan):
            if i % per == 0:
                res = gen.send(tied([tok for _, tok in due[i // per]]))
            gated = []
            for _, refs, _, _ in todo:
                gated += [r for r in refs if not any(r is g for g in gated)]
            row = res.shape[0] * (i % per) // per
            for r in gated:
                gate(r, res[row:row + 8, 0:128])
            for fn, _, lat, _ in todo:
                where = fn()
                j = -(-(i * cyc // per + lat) // cyc)
                if where is not None and j < n:
                    due[j] = [d for d in due[j] if d[0] is not where[0]]
                    due[j].append((where[0], done(*where)))

    def tasks(fn, args, refs, lat, cost):
        return [(functools.partial(fn, *a), refs, cfg[lat], cost) for a in args]

    def staggered(early, late, lag):
        per = len(early) / len(late)
        order = [(j, t) for j, t in enumerate(early)]
        order += [((j + 1) * per + lag - 0.5, t) for j, t in enumerate(late)]
        return [t for _, t in sorted(order, key=lambda p: p[0])]

    gap = [(lambda: None, [], 0, cfg["gap"])]

    def run(todo):
        for t in todo:
            t[0]()

    def left_tasks(ref, key, k, load, refs, rows=None, cols=None, outer=None, rest=True):
        ks = _Split(k, cfg[key])
        h = U // ks.parts

        def put(n, r, c, v):
            ref[_ds(n * h // 2 + r // 2, 8, 8), c:c + 128] = _pack(v)

        def main(r, c, o):
            def get(i, j):
                if ks.level == 1:
                    return load(i * h + r, j, ks.start(j) + c)
                return _factor(LEFT[o], lambda a, b: load((2 * a + i) * h + r, 2 * b + j,
                                                          ks.start(2 * b + j) + c))
            for n, v in enumerate(_factors(LEFT, get)):
                put(7 * o + n, r, c, v)
            return ref, 7 * o * h // 2 + r // 2, c

        def other(r, i):
            vals = _factors(LEFT, lambda a, b: load((2 * a + i) * h + r, None, ks.rest_start(b)))
            for o, v in enumerate(vals):
                put(7 * o + 6 - i, r, ks.width, v)
            return ref, (6 - i) * h // 2 + r // 2, ks.width
        out = []
        for r in range(0, h, 16) if rows is None else rows:
            out += tasks(main, [(r, c, o)
                                for c in (range(0, ks.width, 128) if cols is None else cols)
                                for o in (range(7 ** (ks.level - 1)) if outer is None else outer)],
                         refs, "lat_short", 30)
            out += tasks(other, [(r, 0), (r, 1)] if ks.rest and rest else [], refs, "lat_short", 30)
        return out

    def right_tasks(bufs, key, n, rows, load, refs, lat="lat_short"):
        main_p, rest_p = bufs
        ns = n if isinstance(n, _Blocks) else _Split(n, cfg[key])

        def main(prow, r, c, o):
            def get(i, j):
                if ns.level == 1:
                    return load(i, r, ns.start(j) + c)
                return _factor(RIGHT[o], lambda a, b: load(2 * a + i, r, ns.col(2 * b + j, c)))
            for m, v in enumerate(_factors(RIGHT, get)):
                main_p.at[7 * o + m][_ds(prow, 8, 8), c:c + 128] = _pack(v)
            return main_p, prow, c

        def rest(prow, r, o):
            top, bot = [_factor(RIGHT[o], lambda a, b: load(2 * a + i, r, ns.rest_start(b)))
                        for i in range(2)]
            for m, v in enumerate((top, bot, top - bot)):
                rest_p.at[3 * o + m][_ds(prow, 8, 8), :] = _pack(v)
            return rest_p, prow, 0
        out = []
        for prow, r in rows:
            out += tasks(main, [(prow, r, c, o) for c in range(0, ns.width, 128)
                                for o in range(7 ** (ns.level - 1))], refs, lat, 32)
            out += tasks(rest, [(prow, r, o) for o in range(7)] if ns.rest else [], refs,
                         "lat_short", 16)
        return out

    def matmul(ref, bufs, key, k, n, store, cw=128):
        main_p, rest_p = bufs
        ks = _Split(k, cfg[key])
        ns = n if isinstance(n, _Blocks) else _Split(n, cfg[key])
        h = U // ks.parts

        def lhs(m, lo, hi):
            return _as_bf16(ref[m * h // 2:(m + 1) * h // 2, lo:hi])

        def dot(a, b):
            return jnp.dot(a, _as_bf16(b), preferred_element_type=f32)

        def temps(slot):
            return [tmp_s.at[(5 * slot + j) * h:(5 * slot + j + 1) * h, 0:cw] for j in range(5)]

        def gen1():
            tie = yield
            for c in range(0, ns.width, cw):
                feed = _combiner(temps(0), lambda i, j, v: store(i * h, ns.start(j) + c, v))
                for m in ORDER:
                    res = dot(lhs(m, 0, ks.width), tie(main_p.at[m][:, c:c + cw]))
                    feed(m, res)
                    tie = yield res

        def inner_temps():
            return [_Held() for _ in range(5)] if key in cfg["regs"] else temps(4)

        def chunk(c, tie):
            def put(i, j):
                return lambda a, b, v: store((2 * a + i) * h, ns.col(2 * b + j, c), v)
            outer = {(i, j): _combiner(temps(2 * i + j), put(i, j))
                     for i in range(2) for j in range(2)}
            for o in ORDER:
                def extra(i, j, v):
                    if ks.rest and i != j:
                        v = v + dot(lhs(7 * o + 6 - i, ks.width, ks.width + 128),
                                    rest_p.at[2 * o + j][:, c:c + cw])
                    outer[i, j](o, v)
                feed = _combiner(inner_temps(), extra)
                for m in ORDER:
                    b = main_p.at[7 * o + m][:, c:c + cw]
                    hi = ks.width
                    if ks.rest and m >= 5:
                        b = jnp.concatenate([b, rest_p.at[2 * o + 6 - m][:, c:c + cw]], axis=0)
                        hi += 128
                    res = dot(lhs(7 * o + m, 0, hi), tie(b))
                    feed(m, res)
                    tie = yield res
            return tie

        def rest_chunk(tie):
            def put(i):
                return lambda a, b, v: store((2 * a + i) * h, ns.rest_start(b), v)
            outer = [_combiner(temps(i), put(i)) for i in range(2)]
            for o in ORDER:
                for i, (m0, b0), (m1, b1) in ((1, (3, 2), (1, 0)), (0, (2, 2), (4, 1))):
                    first = dot(lhs(7 * o + m0, 0, ks.width), tie(rest_p.at[3 * o + b0][...]))
                    tie = yield first
                    res = dot(lhs(7 * o + m1, 0, ks.width), tie(rest_p.at[3 * o + b1][...]))
                    outer[i](o, res - first if i else res + first)
                    tie = yield res
            return tie

        def gen2():
            tie = yield
            for c in range(0, ns.width, cw):
                tie = yield from chunk(c, tie)
            if ns.rest:
                tie = yield from rest_chunk(tie)
        cyc = h // 16 * 4 * (ks.width // 128) * (cw // 128)
        if ks.level == 1:
            return 7 * (ns.width // cw), cyc, gen1()
        return 49 * (ns.width // cw) + (28 if ns.rest else 0), cyc, gen2()

    def staged(i):
        return (z_s, zn_s)[i].at[0:D // 4, 0:D]

    def mix_staged(buf, key, shift, rows, plain=None):
        h = _Split(D, cfg[key]).width // 2

        def load(i, r, c):
            r += i * h
            i, r, tile = r // (D // 4), r % (D // 4), c // 128
            v = pltpu.bitcast(staged(i)[r:r + 8, c:c + 128], u32)
            v = pltpu.roll(v, 128 - 4 * tile, 1) if shift and tile else v
            if plain is not None and i != c // (D // 2):
                plain[i * D // 4 + r:i * D // 4 + r + 8, c % (D // 2):c % (D // 2) + 128] = v
            return _unpack(v)
        return right_tasks((buf, None), key, D, [(r, r) for r in rows], load, [z_s, zn_s],
                           "lat_xlu" if shift else "lat_short")

    def prep_qkv(j, buf, part, parts, plain=None):
        def task(i, r):
            w = pltpu.bitcast(raw.at[j][i * D // 2 + r:i * D // 2 + r + 16, :], u32)
            lane = lax.broadcasted_iota(jnp.int32, (8, 128), 1)
            w = [w[:, t * 128:(t + 1) * 128] for t in range(NT)]
            w = [pltpu.roll(v, 4 * t, 1) if t else v for t, v in enumerate(w)]
            w = [w[(-t) % NT] for t in range(NT)]
            for b in range(3):
                m = (lane & (4 << b)) != 0
                w = [jnp.where(m, w[(t - (1 << b)) % NT], w[t]) for t in range(NT)]
            for t in range(NT):
                staged(i)[r // 2:r // 2 + 8, t * 128:(t + 1) * 128] = pltpu.bitcast(w[t], f32)
            return (z_s, zn_s)[i], r // 2, 0
        rows = range(part * D // 2 // parts, (part + 1) * D // 2 // parts, 16)
        return (tasks(task, [(i, r) for r in rows for i in range(2)], [raw], "lat_xlu", 45) + gap
                + mix_staged(buf, "qkv", True, [r // 2 for r in rows], plain))

    def prep_wo():
        def task(d4, t2, hh, c):
            src = [((t2 * 4 + j) * 4 + hh) * 32 + d4 * 16 for j in range(4)]
            v = _pair_transpose([pltpu.bitcast(raw.at[3][s:s + 16, c:c + 256], u32) for s in src])
            for j in range(4):
                r = ((j * 4 + hh) * 32 + t2 * 16) // 2
                staged(d4)[r:r + 8, c:c + 256] = pltpu.bitcast(v[j], f32)
            return (z_s, zn_s)[d4], r, c
        return tasks(task, [(d4, t2, hh, c) for d4 in range(2) for t2 in range(2)
                            for hh in range(4) for c in range(0, D, 256)],
                     [raw], "lat_short", 40) + gap + mix_staged(
            wo_p, "wo", False, range(0, _Split(D, cfg["wo"]).width // 2, 8))

    def prep_win(buf, cols, first, count):
        ks = _Split(D, cfg["win"])

        def load(i, r, c):
            return raw.at[4 + c // (FH // 2)][
                _ds(ks.start(i) + r, 16, 16), c % (FH // 2):c % (FH // 2) + 128].astype(f32)
        rows = [((first + g) * 8, (first + g) * 16) for g in range(count)]
        return right_tasks((buf, None), "win", cols, rows, load, [raw])

    def prep_wout(first, count):
        ks = _Split(FH, cfg["out"])

        def load(i, r, c):
            row = ks.start(i)
            return raw.at[2 + row // (FH // 2)][
                _ds(row % (FH // 2) + r, 16, 16), c:c + 128].astype(f32)
        rows = [((first + g) * 8, (first + g) * 16) for g in range(count)]
        return right_tasks((wout_p, None), "out", D, rows, load, [raw])

    def prep_wout_rest(first, count):
        ks, ns = _Split(FH, cfg["out"]), _Split(D, cfg["out"])

        def task(g, j, c):
            def get(a, b):
                col = ns.start(2 * b + j) + c
                return raw.at[2 + a][_ds(2 * ks.width + (first + g) * 16, 16, 16),
                                     col:col + 128].astype(f32)
            for o, v in enumerate(_factors(RIGHT, get)):
                wout_r.at[2 * o + j][_ds((first + g) * 8, 8, 8), c:c + 128] = _pack(v)
            return wout_r, (first + g) * 8, c
        if not ks.rest:
            return []
        return tasks(task, [(g, j, c) for g in range(count) for j in range(2)
                            for c in range(0, ns.width, 128)], [raw], "lat_short", 28)

    def prep_bias():
        def task(j):
            b = bsp_raw[...].astype(f32).reshape(1, S) * (1.0 / GAIN)
            bias_s[j * 128:(j + 1) * 128, :] = jnp.broadcast_to(
                b[:, j * 128:(j + 1) * 128], (128, 128)).T
            return bias_s, j * 128, 0
        return tasks(task, [(j,) for j in range(S // 128)], [], "lat_xlu", 50)

    def norm_tasks(base, src, st, eps=EPS, scale=None, rows=range(0, U, 16)):
        n = src.shape[1]
        st, inv = st

        def shift(r):
            v = src[_ds(r, 16, 16), 0:128].astype(f32)
            st.at[0][_ds(r, 16, 16), :] = jnp.broadcast_to(v[:, 0:1], (16, 128))
            return st, r, 0

        def stats(r):
            sh = st.at[0][_ds(r, 8, 8), :]
            s1 = s2 = None
            for c in range(0, n, 256):
                v = src[_ds(r, 8, 8), c:c + 256].astype(f32)
                for d in (v[:, :128] - sh, v[:, 128:] - sh):
                    s1 = d if s1 is None else s1 + d
                    s2 = d * d if s2 is None else s2 + d * d
            m = jnp.sum(s1, axis=-1, keepdims=True) * (1.0 / n)
            var = jnp.sum(s2, axis=-1, keepdims=True) * (1.0 / n) - m * m
            st.at[1][_ds(r, 8, 8), :] = sh + m
            st.at[2][_ds(r, 8, 8), :] = jnp.broadcast_to(jnp.maximum(var, 0.0) + eps, (8, 128))
            return st, r, 0

        def rstd(r):
            v = lax.rsqrt(st.at[2][_ds(r, 16, 16), :])
            inv[_ds(r, 16, 16), :] = v if scale is None else v * scale
            return inv, r, 0

        def load(r, c, h=16, w=128):
            v = src[_ds(r, h, h), c:c + w].astype(f32)
            mean, mul = [jnp.concatenate([t[_ds(r, h, h), :]] * (w // 128), axis=1)
                         for t in (st.at[1], inv)]
            return (v - mean) * mul

        def write(dst):
            def task(r, c, w):
                dst[_ds(r, 8, 8), c:c + w] = load(r, c, 8, w)
                return dst, r, c
            return tasks(task, [(r + j, c, min(1024, n - c)) for r in rows for j in (0, 8)
                                for c in range(0, n, 1024)], [base], "lat_short", 22)
        out = tasks(shift, [(r,) for r in rows], [base], "lat_xlu", 10)
        out += staggered(tasks(stats, [(r + j,) for r in rows for j in (0, 8)], [base], "lat_xlu",
                               n // 28 + 8),
                         tasks(rstd, [(r,) for r in rows], [], "lat_short", 22), cfg["lag_rstd"])
        return out, load, write

    def norm_x(u, buf):
        out, load, _ = norm_tasks(x_s, unit(x_s, u), st0)
        return out + left_tasks(buf, "qkv", D, lambda r, j, c: load(r, c), [x_s])

    def norm_h(u, spare, **kw):
        out, _, write = norm_tasks(x_s, unit(x_s, u), st1, scale=ALPHA, **kw)
        return out + write(spare)

    def left_h(spare, **kw):
        return left_tasks(ha, "win", D, lambda r, j, c: spare[_ds(r, 16, 16), c:c + 128], [spare],
                          **kw)

    def take(v, idx):
        return jnp.take_along_axis(v, idx, axis=1)

    def logit_tasks(first, q_s=q_s, k_s=k_s):
        def task(r, b):
            lane = lax.broadcasted_iota(jnp.int32, (8, 128), 1)
            acc = [None] * 4
            for t in range(NT):
                q = q_s[r:r + 8, t * 128:(t + 1) * 128]
                for j in range(4):
                    k0 = HALO + r - DIL * (4 * b + j)
                    term = q * k_s[t, k0:k0 + 8, :]
                    acc[j] = term if t == 0 else acc[j] + term
            for bit in (1, 2):
                odd = (lane & bit) != 0
                acc = [jnp.where(odd, acc[j ^ bit], acc[j]) for j in range(4)]
            lg = acc[0]
            for j in range(1, 4):
                lg = lg + take(acc[j], lane ^ j)
            lg = lg * float(DH) ** -0.5
            if first and r < DIL * WIN:
                pos = r + lax.broadcasted_iota(jnp.int32, (8, 128), 0)
                lg = jnp.where(pos >= DIL * (4 * b + (lane & 3)), lg, -1e9)
            l_s[b, r:r + 8, :] = lg
            return l_s, r, 0
        return tasks(task, [(r, b) for r in range(0, U, 8) for b in range(2)], [q_s, k_s],
                     "lat_xlu", 75)

    def softmax_tasks():
        def exps(r):
            lane = lax.broadcasted_iota(jnp.int32, (16, 128), 1)
            lg = [l_s[b, r:r + 16, :] for b in range(2)]
            mx = jnp.maximum(lg[0], lg[1])
            mx = functools.reduce(jnp.maximum, [mx] + [take(mx, lane ^ j) for j in range(1, 4)])
            for b in range(2):
                e_s[b, r:r + 16, :] = jnp.exp(lg[b] - mx)
            return e_s, r, 0

        def probs(r):
            lane = lax.broadcasted_iota(jnp.int32, (8, 128), 1)
            e = [e_s[b, r:r + 8, :] for b in range(2)]
            e = {4 * b + j: take(e[b], (lane & -4) | j) for j in range(4) for b in range(2)}
            inv = 1.0 / functools.reduce(lambda p, q: p + q, e.values())
            for w in range(WIN):
                p_s[w, r:r + 8, :] = e[w] * inv
            return p_s, r, 0
        return staggered(tasks(exps, [(r,) for r in range(0, U, 16)], [l_s], "lat_xlu", 40),
                         tasks(probs, [(r,) for r in range(0, U, 8)], [], "lat_xlu", 40),
                         cfg["lag_probs"])

    def value_tasks(v_s=v_s):
        def task(r, t0):
            acc = [None] * 4
            for w in range(WIN):
                k0 = HALO + r - DIL * w
                p = p_s[w, r:r + 8, :]
                for j in range(4):
                    term = p * v_s[t0 + j, k0:k0 + 8, :]
                    acc[j] = term if w == 0 else acc[j] + term
            for j in range(4):
                o_s[r:r + 8, (t0 + j) * 128:(t0 + j + 1) * 128] = acc[j]
            return o_s, r, t0 * 128
        out = []
        h = U >> cfg["wo"]
        for g in range(0, h + 16, 16):
            if g < h:
                out += tasks(task, [(g + b + j, t0) for b in range(0, U, h) for j in (0, 8)
                                    for t0 in (0, 4)], [p_s, v_s], "lat_short", 62)
            if g:
                out += [] if g < h else gap
                out += left_tasks(oa, "wo", D, lambda r, j, c: o_s[r:r + 16, c:c + 128], [o_s],
                                  rows=[g - 16])
        return out

    def set_halo(buf, src):
        buf[:, 0:HALO, :] = (jnp.zeros((NT, HALO, 128), f32) if src is None
                             else src[:, U:U + HALO, :])

    def copies():
        half = FH // 2

        def units(lo, hi):
            return [(x_hbm.at[0, lo * U:hi * U], x_s.at[lo * U:hi * U])]

        def weight(j, parts):
            n = D // 2 // parts
            return [("w%d_%d" % (j, p), [(wqkv_hbm.at[r:r + n, j * D:(j + 1) * D],
                                          raw.at[j, r:r + n]) for r in (p * n, D // 2 + p * n)])
                    for p in range(parts)]

        def rows_in(lo, hi):
            return [(win_hbm.at[r + lo:r + hi, j * half:(j + 1) * half],
                     raw.at[4 + j, r + lo:r + hi, 0:half])
                    for r in range(0, D, D // 4) for j in range(4)]
        early = share(0, NU - 2, D // 64)[1] * 16
        pairs = [("x0", units(0, 1))]
        pairs += weight(0, PARTS) + [("x1", units(1, 2))] + weight(1, PARTS) + weight(2, 2)
        pairs += [
            ("wo", [(wo_hbm, raw.at[3, 0:D])] + units(2, 3)),
            ("early", units(3, 4) + rows_in(0, early)),
            ("rest", units(4, NU) + rows_in(early, D // 4) + [(bsp_hbm, bsp_raw)]),
            ("late0", [(wsp_hbm.at[0:D, j * D:(j + 1) * D], raw.at[j, 0:D]) for j in range(2)]
             + [(wout_hbm.at[j * half:(j + 1) * half], raw.at[2 + j, 0:half]) for j in range(2)]),
            ("late1", [(wsp_hbm.at[D:S, j * D:(j + 1) * D], raw.at[4 + j, 0:D])
                       for j in range(2)])]
        return {name: [(a, b, sem.at[j]) for a, b in group]
                for j, (name, group) in enumerate(pairs)}

    def start(*names):
        for name in names:
            for args in copies()[name]:
                pltpu.make_async_copy(*args).start()

    def wait(name):
        for args in copies()[name]:
            pltpu.make_async_copy(*args).wait()

    def out_copy(u, half):
        rows = _ds(u * U + half * U // 2, U // 2, U // 2)
        return pltpu.make_async_copy(x_s.at[rows], out_hbm.at[0, rows], osem.at[2 * u + half])

    def unit(ref, u, n=U):
        return ref.at[_ds(u * n, n, n)]

    def clip(v, lo, hi):
        return min(max(v, lo), hi) if isinstance(v, int) else jnp.clip(v, lo, hi)

    def share(step, steps, total):
        count = -(-total // steps)
        return clip(step * count, 0, total - count), count

    def add_into(u):
        def store(r, c, v):
            idx = (slice(r, r + v.shape[0]), slice(c, c + v.shape[1]))
            dst = unit(x_s, u)
            dst[idx] = (dst[idx].astype(f32) + v).astype(bf16)
        return store

    def put_rows(buf):
        def store(r, c, v):
            buf[r:r + v.shape[0], c:c + 128] = v
        return store

    def put_slab(buf):
        def store(r, c, v):
            buf[c // 128, HALO + r:HALO + r + v.shape[0], :] = v
        return store

    def qkv(src, w, store):
        return matmul(src, (w, None), "qkv", D, D, store)

    def project(u):
        return matmul(oa, (wo_p, None), "wo", D, D, add_into(u), cfg["cw_wo"])

    def first_query(part):
        n = D // 4 // PARTS
        rows, cols, q = slice(part * n, (part + 1) * n), slice(part * 2 * n, (part + 1) * 2 * n), U // 4

        def gen():
            tie = yield
            for j in range(2):
                for c in range(0, D // 2, 128):
                    a = jnp.concatenate([jnp.concatenate([
                        xb[(2 + i) * q:(3 + i) * q, cols] if i == m
                        else sp_s.at[i * q:(i + 1) * q, m * D // 2:(m + 1) * D // 2][:, cols]
                        for m in range(2)], axis=1) for i in range(2)], axis=0)
                    b = jnp.concatenate(
                        [wq_p.at[1 + 3 * i][rows, c:c + 128] if i == j
                         else sa.at[i * D // 4:(i + 1) * D // 4][rows, c:c + 128]
                         for i in range(2)], axis=0)
                    res = jnp.dot(_as_bf16(a), _as_bf16(tie(b)), preferred_element_type=f32)
                    idx = (slice(0, U), slice(j * D // 2 + c, j * D // 2 + c + 128))
                    o_s[idx] = o_s[idx] + res if part else res
                    tie = yield res
        return NT, U // 16 * 4 * 4 * n // 128, gen()

    def arriving(main, j, buf, parts, first=0):
        step = main[0] // (len(parts) + first)
        sides = []
        for i, (part, of) in enumerate(parts, first):
            sides += [([(functools.partial(wait, "w%d_%d" % (j, part)), [], 0, 1)],
                       max(0, i * step - 1), i * step),
                      (prep_qkv(j, buf, part, of), i * step, (i + 1) * step - 2)]
        return sides

    def first_attention():
        wait("x0")
        make_zero()
        stats, load, _ = norm_tasks(x_s, unit(x_s, 0), st0)

        def keeping(r, j, c):
            v = load(r, c)
            if r // (U // 2) != j:
                sp_s[r // 2:r // 2 + 8, c:c + 128] = _pack(v)
            return v
        run(stats + left_tasks(xb, "qkv", D, keeping, [x_s]))
        set_halo(kv_s, None)
        wait("w0_0")
        run(prep_qkv(0, wq_p, 0, PARTS, sa))
        for part in range(1, PARTS):
            wait("w0_%d" % part)
            overlap(first_query(part - 1), (prep_qkv(0, wq_p, part, PARTS, sa), 0, NT - cfg["fq"]))
        wait("x1")
        overlap(first_query(PARTS - 1), (norm_x(1, xa), 0, NT - cfg["fq"]))
        main = qkv(xa, wq_p, put_rows(q_s))
        overlap(main, *arriving(main, 1, wk_p, [(p, PARTS) for p in range(PARTS)]))
        main = qkv(xb, wk_p, put_slab(kv_s))
        overlap(main, *arriving(main, 2, wv_p, [(0, 2)], 1))
        logits, soft = logit_tasks(False), softmax_tasks()
        wait("w2_1")
        set_halo(k_s, kv_s)
        overlap(qkv(xa, wk_p, put_slab(k_s)), prep_qkv(2, wv_p, 1, 2) + logit_tasks(True, o_s, kv_s))
        wait("wo")
        prep = prep_wo()
        cut = len(prep) * cfg["f_cut"] // 8
        overlap(qkv(xb, wv_p, put_slab(kv_s)), soft, prep[:cut])
        set_halo(v_s, kv_s)
        overlap(qkv(xa, wv_p, put_slab(v_s)), value_tasks(kv_s), logits[:cfg["f_log"]],
                prep[cut:])
        overlap(project(0), logits[cfg["f_log"]:], norm_x(2, xa))

    def step_attention(u):
        if cfg["part"] != "s1":
            @pl.when(u == 3)
            def _():
                wait("rest")
        begin, count = share(u - 2, NU - 2, _Split(D, cfg["win"]).width // 16)
        prep = (prep_win(wz2_p, Z2_COLS, begin, count)
                + prep_win(wz1_p, Z1_COLS, begin, count))
        cut = len(prep) * cfg["cut_prep"] // 8
        g = clip(u - 2, 0, U // 64 - 1) * 16
        head = norm_h(0, z_s, rows=[g + b for b in range(0, U, 64)]) + left_h(z_s, rows=[g])
        logits = logit_tasks(False)
        set_halo(k_s, k_s)
        overlap(qkv(xa, wq_p, put_rows(q_s)), softmax_tasks(), prep[:cut])
        overlap(qkv(xa, wk_p, put_slab(k_s)), value_tasks())
        set_halo(v_s, v_s)
        overlap(qkv(xa, wv_p, put_slab(v_s)), logits, head)
        overlap(project(u - 1), norm_x(clip(u + 1, 0, NU - 1), xa), prep[cut:])

    def spatial_left(u, rows=range(0, U // 4, 16)):
        per = D // U

        def regroup(r, m):
            lane = lax.broadcasted_iota(jnp.int32, (8, 128), 1)
            col = 2 * U * m
            w = pltpu.bitcast(raw.at[u // per * 4 + col // D][
                _ds(u % per * U + r, 16, 16), col % D:col % D + 2 * U], u32)
            for a in range(2):
                one, two = w[:, a * 128:(a + 1) * 128], w[:, U + a * 128:U + (a + 1) * 128]
                mid = pltpu.roll(jnp.where(lane < 64, two, one), 64, 1)
                for j, v in ((2 * a, jnp.where(lane < 64, one, mid)),
                             (2 * a + 1, jnp.where(lane < 64, mid, two))):
                    sp_s[_ds(r // 2, 8, 8), j * 512 + m * 128:j * 512 + (m + 1) * 128] = v
            return sp_s, r // 2, m * 128
        return tasks(regroup, [(b + r, m) for r in rows for b in range(0, U, U // 4)
                               for m in range(NU // 2)], [raw], "lat_xlu", 18) + left_tasks(
            sa, "sp", S, lambda r, j, c: _unpack(sp_s[_ds(r // 2, 8, 8), c:c + 128]), [sp_s],
            rows=rows)

    def input_product(u, w, cols):
        def store(r, c, v):
            n = v.shape[0]
            if c >= FH:
                z_s[r:r + n, c - FH:c - FH + 128] = _gelu(v)
            else:
                unit(z1_s, u, U // 2)[r // 2:(r + n) // 2, c:c + 128] = _pack(_gelu(v))
        return matmul(ha, (w, None), "win", D, cols, store)

    def norm_z2(u):
        h = U // 4
        stats, _, write = norm_tasks(z_s, z_s, st0, EPS * GAIN * GAIN, 1.0 / GAIN)
        return stats + write(zn_s), right_tasks(
            (z2n_p, z2n_r), "sp", FH, [(u * (h // 2) + r // 2, r) for r in range(0, h, 16)],
            lambda b, r, c: zn_s[b * h + r:b * h + r + 16, c:c + 128], [zn_s])

    def last_attention():
        main = input_product(0, wz2_p, Z2_COLS)
        overlap(main, (softmax_tasks(), 0, cfg["soft_end"]),
                (value_tasks(), cfg["soft_end"], main[0]), spatial_left(0, [0]))
        overlap(project(NU - 1), prep_bias() + spatial_left(0, [16, 32]) + norm_h(1, q_s))

    def step_input(u):
        norm, factors = norm_z2(u - 1)
        cut, early = len(factors) * cfg["z_cut"] // 8, cfg["z_left"]
        main = input_product(u - 1, wz1_p, Z1_COLS)
        last = main[0] - 49
        overlap(main, (norm + factors[:cut], 0, last + cfg["z_over"]),
                *[(left_h(q_s, outer=[o]), last + 7 * j + 6, last + 7 * j + 13)
                  for j, o in enumerate(ORDER[:early])])
        prep = (prep_wout(*share(u - 1, NU - 1, _Split(FH, cfg["out"]).width // 16))
                + prep_wout_rest(*share(u - 1, NU - 1, 8)))
        main = input_product(u, wz2_p, Z2_COLS)
        busy = 7 * (7 - early)
        overlap(main, (sum((left_h(q_s, outer=[o]) for o in ORDER[early:]), []), 0, busy),
                (norm_h(clip(u + 1, 0, NU - 1), q_s), busy, main[0]),
                (factors[cut:] + prep, busy, main[0]))

    def last_input():
        overlap(input_product(NU - 1, wz1_p, Z1_COLS), sum(norm_z2(NU - 1), []),
                spatial_left(0, [48]))

    def step_output(u):
        bt, z1t = unit(bias_s, u), unit(z1_s, u, U // 2)

        def put_y(r, c, g):
            n = g.shape[0]
            z_s[r:r + n, c:c + 128] = _unpack(z1t[r // 2:(r + n) // 2, c:c + 128]) * (
                g + bt[r:r + n, :])

        def gated(**kw):
            return left_tasks(ya, "out", FH, lambda r, j, c: z_s[r:r + 16, c:c + 128], [z_s], **kw)
        overlap(matmul(sa, (z2n_p, z2n_r), "sp", S, FH, put_y),
                *[(gated(cols=[128 * j], rest=False), 49 * j + 49, 49 * j + 49 + 20)
                  for j in range(3)])
        run(gated(cols=[]))
        overlap(matmul(ya, (wout_p, wout_r), "out", FH, D, add_into(u), 256),
                spatial_left(clip(u + 1, 0, NU - 1)),
                ([(out_copy(u, 1).start, [], 0, 1)], 36, 37))
        out_copy(u, 0).start()

    def make_zero():
        bits = pltpu.bitcast(x_s[0:16, 0:128], jnp.int32)
        zero.append(bits[0, 0] ^ pltpu.roll(bits, 1, 1)[0, 1])

    def keep(j):
        v = None
        for b in (wq_p, wk_p, wv_p, wo_p, wz1_p, wz2_p, wout_p, wout_r, z2n_p,
                  z2n_r, z1_s, bias_s, xa, xb, oa, ha, sa, ya, q_s, o_s, k_s, v_s, kv_s, p_s, l_s, e_s,
                  z_s, zn_s, sp_s, *st0, *st1, tmp_s):
            v = done(b, 0, 0) if v is None else v | done(b, 0, 0)
        x_s[0:16, 0:128] = _as_bf16(v)
        c = pltpu.make_async_copy(x_s.at[0:16, 0:128], out_hbm.at[0, 0:16, 0:128], sem.at[0])
        c.start()
        c.wait()

    if cfg["part"] in ("s1", "s2", "s3", "mid"):
        make_zero()
        if cfg["part"] == "mid":
            last_attention()
            last_input()
        else:
            pl.loop(1, NU)({"s1": step_attention, "s2": step_input, "s3": step_output}[cfg["part"]])
        if cfg["part"] == "s3":
            for u in range(1, NU):
                out_copy(u, 0).wait()
                out_copy(u, 1).wait()
        pl.loop(0, 2)(keep)
        return
    import contextlib
    scope = jax.named_scope if cfg["prof"] else (lambda n: contextlib.nullcontext())
    start(*list(copies())[:-2])
    with scope("p_first"):
        first_attention()
    with scope("p_rest0"):
        wait("early")
    if cfg["part"] == "first":
        wait("rest")
        pl.loop(0, 2)(keep)
        return
    start("late0")

    def sc(name, fn):
        def g(u):
            with scope(name):
                fn(u)
        return g
    with scope("p_loop1"):
        pl.loop(2, NU)(sc("p_it1", step_attention))
    start("late1")
    with scope("p_rest2"):
        wait("late0")
    with scope("p_mid"):
        last_attention()
    with scope("p_loop2"):
        pl.loop(1, NU)(sc("p_it2", step_input))
    with scope("p_mid2"):
        last_input()
    wait("late1")
    with scope("p_loop3"):
        pl.loop(0, NU)(sc("p_it3", step_output))
    with scope("p_out"):
        for u in range(NU):
            out_copy(u, 0).wait()
            out_copy(u, 1).wait()


def build(cfg, interpret=False, name="fused_block"):
    vm = pltpu.VMEM

    def right(key, k, n):
        ks, ns = _Split(k, cfg[key]), _Split(n, cfg[key])
        main = vm((7 ** ks.level, ks.width // 2, ns.width), u32)
        if ns.rest:
            return [main, vm((21, ks.width // 2, 128), u32)]
        if ks.rest:
            return [main, vm((14, 64, ns.width), u32)]
        return [main]

    def left(key, k):
        ks = _Split(k, cfg[key])
        return vm((7 ** ks.level * U // ks.parts // 2, ks.width + ks.rest), u32)
    scratch = [
        vm((S + 16, D), bf16),
        vm((8, D + 16, D), bf16),
        vm((S,), bf16),
        *right("qkv", D, D) * 3, *right("wo", D, D),
        vm((49, D // 8, 384), u32), vm((49, D // 8, 512), u32), *right("out", FH, D), *right("sp", S, FH),
        vm((S // 2, FH), u32),
        vm((S, 128), f32),
        left("qkv", D), left("qkv", D), left("wo", D), left("win", D), left("sp", S),
        left("out", FH),
        *[vm((U + 8, D), f32)] * 2,
        *[vm((NT, HALO + U + 8, 128), f32)] * 3,
        vm((WIN, U + 8, 128), f32),
        *[vm((2, U + 8, 128), f32)] * 2,
        *[vm((U + 8, FH), f32)] * 2,
        vm((U // 2 + 8, S), u32),
        *[vm((3, U + 8, 128), f32)] * 2,
        *[vm((U, 128), f32)] * 2,
        vm((25 * U // 4, 256), f32),
        pltpu.SemaphoreType.DMA((9 + 2 * PARTS,)),
        pltpu.SemaphoreType.DMA((2 * NU,)),
    ]
    hbm = pl.BlockSpec(memory_space=pl.ANY)
    return pl.pallas_call(
        functools.partial(_kernel, cfg),
        out_shape=jax.ShapeDtypeStruct((1, S, D), bf16),
        in_specs=[hbm] * 7,
        out_specs=hbm,
        scratch_shapes=scratch,
        compiler_params=pltpu.CompilerParams(vmem_limit_bytes=127 * 1024 * 1024,
                                             flags=cfg["flags"]),
        interpret=interpret,
        name=name,
    )


@jax.jit
def pallas_sequential_preLN__sliding_local_dilated__mixer_gmlp__prompt_kernel(
    A_x: jax.Array,
    A_wqkv: jax.Array,
    A_wo: jax.Array,
    B_x: jax.Array,
    B_w_in: jax.Array,
    B_w_sp: jax.Array,
    B_b_sp: jax.Array,
    B_w_out: jax.Array,
):
    del B_x
    return build(CFG)(A_x, A_wqkv, A_wo, B_w_in, B_w_sp, B_b_sp, B_w_out)
```

```python
import functools

import jax
import jax.numpy as jnp
import numpy as np
from jax import lax
from jax.experimental import pallas as pl
from jax.experimental.pallas import tpu as pltpu

S = 2048
D = 1024
FH = 1792
DH = 32
WIN = 8
DIL = 2
HALO = 16
U = 256
NU = S // U
NT = D // 128
PARTS = 4
EPS = 1e-5

f32 = jnp.float32
bf16 = jnp.bfloat16
u32 = jnp.uint32

CFG = dict(part="all", flags=None, qkv=1, wo=2, win=2, sp=2, out=2, slot=32,
           lat_short=320, lat_xlu=512, tail=0, regs=('win', 'sp', 'wo'), cw_wo=128, cut_prep=7, z_over=21, z_left=3, z_cut=3, fq=2, lag_mix=6, cp=dict(disable_semaphore_checks=True, disable_bounds_checks=True), f_log=0, f_cut=5, gap=200, lag_rstd=6, lag_probs=2, peel=True, wq_parts=4, depth=6, soft_end=90, prof=False)

ORDER = (0, 3, 1, 2, 5, 4, 6)
REST = (3, 1, 2, 4)


def _pack(v):
    return pltpu.bitcast(v.astype(bf16), u32)


def _as_bf16(v):
    return pltpu.bitcast(v, bf16)


def _unpack(v):
    return pltpu.bitcast(v, bf16).astype(f32)


_C = float(np.sqrt(2.0 / np.pi))
ALPHA = float((_C * 0.044715) ** (1.0 / 3.0))
GAIN = 2.0 * ALPHA


def _gelu(v):
    return v * (1.0 + jnp.tanh(v * (_C / ALPHA + v * v)))


LEFT = (((1, 0, 0), (1, 1, 1)), ((1, 1, 0), (1, 1, 1)), ((1, 0, 0),), ((1, 1, 1),),
        ((1, 0, 0), (1, 0, 1)), ((1, 1, 0), (-1, 0, 0)), ((1, 0, 1), (-1, 1, 1)))
RIGHT = (((1, 0, 0), (1, 1, 1)), ((1, 0, 0),), ((1, 0, 1), (-1, 1, 1)), ((1, 1, 0), (-1, 0, 0)),
         ((1, 1, 1),), ((1, 0, 0), (1, 0, 1)), ((1, 1, 0), (1, 1, 1)))


def _factor(terms, get):
    v = get(*terms[0][1:])
    for sign, i, j in terms[1:]:
        v = v + get(i, j) if sign > 0 else v - get(i, j)
    return v


def _factors(forms, get):
    blk = {(i, j): get(i, j) for i in range(2) for j in range(2)}
    return [_factor(terms, lambda i, j: blk[i, j]) for terms in forms]


class _Blocks:
    level, parts, rest = 2, 4, 0

    def __init__(self, chunks):
        self.chunks, self.width = chunks, 128 * len(chunks)

    def col(self, j, c):
        return self.chunks[c // 128][j]


Z1_COLS = _Blocks([[c + s for s in (0, 384, 896, 1280)] for c in (0, 128, 256)])
Z2_COLS = _Blocks([[FH + c for c in chunk] for chunk in Z1_COLS.chunks]
                  + [[FH + 768, FH + 1664, 768, 1664]])


class _Held:
    def __setitem__(self, _, v):
        self.v = v

    def __getitem__(self, _):
        return self.v


def _combiner(tmp, put):
    t1, t2, t3, t4, t5 = tmp

    def feed(i, m):
        if i == 0:
            t1[...] = m
        elif i == 3:
            t4[...] = m
        elif i == 1:
            t2[...] = m
            put(1, 0, m + t4[...])
        elif i == 2:
            t3[...] = m
        elif i == 5:
            put(1, 1, (t1[...] - t2[...] + t3[...]) + m)
        elif i == 4:
            t5[...] = m
            put(0, 1, m + t3[...])
        else:
            put(0, 0, (t1[...] + t4[...] - t5[...]) + m)
    return feed


class _Split:
    def __init__(self, n, level):
        self.level, self.parts = level, 1 << level
        self.width = n // self.parts // 128 * 128
        self.rest = n // 2 - 2 * self.width if level == 2 else 0
        self.half = n // 2

    def start(self, j):
        if self.level == 1:
            return j * self.half
        return (j // 2) * self.half + (j % 2) * self.width

    def col(self, j, c):
        return self.start(j) + c

    def rest_start(self, h):
        return h * self.half + 2 * self.width


def _pair_transpose(v):
    sub = lax.broadcasted_iota(jnp.int32, v[0].shape, 0)
    v = list(v)
    for b in range(2):
        s = 1 << b
        m = (sub & (2 * s)) != 0
        nv = list(v)
        for j in range(4):
            if j & s:
                continue
            lo, hi = v[j], v[j + s]
            nv[j] = jnp.where(m, pltpu.roll(hi, 2 * s, 0), lo)
            nv[j + s] = jnp.where(m, hi, pltpu.roll(lo, 8 - 2 * s, 0))
        v = nv
    return v


def _ds(start, size, align):
    return pl.ds(start if isinstance(start, int) else pl.multiple_of(start, align), size)


def _kernel(cfg,
            x_hbm, wqkv_hbm, wo_hbm, win_hbm, wsp_hbm, bsp_hbm, wout_hbm, out_hbm,
            x_s, raw, bsp_raw,
            wq_p, wk_p, wv_p, wo_p, wz1_p, wz2_p, wout_p, wout_r, z2n_p, z2n_r,
            z1_s, bias_s, xa, xb, oa, ha, sa, ya,
            q_s, o_s, k_s, v_s, kv_s, p_s, l_s, e_s, z_s, zn_s, sp_s, st0_s, st1_s, inv0_s, inv1_s, tmp_s,
            sem, osem):
    st0, st1 = (st0_s, inv0_s), (st1_s, inv1_s)
    zero = []

    def spot(ref, row, col):
        n = 8 * (4 // ref.dtype.itemsize)
        ref = ref if len(ref.shape) == 2 else ref.at[zero[0]]
        return ref.at[_ds(row + zero[0] * n, n, n), _ds(col + zero[0] * 128, 128, 128)]

    def gate(ref, v):
        n = 8 * (4 // ref.dtype.itemsize)
        spot(ref, ref.shape[-2] - n, 0)[0:8, :] = v.astype(ref.dtype)

    def done(ref, row, col):
        v = spot(ref, row, col)[...]
        return v if v.dtype == u32 else pltpu.bitcast(v, u32)

    def tied(toks):
        def tie(b):
            if not toks:
                return b
            tok = functools.reduce(lambda p, q: p | q, toks)
            tok = jnp.concatenate([tok] * (b.shape[1] // 128), axis=1)
            always = lax.broadcasted_iota(jnp.int32, tok.shape, 0) >= zero[0]
            parts = []
            for r in range(0, b.shape[0], 64):
                parts += [b[r:r + 56], jnp.where(always, b[r + 56:r + 64], tok)]
            return jnp.concatenate(parts, axis=0)
        return tie

    def overlap(main, *sides):
        n, cyc, gen = main
        per = max(1, cyc // cfg["slot"])
        plan = [[] for _ in range(n * per)]
        for side in sides:
            if not isinstance(side, tuple):
                side = (side, 0, n)
            todo, first, last = side
            if todo and last == n:
                last -= (todo[-1][2] + cfg["tail"]) / cyc
            span = max(1, int((last - first) * per))
            total, spent = sum(t[3] for t in todo), 0
            for t in todo:
                plan[int(first * per) + spent * span // total].append(t)
                spent += t[3]
        next(gen)
        due = [[] for _ in range(n)]
        for i, todo in enumerate(plan):
            if i % per == 0:
                res = gen.send(tied([tok for _, tok in due[i // per]]))
            gated = []
            for _, refs, _, _ in todo:
                gated += [r for r in refs if not any(r is g for g in gated)]
            row = res.shape[0] * (i % per) // per
            for r in gated:
                gate(r, res[row:row + 8, 0:128])
            for fn, _, lat, _ in todo:
                where = fn()
                j = -(-(i * cyc // per + lat) // cyc)
                if where is not None and j < n:
                    due[j] = [d for d in due[j] if d[0] is not where[0]]
                    due[j].append((where[0], done(*where)))

    def tasks(fn, args, refs, lat, cost):
        return [(functools.partial(fn, *a), refs, cfg[lat], cost) for a in args]

    def staggered(early, late, lag):
        per = len(early) / len(late)
        order = [(j, t) for j, t in enumerate(early)]
        order += [((j + 1) * per + lag - 0.5, t) for j, t in enumerate(late)]
        return [t for _, t in sorted(order, key=lambda p: p[0])]

    gap = [(lambda: None, [], 0, cfg["gap"])]

    def run(todo):
        for t in todo:
            t[0]()

    def left_tasks(ref, key, k, load, refs, rows=None, cols=None, outer=None, rest=True):
        ks = _Split(k, cfg[key])
        h = U // ks.parts

        def put(n, r, c, v):
            ref[_ds(n * h // 2 + r // 2, 8, 8), c:c + 128] = _pack(v)

        def main(r, c, o):
            def get(i, j):
                if ks.level == 1:
                    return load(i * h + r, j, ks.start(j) + c)
                return _factor(LEFT[o], lambda a, b: load((2 * a + i) * h + r, 2 * b + j,
                                                          ks.start(2 * b + j) + c))
            for n, v in enumerate(_factors(LEFT, get)):
                put(7 * o + n, r, c, v)
            return ref, 7 * o * h // 2 + r // 2, c

        def other(r, i):
            vals = _factors(LEFT, lambda a, b: load((2 * a + i) * h + r, None, ks.rest_start(b)))
            for o, v in enumerate(vals):
                put(7 * o + 6 - i, r, ks.width, v)
            return ref, (6 - i) * h // 2 + r // 2, ks.width
        out = []
        for r in range(0, h, 16) if rows is None else rows:
            out += tasks(main, [(r, c, o)
                                for c in (range(0, ks.width, 128) if cols is None else cols)
                                for o in (range(7 ** (ks.level - 1)) if outer is None else outer)],
                         refs, "lat_short", 30)
            out += tasks(other, [(r, 0), (r, 1)] if ks.rest and rest else [], refs, "lat_short", 30)
        return out

    def right_tasks(bufs, key, n, rows, load, refs, lat="lat_short"):
        main_p, rest_p = bufs
        ns = n if isinstance(n, _Blocks) else _Split(n, cfg[key])

        def main(prow, r, c, o):
            def get(i, j):
                if ns.level == 1:
                    return load(i, r, ns.start(j) + c)
                return _factor(RIGHT[o], lambda a, b: load(2 * a + i, r, ns.col(2 * b + j, c)))
            for m, v in enumerate(_factors(RIGHT, get)):
                main_p.at[7 * o + m][_ds(prow, 8, 8), c:c + 128] = _pack(v)
            return main_p, prow, c

        def rest(prow, r, o):
            top, bot = [_factor(RIGHT[o], lambda a, b: load(2 * a + i, r, ns.rest_start(b)))
                        for i in range(2)]
            for m, v in enumerate((top, bot, top - bot)):
                rest_p.at[3 * o + m][_ds(prow, 8, 8), :] = _pack(v)
            return rest_p, prow, 0
        out = []
        for prow, r in rows:
            out += tasks(main, [(prow, r, c, o) for c in range(0, ns.width, 128)
                                for o in range(7 ** (ns.level - 1))], refs, lat, 32)
            out += tasks(rest, [(prow, r, o) for o in range(7)] if ns.rest else [], refs,
                         "lat_short", 16)
        return out

    def matmul(ref, bufs, key, k, n, store, cw=128):
        main_p, rest_p = bufs
        ks = _Split(k, cfg[key])
        ns = n if isinstance(n, _Blocks) else _Split(n, cfg[key])
        h = U // ks.parts

        def lhs(m, lo, hi):
            return _as_bf16(ref[m * h // 2:(m + 1) * h // 2, lo:hi])

        def dot(a, b):
            return jnp.dot(a, _as_bf16(b), preferred_element_type=f32)

        def temps(slot):
            return [tmp_s.at[(5 * slot + j) * h:(5 * slot + j + 1) * h, 0:cw] for j in range(5)]

        def gen1():
            tie = yield
            for c in range(0, ns.width, cw):
                feed = _combiner(temps(0), lambda i, j, v: store(i * h, ns.start(j) + c, v))
                for m in ORDER:
                    res = dot(lhs(m, 0, ks.width), tie(main_p.at[m][:, c:c + cw]))
                    feed(m, res)
                    tie = yield res

        def inner_temps():
            return [_Held() for _ in range(5)] if key in cfg["regs"] else temps(4)

        def chunk(c, tie):
            def put(i, j):
                return lambda a, b, v: store((2 * a + i) * h, ns.col(2 * b + j, c), v)
            outer = {(i, j): _combiner(temps(2 * i + j), put(i, j))
                     for i in range(2) for j in range(2)}
            for o in ORDER:
                def extra(i, j, v):
                    if ks.rest and i != j:
                        v = v + dot(lhs(7 * o + 6 - i, ks.width, ks.width + 128),
                                    rest_p.at[2 * o + j][:, c:c + cw])
                    outer[i, j](o, v)
                feed = _combiner(inner_temps(), extra)
                for m in ORDER:
                    b = main_p.at[7 * o + m][:, c:c + cw]
                    hi = ks.width
                    if ks.rest and m >= 5:
                        b = jnp.concatenate([b, rest_p.at[2 * o + 6 - m][:, c:c + cw]], axis=0)
                        hi += 128
                    res = dot(lhs(7 * o + m, 0, hi), tie(b))
                    feed(m, res)
                    tie = yield res
            return tie

        def rest_chunk(tie):
            def put(i):
                return lambda a, b, v: store((2 * a + i) * h, ns.rest_start(b), v)
            outer = [_combiner(temps(i), put(i)) for i in range(2)]
            for o in ORDER:
                for i, (m0, b0), (m1, b1) in ((1, (3, 2), (1, 0)), (0, (2, 2), (4, 1))):
                    first = dot(lhs(7 * o + m0, 0, ks.width), tie(rest_p.at[3 * o + b0][...]))
                    tie = yield first
                    res = dot(lhs(7 * o + m1, 0, ks.width), tie(rest_p.at[3 * o + b1][...]))
                    outer[i](o, res - first if i else res + first)
                    tie = yield res
            return tie

        def gen2():
            tie = yield
            for c in range(0, ns.width, cw):
                tie = yield from chunk(c, tie)
            if ns.rest:
                tie = yield from rest_chunk(tie)
        cyc = h // 16 * 4 * (ks.width // 128) * (cw // 128)
        if ks.level == 1:
            return 7 * (ns.width // cw), cyc, gen1()
        return 49 * (ns.width // cw) + (28 if ns.rest else 0), cyc, gen2()

    def staged(i):
        return (z_s, zn_s)[i].at[0:D // 4, 0:D]

    def mix_staged(buf, key, shift, rows, plain=None):
        h = _Split(D, cfg[key]).width // 2

        def load(i, r, c):
            r += i * h
            i, r, tile = r // (D // 4), r % (D // 4), c // 128
            v = pltpu.bitcast(staged(i)[r:r + 8, c:c + 128], u32)
            v = pltpu.roll(v, 128 - 4 * tile, 1) if shift and tile else v
            if plain is not None and i != c // (D // 2):
                plain[i * D // 4 + r:i * D // 4 + r + 8, c % (D // 2):c % (D // 2) + 128] = v
            return _unpack(v)
        return right_tasks((buf, None), key, D, [(r, r) for r in rows], load,
                           [raw] if shift else [z_s, zn_s],
                           "lat_xlu" if shift else "lat_short")

    def prep_qkv(j, buf, part, parts, plain=None):
        def task(i, r):
            w = pltpu.bitcast(raw.at[j][i * D // 2 + r:i * D // 2 + r + 16, :], u32)
            lane = lax.broadcasted_iota(jnp.int32, (8, 128), 1)
            w = [w[:, t * 128:(t + 1) * 128] for t in range(NT)]
            w = [pltpu.roll(v, 4 * t, 1) if t else v for t, v in enumerate(w)]
            w = [w[(-t) % NT] for t in range(NT)]
            for b in range(3):
                m = (lane & (4 << b)) != 0
                w = [jnp.where(m, w[(t - (1 << b)) % NT], w[t]) for t in range(NT)]
            for t in range(NT):
                staged(i)[r // 2:r // 2 + 8, t * 128:(t + 1) * 128] = pltpu.bitcast(w[t], f32)
            return (z_s, zn_s)[i], r // 2, 0
        rows = range(part * D // 2 // parts, (part + 1) * D // 2 // parts, 16)
        return staggered(
            tasks(task, [(i, r) for r in rows for i in range(2)], [raw], "lat_xlu", 45),
            mix_staged(buf, "qkv", True, [r // 2 for r in rows], plain), cfg["lag_mix"])

    def prep_wo():
        def task(d4, t2, hh, c):
            src = [((t2 * 4 + j) * 4 + hh) * 32 + d4 * 16 for j in range(4)]
            v = _pair_transpose([pltpu.bitcast(raw.at[3][s:s + 16, c:c + 256], u32) for s in src])
            for j in range(4):
                r = ((j * 4 + hh) * 32 + t2 * 16) // 2
                staged(d4)[r:r + 8, c:c + 256] = pltpu.bitcast(v[j], f32)
            return (z_s, zn_s)[d4], r, c
        return tasks(task, [(d4, t2, hh, c) for d4 in range(2) for t2 in range(2)
                            for hh in range(4) for c in range(0, D, 256)],
                     [raw], "lat_short", 40) + gap + mix_staged(
            wo_p, "wo", False, range(0, _Split(D, cfg["wo"]).width // 2, 8))

    def prep_win(buf, cols, first, count):
        ks = _Split(D, cfg["win"])

        def load(i, r, c):
            return raw.at[4 + c // (FH // 2)][
                _ds(ks.start(i) + r, 16, 16), c % (FH // 2):c % (FH // 2) + 128].astype(f32)
        rows = [((first + g) * 8, (first + g) * 16) for g in range(count)]
        return right_tasks((buf, None), "win", cols, rows, load, [raw])

    def prep_wout(first, count):
        ks = _Split(FH, cfg["out"])

        def load(i, r, c):
            row = ks.start(i)
            return raw.at[2 + row // (FH // 2)][
                _ds(row % (FH // 2) + r, 16, 16), c:c + 128].astype(f32)
        rows = [((first + g) * 8, (first + g) * 16) for g in range(count)]
        return right_tasks((wout_p, None), "out", D, rows, load, [raw])

    def prep_wout_rest(first, count):
        ks, ns = _Split(FH, cfg["out"]), _Split(D, cfg["out"])

        def task(g, j, c):
            def get(a, b):
                col = ns.start(2 * b + j) + c
                return raw.at[2 + a][_ds(2 * ks.width + (first + g) * 16, 16, 16),
                                     col:col + 128].astype(f32)
            for o, v in enumerate(_factors(RIGHT, get)):
                wout_r.at[2 * o + j][_ds((first + g) * 8, 8, 8), c:c + 128] = _pack(v)
            return wout_r, (first + g) * 8, c
        if not ks.rest:
            return []
        return tasks(task, [(g, j, c) for g in range(count) for j in range(2)
                            for c in range(0, ns.width, 128)], [raw], "lat_short", 28)

    def prep_bias():
        def task(j):
            b = bsp_raw[...].astype(f32).reshape(1, S) * (1.0 / GAIN)
            bias_s[j * 128:(j + 1) * 128, :] = jnp.broadcast_to(
                b[:, j * 128:(j + 1) * 128], (128, 128)).T
            return bias_s, j * 128, 0
        return tasks(task, [(j,) for j in range(S // 128)], [], "lat_xlu", 50)

    def norm_tasks(base, src, st, eps=EPS, scale=None, rows=range(0, U, 16)):
        n = src.shape[1]
        st, inv = st

        def shift(r):
            v = src[_ds(r, 16, 16), 0:128].astype(f32)
            st.at[0][_ds(r, 16, 16), :] = jnp.broadcast_to(v[:, 0:1], (16, 128))
            return st, r, 0

        def stats(r):
            sh = st.at[0][_ds(r, 8, 8), :]
            s1 = s2 = None
            for c in range(0, n, 256):
                v = src[_ds(r, 8, 8), c:c + 256].astype(f32)
                for d in (v[:, :128] - sh, v[:, 128:] - sh):
                    s1 = d if s1 is None else s1 + d
                    s2 = d * d if s2 is None else s2 + d * d
            m = jnp.sum(s1, axis=-1, keepdims=True) * (1.0 / n)
            var = jnp.sum(s2, axis=-1, keepdims=True) * (1.0 / n) - m * m
            st.at[1][_ds(r, 8, 8), :] = sh + m
            st.at[2][_ds(r, 8, 8), :] = jnp.broadcast_to(jnp.maximum(var, 0.0) + eps, (8, 128))
            return st, r, 0

        def rstd(r):
            v = lax.rsqrt(st.at[2][_ds(r, 16, 16), :])
            inv[_ds(r, 16, 16), :] = v if scale is None else v * scale
            return inv, r, 0

        def load(r, c, h=16, w=128):
            v = src[_ds(r, h, h), c:c + w].astype(f32)
            mean, mul = [jnp.concatenate([t[_ds(r, h, h), :]] * (w // 128), axis=1)
                         for t in (st.at[1], inv)]
            return (v - mean) * mul

        def write(dst):
            def task(r, c, w):
                dst[_ds(r, 8, 8), c:c + w] = load(r, c, 8, w)
                return dst, r, c
            return tasks(task, [(r + j, c, min(1024, n - c)) for r in rows for j in (0, 8)
                                for c in range(0, n, 1024)], [base], "lat_short", 22)
        out = tasks(shift, [(r,) for r in rows], [base], "lat_xlu", 10)
        out += staggered(tasks(stats, [(r + j,) for r in rows for j in (0, 8)], [base], "lat_xlu",
                               n // 28 + 8),
                         tasks(rstd, [(r,) for r in rows], [], "lat_short", 22), cfg["lag_rstd"])
        return out, load, write

    def norm_x(u, buf):
        out, load, _ = norm_tasks(x_s, unit(x_s, u), st0)
        return out + left_tasks(buf, "qkv", D, lambda r, j, c: load(r, c), [x_s])

    def norm_h(u, spare, **kw):
        out, _, write = norm_tasks(x_s, unit(x_s, u), st1, scale=ALPHA, **kw)
        return out + write(spare)

    def left_h(spare, **kw):
        return left_tasks(ha, "win", D, lambda r, j, c: spare[_ds(r, 16, 16), c:c + 128], [spare],
                          **kw)

    def take(v, idx):
        return jnp.take_along_axis(v, idx, axis=1)

    def logit_tasks(first, q_s=q_s, k_s=k_s):
        def task(r, b):
            lane = lax.broadcasted_iota(jnp.int32, (8, 128), 1)
            acc = [None] * 4
            for t in range(NT):
                q = q_s[r:r + 8, t * 128:(t + 1) * 128]
                for j in range(4):
                    k0 = HALO + r - DIL * (4 * b + j)
                    term = q * k_s[t, k0:k0 + 8, :]
                    acc[j] = term if t == 0 else acc[j] + term
            for bit in (1, 2):
                odd = (lane & bit) != 0
                acc = [jnp.where(odd, acc[j ^ bit], acc[j]) for j in range(4)]
            lg = acc[0]
            for j in range(1, 4):
                lg = lg + take(acc[j], lane ^ j)
            lg = lg * float(DH) ** -0.5
            if first and r < DIL * WIN:
                pos = r + lax.broadcasted_iota(jnp.int32, (8, 128), 0)
                lg = jnp.where(pos >= DIL * (4 * b + (lane & 3)), lg, -1e9)
            l_s[b, r:r + 8, :] = lg
            return l_s, r, 0
        return tasks(task, [(r, b) for r in range(0, U, 8) for b in range(2)], [q_s, k_s],
                     "lat_xlu", 75)

    def softmax_tasks():
        def exps(r):
            lane = lax.broadcasted_iota(jnp.int32, (16, 128), 1)
            lg = [l_s[b, r:r + 16, :] for b in range(2)]
            mx = jnp.maximum(lg[0], lg[1])
            mx = functools.reduce(jnp.maximum, [mx] + [take(mx, lane ^ j) for j in range(1, 4)])
            for b in range(2):
                e_s[b, r:r + 16, :] = jnp.exp(lg[b] - mx)
            return e_s, r, 0

        def probs(r):
            lane = lax.broadcasted_iota(jnp.int32, (8, 128), 1)
            e = [e_s[b, r:r + 8, :] for b in range(2)]
            e = {4 * b + j: take(e[b], (lane & -4) | j) for j in range(4) for b in range(2)}
            inv = 1.0 / functools.reduce(lambda p, q: p + q, e.values())
            for w in range(WIN):
                p_s[w, r:r + 8, :] = e[w] * inv
            return p_s, r, 0
        return staggered(tasks(exps, [(r,) for r in range(0, U, 16)], [l_s], "lat_xlu", 40),
                         tasks(probs, [(r,) for r in range(0, U, 8)], [], "lat_xlu", 40),
                         cfg["lag_probs"])

    def value_tasks(v_s=v_s):
        def task(r, t0):
            acc = [None] * 4
            for w in range(WIN):
                k0 = HALO + r - DIL * w
                p = p_s[w, r:r + 8, :]
                for j in range(4):
                    term = p * v_s[t0 + j, k0:k0 + 8, :]
                    acc[j] = term if w == 0 else acc[j] + term
            for j in range(4):
                o_s[r:r + 8, (t0 + j) * 128:(t0 + j + 1) * 128] = acc[j]
            return o_s, r, t0 * 128
        out = []
        h = U >> cfg["wo"]
        for g in range(0, h + 16, 16):
            if g < h:
                out += tasks(task, [(g + b + j, t0) for b in range(0, U, h) for j in (0, 8)
                                    for t0 in (0, 4)], [p_s, v_s], "lat_short", 62)
            if g:
                out += [] if g < h else gap
                out += left_tasks(oa, "wo", D, lambda r, j, c: o_s[r:r + 16, c:c + 128], [o_s],
                                  rows=[g - 16])
        return out

    def set_halo(buf, src):
        buf[:, 0:HALO, :] = (jnp.zeros((NT, HALO, 128), f32) if src is None
                             else src[:, U:U + HALO, :])

    def copies():
        half = FH // 2

        def units(lo, hi):
            return [(x_hbm.at[0, lo * U:hi * U], x_s.at[lo * U:hi * U])]

        def weight(j, parts):
            n = D // 2 // parts
            return [("w%d_%d" % (j, p), [(wqkv_hbm.at[r:r + n, j * D:(j + 1) * D],
                                          raw.at[j, r:r + n]) for r in (p * n, D // 2 + p * n)])
                    for p in range(parts)]

        def rows_in(lo, hi):
            return [(win_hbm.at[r + lo:r + hi, j * half:(j + 1) * half],
                     raw.at[4 + j, r + lo:r + hi, 0:half])
                    for r in range(0, D, D // 4) for j in range(4)]
        early = share(0, NU - 2, D // 64)[1] * 16
        pairs = [("x0", units(0, 1))]
        pairs += weight(0, PARTS) + [("x1", units(1, 2))] + weight(1, PARTS) + weight(2, 2)
        pairs += [
            ("wo", [(wo_hbm, raw.at[3, 0:D])] + units(2, 3)),
            ("early", units(3, 4) + rows_in(0, early)),
            ("rest", units(4, NU) + rows_in(early, D // 4) + [(bsp_hbm, bsp_raw)]),
            ("late0", [(wsp_hbm.at[0:D, j * D:(j + 1) * D], raw.at[j, 0:D]) for j in range(2)]
             + [(wout_hbm.at[j * half:(j + 1) * half], raw.at[2 + j, 0:half]) for j in range(2)]),
            ("late1", [(wsp_hbm.at[D:S, j * D:(j + 1) * D], raw.at[4 + j, 0:D])
                       for j in range(2)])]
        return {name: [(a, b, sem.at[j]) for a, b in group]
                for j, (name, group) in enumerate(pairs)}

    def start(*names):
        for name in names:
            for args in copies()[name]:
                pltpu.make_async_copy(*args).start()

    def wait(name):
        with scope("p_" + name):
            for args in copies()[name]:
                pltpu.make_async_copy(*args).wait()

    def out_copy(u, part):
        rows = _ds(u * U + (0 if part else U // 2), U // 2, U // 2)
        cols = (slice(0, D), slice(D // 2, D), slice(0, D // 2))[part]
        return pltpu.make_async_copy(x_s.at[rows, cols], out_hbm.at[0, rows, cols], osem.at[0])

    def unit(ref, u, n=U):
        return ref.at[_ds(u * n, n, n)]

    def clip(v, lo, hi):
        return min(max(v, lo), hi) if isinstance(v, int) else jnp.clip(v, lo, hi)

    def share(step, steps, total):
        count = -(-total // steps)
        return clip(step * count, 0, total - count), count

    def add_into(u):
        def store(r, c, v):
            idx = (slice(r, r + v.shape[0]), slice(c, c + v.shape[1]))
            dst = unit(x_s, u)
            dst[idx] = (dst[idx].astype(f32) + v).astype(bf16)
        return store

    def put_rows(buf):
        def store(r, c, v):
            buf[r:r + v.shape[0], c:c + 128] = v
        return store

    def put_slab(buf):
        def store(r, c, v):
            buf[c // 128, HALO + r:HALO + r + v.shape[0], :] = v
        return store

    def qkv(src, w, store):
        return matmul(src, (w, None), "qkv", D, D, store)

    def project(u):
        return matmul(oa, (wo_p, None), "wo", D, D, add_into(u), cfg["cw_wo"])

    def first_query(part):
        n = D // 4 // PARTS
        rows, cols, q = slice(part * n, (part + 1) * n), slice(part * 2 * n, (part + 1) * 2 * n), U // 4

        def gen():
            tie = yield
            for j in range(2):
                for c in range(0, D // 2, 128):
                    a = jnp.concatenate([jnp.concatenate([
                        xb[(2 + i) * q:(3 + i) * q, cols] if i == m
                        else sp_s.at[i * q:(i + 1) * q, m * D // 2:(m + 1) * D // 2][:, cols]
                        for m in range(2)], axis=1) for i in range(2)], axis=0)
                    b = jnp.concatenate(
                        [wq_p.at[1 + 3 * i][rows, c:c + 128] if i == j
                         else sa.at[i * D // 4:(i + 1) * D // 4][rows, c:c + 128]
                         for i in range(2)], axis=0)
                    res = jnp.dot(_as_bf16(a), _as_bf16(tie(b)), preferred_element_type=f32)
                    idx = (slice(0, U), slice(j * D // 2 + c, j * D // 2 + c + 128))
                    o_s[idx] = o_s[idx] + res if part else res
                    tie = yield res
        return NT, U // 16 * 4 * 4 * n // 128, gen()

    def arriving(main, j, buf, parts, first=0):
        step = main[0] // (len(parts) + first)
        sides = []
        for i, (part, of) in enumerate(parts, first):
            sides += [([(functools.partial(wait, "w%d_%d" % (j, part)), [], 0, 1)],
                       max(0, i * step - 1), i * step),
                      (prep_qkv(j, buf, part, of), i * step, (i + 1) * step - 2)]
        return sides

    def first_attention():
        wait("x0")
        make_zero()
        stats, load, _ = norm_tasks(x_s, unit(x_s, 0), st0)

        def keeping(r, j, c):
            v = load(r, c)
            if r // (U // 2) != j:
                sp_s[r // 2:r // 2 + 8, c:c + 128] = _pack(v)
            return v
        run(stats + left_tasks(xb, "qkv", D, keeping, [x_s]))
        set_halo(kv_s, None)
        wait("w0_0")
        run(prep_qkv(0, wq_p, 0, PARTS, sa))
        for part in range(1, PARTS):
            wait("w0_%d" % part)
            overlap(first_query(part - 1), (prep_qkv(0, wq_p, part, PARTS, sa), 0, NT - cfg["fq"]))
        wait("x1")
        overlap(first_query(PARTS - 1), (norm_x(1, xa), 0, NT - cfg["fq"]))
        main = qkv(xa, wq_p, put_rows(q_s))
        overlap(main, *arriving(main, 1, wk_p, [(p, PARTS) for p in range(PARTS)]))
        main = qkv(xb, wk_p, put_slab(kv_s))
        overlap(main, *arriving(main, 2, wv_p, [(0, 2)], 1))
        logits, soft = logit_tasks(False), softmax_tasks()
        wait("w2_1")
        set_halo(k_s, kv_s)
        overlap(qkv(xa, wk_p, put_slab(k_s)), prep_qkv(2, wv_p, 1, 2) + gap + logit_tasks(True, o_s, kv_s))
        wait("wo")
        prep = prep_wo()
        cut = len(prep) * cfg["f_cut"] // 8
        overlap(qkv(xb, wv_p, put_slab(kv_s)), soft, prep[:cut])
        set_halo(v_s, kv_s)
        overlap(qkv(xa, wv_p, put_slab(v_s)), value_tasks(kv_s), logits[:cfg["f_log"]],
                prep[cut:])
        overlap(project(0), logits[cfg["f_log"]:], norm_x(2, xa))

    def step_attention(u):
        if cfg["part"] != "s1":
            @pl.when(u == 3)
            def _():
                wait("rest")
        begin, count = share(u - 2, NU - 2, _Split(D, cfg["win"]).width // 16)
        prep = (prep_win(wz2_p, Z2_COLS, begin, count)
                + prep_win(wz1_p, Z1_COLS, begin, count))
        cut = len(prep) * cfg["cut_prep"] // 8
        g = clip(u - 2, 0, U // 64 - 1) * 16
        head = norm_h(0, z_s, rows=[g + b for b in range(0, U, 64)]) + left_h(z_s, rows=[g])
        logits = logit_tasks(False)
        set_halo(k_s, k_s)
        overlap(qkv(xa, wq_p, put_rows(q_s)), softmax_tasks(), prep[:cut])
        overlap(qkv(xa, wk_p, put_slab(k_s)), value_tasks())
        set_halo(v_s, v_s)
        overlap(qkv(xa, wv_p, put_slab(v_s)), logits, head)
        overlap(project(u - 1), norm_x(clip(u + 1, 0, NU - 1), xa), prep[cut:])

    def spatial_left(u, rows=range(0, U // 4, 16)):
        per = D // U

        def regroup(r, m):
            lane = lax.broadcasted_iota(jnp.int32, (8, 128), 1)
            col = 2 * U * m
            w = pltpu.bitcast(raw.at[u // per * 4 + col // D][
                _ds(u % per * U + r, 16, 16), col % D:col % D + 2 * U], u32)
            for a in range(2):
                one, two = w[:, a * 128:(a + 1) * 128], w[:, U + a * 128:U + (a + 1) * 128]
                mid = pltpu.roll(jnp.where(lane < 64, two, one), 64, 1)
                for j, v in ((2 * a, jnp.where(lane < 64, one, mid)),
                             (2 * a + 1, jnp.where(lane < 64, mid, two))):
                    sp_s[_ds(r // 2, 8, 8), j * 512 + m * 128:j * 512 + (m + 1) * 128] = v
            return sp_s, r // 2, m * 128
        return [tasks(regroup, [(b + r, m) for r in rows for b in range(0, U, U // 4)
                                for m in range(NU // 2)], [raw], "lat_xlu", 18),
                left_tasks(sa, "sp", S, lambda r, j, c: _unpack(sp_s[r // 2:r // 2 + 8, c:c + 128]),
                           [sp_s], rows=rows)]

    def input_product(u, w, cols):
        def store(r, c, v):
            n = v.shape[0]
            if c >= FH:
                z_s[r:r + n, c - FH:c - FH + 128] = _gelu(v)
            else:
                unit(z1_s, u, U // 2)[r // 2:(r + n) // 2, c:c + 128] = _pack(_gelu(v))
        return matmul(ha, (w, None), "win", D, cols, store)

    def norm_z2(u):
        h = U // 4
        stats, _, write = norm_tasks(z_s, z_s, st0, EPS * GAIN * GAIN, 1.0 / GAIN)
        return stats + write(zn_s), right_tasks(
            (z2n_p, z2n_r), "sp", FH, [(u * (h // 2) + r // 2, r) for r in range(0, h, 16)],
            lambda b, r, c: zn_s[b * h + r:b * h + r + 16, c:c + 128], [zn_s])

    def last_attention():
        main = input_product(0, wz2_p, Z2_COLS)
        overlap(main, (softmax_tasks(), 0, cfg["soft_end"]),
                (value_tasks(), cfg["soft_end"], main[0]), spatial_left(0)[0])
        overlap(project(NU - 1), prep_bias() + spatial_left(0, [0, 16])[1] + norm_h(1, q_s))

    def step_input(u):
        norm, factors = norm_z2(u - 1)
        cut, early = len(factors) * cfg["z_cut"] // 8, cfg["z_left"]
        main = input_product(u - 1, wz1_p, Z1_COLS)
        last = main[0] - 49
        overlap(main, (norm + factors[:cut], 0, last + cfg["z_over"]),
                *[(left_h(q_s, outer=[o]), last + 7 * j + 6, last + 7 * j + 13)
                  for j, o in enumerate(ORDER[:early])])
        prep = (prep_wout(*share(u - 1, NU - 1, _Split(FH, cfg["out"]).width // 16))
                + prep_wout_rest(*share(u - 1, NU - 1, 8)))
        main = input_product(u, wz2_p, Z2_COLS)
        busy = 7 * (7 - early)
        overlap(main, (sum((left_h(q_s, outer=[o]) for o in ORDER[early:]), []), 0, busy),
                (norm_h(clip(u + 1, 0, NU - 1), q_s), busy, main[0]),
                (factors[cut:] + prep, busy, main[0]))

    def last_input():
        overlap(input_product(NU - 1, wz1_p, Z1_COLS), sum(norm_z2(NU - 1), []),
                spatial_left(0, [32, 48])[1])

    def step_output(u):
        bt, z1t = unit(bias_s, u), unit(z1_s, u, U // 2)

        def put_y(r, c, g):
            n = g.shape[0]
            z_s[r:r + n, c:c + 128] = _unpack(z1t[r // 2:(r + n) // 2, c:c + 128]) * (
                g + bt[r:r + n, :])

        def gated(**kw):
            return left_tasks(ya, "out", FH, lambda r, j, c: z_s[r:r + 16, c:c + 128], [z_s], **kw)
        regroup, factors = spatial_left(clip(u + 1, 0, NU - 1))
        overlap(matmul(sa, (z2n_p, z2n_r), "sp", S, FH, put_y), (regroup, 0, 49),
                *[(gated(cols=[128 * j], rest=False), 49 * j + 49, 49 * j + 49 + 20)
                  for j in range(3)])
        run(gated(cols=[]))
        overlap(matmul(ya, (wout_p, wout_r), "out", FH, D, add_into(u), 256),
                factors,
                ([(out_copy(u, 0).start, [], 0, 1)], 36, 37),
                ([(out_copy(u, 1).start, [], 0, 1)], 43, 44))
        out_copy(u, 2).start()

    def make_zero():
        bits = pltpu.bitcast(x_s[0:16, 0:128], jnp.int32)
        zero.append(bits[0, 0] ^ pltpu.roll(bits, 1, 1)[0, 1])

    def keep(j):
        v = None
        for b in (wq_p, wk_p, wv_p, wo_p, wz1_p, wz2_p, wout_p, wout_r, z2n_p,
                  z2n_r, z1_s, bias_s, xa, xb, oa, ha, sa, ya, q_s, o_s, k_s, v_s, kv_s, p_s, l_s, e_s,
                  z_s, zn_s, sp_s, *st0, *st1, tmp_s):
            v = done(b, 0, 0) if v is None else v | done(b, 0, 0)
        x_s[0:16, 0:128] = _as_bf16(v)
        c = pltpu.make_async_copy(x_s.at[0:16, 0:128], out_hbm.at[0, 0:16, 0:128], sem.at[0])
        c.start()
        c.wait()

    if cfg["part"] in ("s1", "s2", "s3", "mid"):
        make_zero()
        if cfg["part"] == "mid":
            last_attention()
            last_input()
        else:
            pl.loop(1, NU)({"s1": step_attention, "s2": step_input, "s3": step_output}[cfg["part"]])
        if cfg["part"] == "s3":
            for u in range(1, NU):
                out_copy(u, 0).wait()
                out_copy(u, 1).wait()
            out_copy(u, 2).wait()
        pl.loop(0, 2)(keep)
        return
    import contextlib
    scope = jax.named_scope if cfg["prof"] else (lambda n: contextlib.nullcontext())
    start(*list(copies())[:-2])
    with scope("p_first"):
        first_attention()
    with scope("p_rest0"):
        wait("early")
    if cfg["part"] == "first":
        wait("rest")
        pl.loop(0, 2)(keep)
        return
    start("late0")

    def sc(name, fn):
        def g(u):
            with scope(name):
                fn(u)
        return g
    with scope("p_loop1"):
        pl.loop(2, NU)(sc("p_it1", step_attention))
    start("late1")
    with scope("p_rest2"):
        wait("late0")
    with scope("p_mid"):
        last_attention()
    with scope("p_loop2"):
        pl.loop(1, NU)(sc("p_it2", step_input))
    with scope("p_mid2"):
        last_input()
    wait("late1")
    with scope("p_loop3"):
        pl.loop(0, NU)(sc("p_it3", step_output))
    with scope("p_out"):
        for u in range(NU):
            out_copy(u, 0).wait()
            out_copy(u, 1).wait()
            out_copy(u, 2).wait()


def build(cfg, interpret=False, name="fused_block"):
    vm = pltpu.VMEM

    def right(key, k, n):
        ks, ns = _Split(k, cfg[key]), _Split(n, cfg[key])
        main = vm((7 ** ks.level, ks.width // 2, ns.width), u32)
        if ns.rest:
            return [main, vm((21, ks.width // 2, 128), u32)]
        if ks.rest:
            return [main, vm((14, 64, ns.width), u32)]
        return [main]

    def left(key, k):
        ks = _Split(k, cfg[key])
        return vm((7 ** ks.level * U // ks.parts // 2, ks.width + ks.rest), u32)
    scratch = [
        vm((S + 16, D), bf16),
        vm((8, D + 16, D), bf16),
        vm((S,), bf16),
        *right("qkv", D, D) * 3, *right("wo", D, D),
        vm((49, D // 8, 384), u32), vm((49, D // 8, 512), u32), *right("out", FH, D), *right("sp", S, FH),
        vm((S // 2, FH), u32),
        vm((S, 128), f32),
        left("qkv", D), left("qkv", D), left("wo", D), left("win", D), left("sp", S),
        left("out", FH),
        *[vm((U + 8, D), f32)] * 2,
        *[vm((NT, HALO + U + 8, 128), f32)] * 3,
        vm((WIN, U + 8, 128), f32),
        *[vm((2, U + 8, 128), f32)] * 2,
        *[vm((U + 8, FH), f32)] * 2,
        vm((U // 2 + 8, S), u32),
        *[vm((3, U + 8, 128), f32)] * 2,
        *[vm((U, 128), f32)] * 2,
        vm((25 * U // 4, 256), f32),
        pltpu.SemaphoreType.DMA((9 + 2 * PARTS,)),
        pltpu.SemaphoreType.DMA((1,)),
    ]
    hbm = pl.BlockSpec(memory_space=pl.ANY)
    return pl.pallas_call(
        functools.partial(_kernel, cfg),
        out_shape=jax.ShapeDtypeStruct((1, S, D), bf16),
        in_specs=[hbm] * 7,
        out_specs=hbm,
        scratch_shapes=scratch,
        compiler_params=pltpu.CompilerParams(vmem_limit_bytes=127 * 1024 * 1024,
                                             flags=cfg["flags"], **cfg["cp"]),
        interpret=interpret,
        name=name,
    )


@jax.jit
def pallas_sequential_preLN__sliding_local_dilated__mixer_gmlp__prompt_kernel(
    A_x: jax.Array,
    A_wqkv: jax.Array,
    A_wo: jax.Array,
    B_x: jax.Array,
    B_w_in: jax.Array,
    B_w_sp: jax.Array,
    B_b_sp: jax.Array,
    B_w_out: jax.Array,
):
    del B_x
    return build(CFG)(A_x, A_wqkv, A_wo, B_w_in, B_w_sp, B_b_sp, B_w_out)
```

```python
import functools

import jax
import jax.numpy as jnp
import numpy as np
from jax import lax
from jax.experimental import pallas as pl
from jax.experimental.pallas import tpu as pltpu

S = 2048
D = 1024
FH = 1792
DH = 32
WIN = 8
DIL = 2
EPS = 1e-5

U = 256
NU = S // U
NT = D // 128
HALO = 16
PARTS = 4

SLOT = 32
SHORT = 320
LONG = 512

f32 = jnp.float32
bf16 = jnp.bfloat16
u32 = jnp.uint32


def _pack(v):
    return pltpu.bitcast(v.astype(bf16), u32)


def _as_bf16(v):
    return pltpu.bitcast(v, bf16)


def _unpack(v):
    return _as_bf16(v).astype(f32)


def _dot(a, b):
    return jnp.dot(_as_bf16(a), _as_bf16(b), preferred_element_type=f32)


def _ds(start, size):
    return pl.ds(start if isinstance(start, int) else pl.multiple_of(start, size), size)


def _clip(v, lo, hi):
    return min(max(v, lo), hi) if isinstance(v, int) else jnp.clip(v, lo, hi)


def _share(step, steps, total):
    count = -(-total // steps)
    return _clip(step * count, 0, total - count), count


_C = float(np.sqrt(2.0 / np.pi))
ALPHA = float((_C * 0.044715) ** (1.0 / 3.0))
GAIN = 2.0 * ALPHA


def _gelu(v):
    return v * (1.0 + jnp.tanh(v * (_C / ALPHA + v * v)))


LEFT = (((1, 0, 0), (1, 1, 1)), ((1, 1, 0), (1, 1, 1)), ((1, 0, 0),), ((1, 1, 1),),
        ((1, 0, 0), (1, 0, 1)), ((1, 1, 0), (-1, 0, 0)), ((1, 0, 1), (-1, 1, 1)))
RIGHT = (((1, 0, 0), (1, 1, 1)), ((1, 0, 0),), ((1, 0, 1), (-1, 1, 1)), ((1, 1, 0), (-1, 0, 0)),
         ((1, 1, 1),), ((1, 0, 0), (1, 0, 1)), ((1, 1, 0), (1, 1, 1)))
ORDER = (0, 3, 1, 2, 5, 4, 6)


def _factor(terms, get):
    v = get(*terms[0][1:])
    for sign, i, j in terms[1:]:
        v = v + get(i, j) if sign > 0 else v - get(i, j)
    return v


def _factors(forms, get):
    blk = {(i, j): get(i, j) for i in range(2) for j in range(2)}
    return [_factor(terms, lambda i, j: blk[i, j]) for terms in forms]


class _Held:
    def __setitem__(self, _, v):
        self.v = v

    def __getitem__(self, _):
        return self.v


def _combiner(tmp, put):
    t1, t2, t3, t4, t5 = tmp

    def feed(i, m):
        if i == 0:
            t1[...] = m
        elif i == 3:
            t4[...] = m
        elif i == 1:
            t2[...] = m
            put(1, 0, m + t4[...])
        elif i == 2:
            t3[...] = m
        elif i == 5:
            put(1, 1, (t1[...] - t2[...] + t3[...]) + m)
        elif i == 4:
            t5[...] = m
            put(0, 1, m + t3[...])
        else:
            put(0, 0, (t1[...] + t4[...] - t5[...]) + m)
    return feed


class _Split:
    def __init__(self, n, level):
        self.level, self.parts, self.half = level, 1 << level, n // 2
        self.width = n // self.parts // 128 * 128
        self.rest = self.half - 2 * self.width if level == 2 else 0

    def at(self, j, offset=0):
        if self.level == 1:
            return j * self.half + offset
        return (j // 2) * self.half + (j % 2) * self.width + offset

    def rest_at(self, h):
        return h * self.half + 2 * self.width


class _Blocks:
    level, parts, rest = 2, 4, 0

    def __init__(self, tiles):
        self.tiles, self.width = tiles, 128 * len(tiles)

    def at(self, j, offset):
        return self.tiles[offset // 128][j]


D1, D2, S2, F2 = _Split(D, 1), _Split(D, 2), _Split(S, 2), _Split(FH, 2)
Z1 = _Blocks([[F2.at(j, c) for j in range(4)] for c in range(0, F2.width, 128)])
Z2 = _Blocks([[FH + c for c in tile] for tile in Z1.tiles]
             + [[FH + F2.rest_at(0), FH + F2.rest_at(1), F2.rest_at(0), F2.rest_at(1)]])


def _pair_transpose(v):
    sub = lax.broadcasted_iota(jnp.int32, v[0].shape, 0)
    v = list(v)
    for s in (1, 2):
        m = (sub & (2 * s)) != 0
        new = list(v)
        for j in range(4):
            if not j & s:
                new[j] = jnp.where(m, pltpu.roll(v[j + s], 2 * s, 0), v[j])
                new[j + s] = jnp.where(m, v[j + s], pltpu.roll(v[j], 8 - 2 * s, 0))
        v = new
    return v


def _take(v, idx):
    return jnp.take_along_axis(v, idx, axis=1)


def _tasks(fn, args, gated, latency, cost):
    return [(functools.partial(fn, *a), gated, latency, cost) for a in args]


def _staggered(early, late, lag):
    per = len(early) / len(late)
    order = list(enumerate(early)) + [((j + 1) * per + lag - 0.5, t) for j, t in enumerate(late)]
    return [t for _, t in sorted(order, key=lambda p: p[0])]


def _run(todo):
    for t in todo:
        t[0]()


GAP = [(lambda: None, [], 0, 200)]


def _kernel(x_hbm, wqkv_hbm, wo_hbm, win_hbm, wsp_hbm, bsp_hbm, wout_hbm, out_hbm,
            x_s, raw, bsp_raw,
            wq_p, wk_p, wv_p, wo_p, wz1_p, wz2_p, wout_p, wout_r, z2n_p, z2n_r,
            z1_s, bias_s, xa, xb, oa, ha, sa, ya,
            q_s, o_s, k_s, v_s, kv_s, p_s, l_s, e_s, z_s, zn_s, sp_s,
            st0, st1, inv0, inv1, tmp_s, sem, out_sem):
    zero = []

    def spot(ref, row, col):
        n = 8 * (4 // ref.dtype.itemsize)
        ref = ref if len(ref.shape) == 2 else ref.at[zero[0]]
        return ref.at[_ds(row + zero[0] * n, n), _ds(col + zero[0] * 128, 128)]

    def gate(ref, v):
        n = 8 * (4 // ref.dtype.itemsize)
        spot(ref, ref.shape[-2] - n, 0)[0:8, :] = v.astype(ref.dtype)

    def done(ref, row, col):
        v = spot(ref, row, col)[...]
        return v if v.dtype == u32 else pltpu.bitcast(v, u32)

    def after(tokens):
        def tie(b):
            if not tokens:
                return b
            tok = functools.reduce(lambda p, q: p | q, tokens)
            tok = jnp.concatenate([tok] * (b.shape[1] // 128), axis=1)
            always = lax.broadcasted_iota(jnp.int32, tok.shape, 0) >= zero[0]
            parts = []
            for r in range(0, b.shape[0], 64):
                parts += [b[r:r + 56], jnp.where(always, b[r + 56:r + 64], tok)]
            return jnp.concatenate(parts, axis=0)
        return tie

    def overlap(main, *sides):
        n, cycles, gen = main
        per = max(1, cycles // SLOT)
        plan = [[] for _ in range(n * per)]
        for side in sides:
            todo, first, last = side if isinstance(side, tuple) else (side, 0, n)
            if last == n:
                last -= todo[-1][2] / cycles
            span = max(1, int((last - first) * per))
            total, spent = sum(t[3] for t in todo), 0
            for t in todo:
                plan[first * per + spent * span // total].append(t)
                spent += t[3]
        next(gen)
        due = [[] for _ in range(n)]
        for i, todo in enumerate(plan):
            if i % per == 0:
                res = gen.send(after([tok for _, tok in due[i // per]]))
            gated = []
            for _, refs, _, _ in todo:
                gated += [r for r in refs if not any(r is g for g in gated)]
            row = res.shape[0] * (i % per) // per
            for ref in gated:
                gate(ref, res[row:row + 8, 0:128])
            for fn, _, latency, _ in todo:
                where = fn()
                j = -(-(i * cycles // per + latency) // cycles)
                if where is not None and j < n:
                    due[j] = [d for d in due[j] if d[0] is not where[0]]
                    due[j].append((where[0], done(*where)))

    def left_tasks(ref, ks, load, gated, rows=None, cols=None, outer=None, rest=True):
        h = U // ks.parts

        def put(n, r, c, v):
            ref[_ds(n * h // 2 + r // 2, 8), c:c + 128] = _pack(v)

        def main(r, c, o):
            def get(i, j):
                if ks.level == 1:
                    return load(i * h + r, ks.at(j, c))
                return _factor(LEFT[o],
                               lambda a, b: load((2 * a + i) * h + r, ks.at(2 * b + j, c)))
            for n, v in enumerate(_factors(LEFT, get)):
                put(7 * o + n, r, c, v)
            return ref, 7 * o * h // 2 + r // 2, c

        def other(r, i):
            vals = _factors(LEFT, lambda a, b: load((2 * a + i) * h + r, ks.rest_at(b)))
            for o, v in enumerate(vals):
                put(7 * o + 6 - i, r, ks.width, v)
            return ref, (6 - i) * h // 2 + r // 2, ks.width
        cols = range(0, ks.width, 128) if cols is None else cols
        outer = range(7 ** (ks.level - 1)) if outer is None else outer
        out = []
        for r in range(0, h, 16) if rows is None else rows:
            out += _tasks(main, [(r, c, o) for c in cols for o in outer], gated, SHORT, 30)
            out += _tasks(other, [(r, 0), (r, 1)] if ks.rest and rest else [], gated, SHORT, 30)
        return out

    def right_tasks(main_p, rest_p, ns, rows, load, gated, latency=SHORT):
        def main(prow, r, c, o):
            def get(i, j):
                if ns.level == 1:
                    return load(i, r, ns.at(j, c))
                return _factor(RIGHT[o], lambda a, b: load(2 * a + i, r, ns.at(2 * b + j, c)))
            for m, v in enumerate(_factors(RIGHT, get)):
                main_p.at[7 * o + m][_ds(prow, 8), c:c + 128] = _pack(v)
            return main_p, prow, c

        def other(prow, r, o):
            top, bot = [_factor(RIGHT[o], lambda a, b: load(2 * a + i, r, ns.rest_at(b)))
                        for i in range(2)]
            for m, v in enumerate((top, bot, top - bot)):
                rest_p.at[3 * o + m][_ds(prow, 8), :] = _pack(v)
            return rest_p, prow, 0
        out = []
        for prow, r in rows:
            out += _tasks(main, [(prow, r, c, o) for c in range(0, ns.width, 128)
                                 for o in range(7 ** (ns.level - 1))], gated, latency, 32)
            out += _tasks(other, [(prow, r, o) for o in range(7)] if ns.rest else [], gated,
                          SHORT, 16)
        return out

    def matmul(ref, main_p, rest_p, ks, ns, store, cw=128):
        h = U // ks.parts

        def lhs(m, lo, hi):
            return ref[m * h // 2:(m + 1) * h // 2, lo:hi]

        def temps(slot):
            return [tmp_s.at[(5 * slot + j) * h:(5 * slot + j + 1) * h, 0:cw] for j in range(5)]

        def one_level(c, tie):
            feed = _combiner(temps(0), lambda i, j, v: store(i * h, ns.at(j, c), v))
            for m in ORDER:
                res = _dot(lhs(m, 0, ks.width), tie(main_p.at[m][:, c:c + cw]))
                feed(m, res)
                tie = yield res
            return tie

        def two_levels(c, tie):
            def put(i, j):
                return lambda a, b, v: store((2 * a + i) * h, ns.at(2 * b + j, c), v)
            outer = {(i, j): _combiner(temps(2 * i + j), put(i, j))
                     for i in range(2) for j in range(2)}
            for o in ORDER:
                def finish(i, j, v):
                    if ks.rest and i != j:
                        v = v + _dot(lhs(7 * o + 6 - i, ks.width, ks.width + 128),
                                     rest_p.at[2 * o + j][:, c:c + cw])
                    outer[i, j](o, v)
                feed = _combiner([_Held() for _ in range(5)], finish)
                for m in ORDER:
                    b, hi = main_p.at[7 * o + m][:, c:c + cw], ks.width
                    if ks.rest and m >= 5:
                        b = jnp.concatenate([b, rest_p.at[2 * o + 6 - m][:, c:c + cw]], axis=0)
                        hi += 128
                    res = _dot(lhs(7 * o + m, 0, hi), tie(b))
                    feed(m, res)
                    tie = yield res
            return tie

        def rest_of_n(tie):
            def put(i):
                return lambda a, b, v: store((2 * a + i) * h, ns.rest_at(b), v)
            outer = [_combiner(temps(i), put(i)) for i in range(2)]
            for o in ORDER:
                for i, (m0, b0), (m1, b1) in ((1, (3, 2), (1, 0)), (0, (2, 2), (4, 1))):
                    first = _dot(lhs(7 * o + m0, 0, ks.width), tie(rest_p.at[3 * o + b0][...]))
                    tie = yield first
                    res = _dot(lhs(7 * o + m1, 0, ks.width), tie(rest_p.at[3 * o + b1][...]))
                    outer[i](o, res - first if i else res + first)
                    tie = yield res

        def gen():
            tie = yield
            for c in range(0, ns.width, cw):
                tie = yield from (one_level if ks.level == 1 else two_levels)(c, tie)
            if ns.rest:
                yield from rest_of_n(tie)
        return (7 ** ks.level * (ns.width // cw) + (28 if ns.rest else 0),
                h // 4 * (ks.width // 128) * (cw // 128), gen())

    def staged(i):
        return (z_s, zn_s)[i].at[0:D // 4, 0:D]

    def factor_staged(buf, split, rotate, rows, aside=None):
        def load(i, r, c):
            r += i * split.width // 2
            i, r, tile = r // (D // 4), r % (D // 4), c // 128
            v = pltpu.bitcast(staged(i)[r:r + 8, c:c + 128], u32)
            v = pltpu.roll(v, 128 - 4 * tile, 1) if rotate and tile else v
            if aside is not None and i != c // (D // 2):
                aside[i * D // 4 + r:i * D // 4 + r + 8, c % (D // 2):c % (D // 2) + 128] = v
            return _unpack(v)
        return right_tasks(buf, None, split, [(r, r) for r in rows], load,
                           [raw] if rotate else [z_s, zn_s], LONG if rotate else SHORT)

    def prepare_qkv(j, buf, part, parts, aside=None):
        def task(i, r):
            w = pltpu.bitcast(raw.at[j][i * D // 2 + r:i * D // 2 + r + 16, :], u32)
            lane = lax.broadcasted_iota(jnp.int32, (8, 128), 1)
            w = [w[:, t * 128:(t + 1) * 128] for t in range(NT)]
            w = [pltpu.roll(v, 4 * t, 1) if t else v for t, v in enumerate(w)]
            w = [w[(-t) % NT] for t in range(NT)]
            for b in range(3):
                m = (lane & (4 << b)) != 0
                w = [jnp.where(m, w[(t - (1 << b)) % NT], w[t]) for t in range(NT)]
            for t in range(NT):
                staged(i)[r // 2:r // 2 + 8, t * 128:(t + 1) * 128] = pltpu.bitcast(w[t], f32)
            return (z_s, zn_s)[i], r // 2, 0
        rows = range(part * D // 2 // parts, (part + 1) * D // 2 // parts, 16)
        return _staggered(_tasks(task, [(i, r) for r in rows for i in range(2)], [raw], LONG, 45),
                          factor_staged(buf, D1, True, [r // 2 for r in rows], aside), 6)

    def prepare_wo():
        def task(d4, t2, hh, c):
            src = [((t2 * 4 + j) * 4 + hh) * 32 + d4 * 16 for j in range(4)]
            v = _pair_transpose([pltpu.bitcast(raw.at[3][s:s + 16, c:c + 256], u32) for s in src])
            for j in range(4):
                r = ((j * 4 + hh) * 32 + t2 * 16) // 2
                staged(d4)[r:r + 8, c:c + 256] = pltpu.bitcast(v[j], f32)
            return (z_s, zn_s)[d4], r, c
        return (_tasks(task, [(d4, t2, hh, c) for d4 in range(2) for t2 in range(2)
                              for hh in range(4) for c in range(0, D, 256)], [raw], SHORT, 40)
                + GAP + factor_staged(wo_p, D2, False, range(0, D2.width // 2, 8)))

    def groups(first, count):
        return [((first + g) * 8, (first + g) * 16) for g in range(count)]

    def prepare_win(buf, cols, first, count):
        def load(i, r, c):
            lo = c % F2.half
            return raw.at[4 + c // F2.half][_ds(D2.at(i) + r, 16), lo:lo + 128].astype(f32)
        return right_tasks(buf, None, cols, groups(first, count), load, [raw])

    def prepare_wout(step, steps):
        def load(i, r, c):
            return raw.at[2 + i // 2][_ds(F2.at(i % 2) + r, 16), c:c + 128].astype(f32)

        def other(prow, r, j, c):
            def get(a, b):
                lo = D2.at(2 * b + j, c)
                return raw.at[2 + a][_ds(F2.rest_at(0) + r, 16), lo:lo + 128].astype(f32)
            for o, v in enumerate(_factors(RIGHT, get)):
                wout_r.at[2 * o + j][_ds(prow, 8), c:c + 128] = _pack(v)
            return wout_r, prow, c
        return (right_tasks(wout_p, None, D2, groups(*_share(step, steps, F2.width // 16)), load,
                            [raw])
                + _tasks(other, [(*g, j, c) for g in groups(*_share(step, steps, F2.rest // 16))
                                 for j in range(2) for c in range(0, D2.width, 128)],
                         [raw], SHORT, 28))

    def prepare_bias():
        def task(r):
            b = bsp_raw[...].astype(f32).reshape(1, S) * (1.0 / GAIN)
            bias_s[r:r + 128, :] = jnp.broadcast_to(b[:, r:r + 128], (128, 128)).T
            return bias_s, r, 0
        return _tasks(task, [(r,) for r in range(0, S, 128)], [], LONG, 50)

    def spatial_tasks(u, rows=None):
        per = D // U

        def regroup(r, m):
            low = lax.broadcasted_iota(jnp.int32, (8, 128), 1) < 64
            col = 2 * U * m
            w = pltpu.bitcast(raw.at[u // per * 4 + col // D][
                _ds(u % per * U + r, 16), col % D:col % D + 2 * U], u32)
            for a in range(2):
                one, two = w[:, a * 128:(a + 1) * 128], w[:, U + a * 128:U + (a + 1) * 128]
                mid = pltpu.roll(jnp.where(low, two, one), 64, 1)
                for j, v in enumerate((jnp.where(low, one, mid), jnp.where(low, mid, two))):
                    lo = S2.at(2 * a + j, m * 128)
                    sp_s[r // 2:r // 2 + 8, lo:lo + 128] = v
            return sp_s, r // 2, m * 128
        return (_tasks(regroup, [(b + r, m) for r in range(0, U // 4, 16)
                                 for b in range(0, U, U // 4) for m in range(NU // 2)],
                       [raw], LONG, 18),
                left_tasks(sa, S2, lambda r, c: _unpack(sp_s[r // 2:r // 2 + 8, c:c + 128]),
                           [sp_s], rows=rows))

    def unit(ref, u, n=U):
        return ref.at[_ds(u * n, n)]

    def norm_tasks(base, src, st, inv, eps=EPS, scale=None, rows=range(0, U, 16)):
        n = src.shape[1]

        def shift(r):
            v = src[_ds(r, 16), 0:128].astype(f32)
            st.at[0][_ds(r, 16), :] = jnp.broadcast_to(v[:, 0:1], (16, 128))
            return st, r, 0

        def moments(r):
            first = st.at[0][_ds(r, 8), :]
            s1 = s2 = None
            for c in range(0, n, 256):
                v = src[_ds(r, 8), c:c + 256].astype(f32)
                for d in (v[:, :128] - first, v[:, 128:] - first):
                    s1 = d if s1 is None else s1 + d
                    s2 = d * d if s2 is None else s2 + d * d
            m = jnp.sum(s1, axis=-1, keepdims=True) * (1.0 / n)
            var = jnp.sum(s2, axis=-1, keepdims=True) * (1.0 / n) - m * m
            st.at[1][_ds(r, 8), :] = first + m
            st.at[2][_ds(r, 8), :] = jnp.broadcast_to(jnp.maximum(var, 0.0) + eps, (8, 128))
            return st, r, 0

        def invert(r):
            v = lax.rsqrt(st.at[2][_ds(r, 16), :])
            inv[_ds(r, 16), :] = v if scale is None else v * scale
            return inv, r, 0

        def load(r, c, h=16, w=128):
            v = src[_ds(r, h), c:c + w].astype(f32)
            mean, mul = [jnp.concatenate([t[_ds(r, h), :]] * (w // 128), axis=1)
                         for t in (st.at[1], inv)]
            return (v - mean) * mul

        def write(dst):
            def task(r, c, w):
                dst[_ds(r, 8), c:c + w] = load(r, c, 8, w)
                return dst, r, c
            return _tasks(task, [(r + j, c, min(1024, n - c)) for r in rows for j in (0, 8)
                                 for c in range(0, n, 1024)], [base], SHORT, 22)
        out = _tasks(shift, [(r,) for r in rows], [base], LONG, 10)
        out += _staggered(
            _tasks(moments, [(r + j,) for r in rows for j in (0, 8)], [base], LONG, n // 28 + 8),
            _tasks(invert, [(r,) for r in rows], [], SHORT, 22), 6)
        return out, load, write

    def norm_x(u):
        out, load, _ = norm_tasks(x_s, unit(x_s, u), st0, inv0)
        return out + left_tasks(xa, D1, load, [x_s])

    def norm_h(u, dst, **kw):
        out, _, write = norm_tasks(x_s, unit(x_s, u), st1, inv1, scale=ALPHA, **kw)
        return out + write(dst)

    def left_h(src, **kw):
        return left_tasks(ha, D2, lambda r, c: src[_ds(r, 16), c:c + 128], [src], **kw)

    def norm_z2(u):
        h = U // 4
        out, _, write = norm_tasks(z_s, z_s, st0, inv0, EPS * GAIN * GAIN, 1.0 / GAIN)
        return out + write(zn_s), right_tasks(
            z2n_p, z2n_r, F2, [(u * (h // 2) + r // 2, r) for r in range(0, h, 16)],
            lambda b, r, c: zn_s[b * h + r:b * h + r + 16, c:c + 128], [zn_s])

    def logit_tasks(q_buf, k_buf, masked=False):
        def task(r, b):
            lane = lax.broadcasted_iota(jnp.int32, (8, 128), 1)
            acc = [None] * 4
            for t in range(NT):
                q = q_buf[r:r + 8, t * 128:(t + 1) * 128]
                for j in range(4):
                    k0 = HALO + r - DIL * (4 * b + j)
                    term = q * k_buf[t, k0:k0 + 8, :]
                    acc[j] = term if t == 0 else acc[j] + term
            for bit in (1, 2):
                odd = (lane & bit) != 0
                acc = [jnp.where(odd, acc[j ^ bit], acc[j]) for j in range(4)]
            lg = acc[0]
            for j in range(1, 4):
                lg = lg + _take(acc[j], lane ^ j)
            lg = lg * float(DH) ** -0.5
            if masked and r < DIL * WIN:
                pos = r + lax.broadcasted_iota(jnp.int32, (8, 128), 0)
                lg = jnp.where(pos >= DIL * (4 * b + (lane & 3)), lg, -1e9)
            l_s[b, r:r + 8, :] = lg
            return l_s, r, 0
        return _tasks(task, [(r, b) for r in range(0, U, 8) for b in range(2)], [q_buf, k_buf],
                      LONG, 75)

    def softmax_tasks():
        def exps(r):
            lane = lax.broadcasted_iota(jnp.int32, (16, 128), 1)
            lg = [l_s[b, r:r + 16, :] for b in range(2)]
            mx = jnp.maximum(lg[0], lg[1])
            mx = functools.reduce(jnp.maximum, [mx] + [_take(mx, lane ^ j) for j in range(1, 4)])
            for b in range(2):
                e_s[b, r:r + 16, :] = jnp.exp(lg[b] - mx)
            return e_s, r, 0

        def probs(r):
            lane = lax.broadcasted_iota(jnp.int32, (8, 128), 1)
            e = [e_s[b, r:r + 8, :] for b in range(2)]
            e = {4 * b + j: _take(e[b], (lane & -4) | j) for j in range(4) for b in range(2)}
            inv = 1.0 / functools.reduce(lambda p, q: p + q, e.values())
            for w in range(WIN):
                p_s[w, r:r + 8, :] = e[w] * inv
            return p_s, r, 0
        return _staggered(_tasks(exps, [(r,) for r in range(0, U, 16)], [l_s], LONG, 40),
                          _tasks(probs, [(r,) for r in range(0, U, 8)], [], LONG, 40), 2)

    def value_tasks(v_buf):
        def task(r, t0):
            acc = [None] * 4
            for w in range(WIN):
                k0 = HALO + r - DIL * w
                p = p_s[w, r:r + 8, :]
                for j in range(4):
                    term = p * v_buf[t0 + j, k0:k0 + 8, :]
                    acc[j] = term if w == 0 else acc[j] + term
            for j in range(4):
                o_s[r:r + 8, (t0 + j) * 128:(t0 + j + 1) * 128] = acc[j]
            return o_s, r, t0 * 128
        out, h = [], U // 4
        for g in range(0, h + 16, 16):
            if g < h:
                out += _tasks(task, [(g + b + j, t0) for b in range(0, U, h) for j in (0, 8)
                                     for t0 in (0, 4)], [p_s, v_buf], SHORT, 62)
            else:
                out += GAP
            if g:
                out += left_tasks(oa, D2, lambda r, c: o_s[r:r + 16, c:c + 128], [o_s],
                                  rows=[g - 16])
        return out

    def carry_over(buf, src):
        buf[:, 0:HALO, :] = src[:, U:U + HALO, :]

    def clamp_left(buf):
        for t in range(NT):
            buf[t, 0:HALO, :] = jnp.broadcast_to(buf[t, HALO:HALO + 1, :], (HALO, 128))

    def copies():
        def units(lo, hi):
            return [(x_hbm.at[0, lo * U:hi * U], x_s.at[lo * U:hi * U])]

        def qkv_parts(j, parts):
            n = D // 2 // parts
            return [((j, p), [(wqkv_hbm.at[r:r + n, j * D:(j + 1) * D], raw.at[j, r:r + n])
                              for r in (p * n, D // 2 + p * n)]) for p in range(parts)]

        def win_rows(lo, hi):
            return [(win_hbm.at[r + lo:r + hi, j * F2.half:(j + 1) * F2.half],
                     raw.at[4 + j, r + lo:r + hi, 0:F2.half])
                    for r in range(0, D, D2.width) for j in range(4)]
        early = _share(0, NU - 2, D2.width // 16)[1] * 16
        pairs = [("x0", units(0, 1)), *qkv_parts(0, PARTS), ("x1", units(1, 2)),
                 *qkv_parts(1, PARTS), *qkv_parts(2, 2),
                 ("wo", [(wo_hbm, raw.at[3, 0:D])] + units(2, 3)),
                 ("early", units(3, 4) + win_rows(0, early)),
                 ("rest", units(4, NU) + win_rows(early, D2.width) + [(bsp_hbm, bsp_raw)]),
                 ("late0", [(wsp_hbm.at[0:D, j * D:(j + 1) * D], raw.at[j, 0:D]) for j in range(2)]
                  + [(wout_hbm.at[j * F2.half:(j + 1) * F2.half], raw.at[2 + j, 0:F2.half])
                     for j in range(2)]),
                 ("late1", [(wsp_hbm.at[D:S, j * D:(j + 1) * D], raw.at[4 + j, 0:D])
                            for j in range(2)])]
        return {name: [(a, b, sem.at[j]) for a, b in group]
                for j, (name, group) in enumerate(pairs)}

    def start(*names):
        for name in names:
            for args in copies()[name]:
                pltpu.make_async_copy(*args).start()

    def wait(name):
        for args in copies()[name]:
            pltpu.make_async_copy(*args).wait()

    def out_copy(u, part):
        rows = _ds(u * U + (0 if part else U // 2), U // 2)
        cols = (slice(0, D), slice(D // 2, D), slice(0, D // 2))[part]
        return pltpu.make_async_copy(x_s.at[rows, cols], out_hbm.at[0, rows, cols], out_sem)

    def at_dot(fn, i):
        return [(fn, [], 0, 1)], i, i + 1

    def add_into(u):
        def store(r, c, v):
            idx = (slice(r, r + v.shape[0]), slice(c, c + v.shape[1]))
            dst = unit(x_s, u)
            dst[idx] = (dst[idx].astype(f32) + v).astype(bf16)
        return store

    def queries(src):
        def store(r, c, v):
            q_s[r:r + v.shape[0], c:c + 128] = v
        return matmul(src, wq_p, None, D1, D1, store)

    def by_tile(src, w, buf):
        def store(r, c, v):
            buf[c // 128, HALO + r:HALO + r + v.shape[0], :] = v
        return matmul(src, w, None, D1, D1, store)

    def project(u):
        return matmul(oa, wo_p, None, D2, D2, add_into(u))

    def first_queries(part):
        n, h = D // 4 // PARTS, U // 4
        rows, cols = slice(part * n, (part + 1) * n), slice(part * 2 * n, (part + 1) * 2 * n)

        def gen():
            tie = yield
            for j in range(2):
                for c in range(0, D // 2, 128):
                    a = jnp.concatenate([jnp.concatenate([
                        xb[(2 + i) * h:(3 + i) * h, cols] if i == m
                        else sp_s.at[i * h:(i + 1) * h, m * D // 2:(m + 1) * D // 2][:, cols]
                        for m in range(2)], axis=1) for i in range(2)], axis=0)
                    b = jnp.concatenate([
                        wq_p.at[1 + 3 * i][rows, c:c + 128] if i == j
                        else sa.at[i * D // 4:(i + 1) * D // 4][rows, c:c + 128]
                        for i in range(2)], axis=0)
                    res = _dot(a, tie(b))
                    idx = (slice(0, U), slice(D1.at(j, c), D1.at(j, c) + 128))
                    o_s[idx] = o_s[idx] + res if part else res
                    tie = yield res
        return NT, U * n // 128, gen()

    def on_arrival(j, buf, part, parts, first, last):
        return (at_dot(functools.partial(wait, (j, part)), max(0, first - 1)),
                (prepare_qkv(j, buf, part, parts), first, last - 2))

    def first_attention():
        wait("x0")
        bits = pltpu.bitcast(x_s[0:16, 0:128], jnp.int32)
        zero.append(bits[0, 0] ^ pltpu.roll(bits, 1, 1)[0, 1])
        stats, load, _ = norm_tasks(x_s, unit(x_s, 0), st0, inv0)

        def keep_aside(r, c):
            v = load(r, c)
            if r // (U // 2) != c // (D // 2):
                sp_s[r // 2:r // 2 + 8, c:c + 128] = _pack(v)
            return v
        _run(stats + left_tasks(xb, D1, keep_aside, [x_s]))
        wait((0, 0))
        _run(prepare_qkv(0, wq_p, 0, PARTS, sa))
        for part in range(1, PARTS):
            wait((0, part))
            overlap(first_queries(part - 1), (prepare_qkv(0, wq_p, part, PARTS, sa), 0, NT - 2))
        wait("x1")
        overlap(first_queries(PARTS - 1), (norm_x(1), 0, NT - 2))
        overlap(queries(xa), *[side for p in range(PARTS)
                               for side in on_arrival(1, wk_p, p, PARTS, 7 * p, 7 * p + 7)])
        overlap(by_tile(xb, wk_p, kv_s), *on_arrival(2, wv_p, 0, 2, 14, 28))
        wait((2, 1))
        clamp_left(kv_s)
        carry_over(k_s, kv_s)
        overlap(by_tile(xa, wk_p, k_s),
                prepare_qkv(2, wv_p, 1, 2) + GAP + logit_tasks(o_s, kv_s, True))
        wait("wo")
        prep = prepare_wo()
        cut = len(prep) * 5 // 8
        overlap(by_tile(xb, wv_p, kv_s), softmax_tasks(), prep[:cut])
        clamp_left(kv_s)
        carry_over(v_s, kv_s)
        overlap(by_tile(xa, wv_p, v_s), value_tasks(kv_s), prep[cut:])
        overlap(project(0), logit_tasks(q_s, k_s), norm_x(2))

    def step_attention(u):
        @pl.when(u == 3)
        def _():
            wait("rest")
        window = _share(u - 2, NU - 2, D2.width // 16)
        prep = prepare_win(wz2_p, Z2, *window) + prepare_win(wz1_p, Z1, *window)
        cut = len(prep) * 7 // 8
        g = _clip(u - 2, 0, U // 64 - 1) * 16
        head = norm_h(0, z_s, rows=[g + b for b in range(0, U, 64)]) + left_h(z_s, rows=[g])
        carry_over(k_s, k_s)
        overlap(queries(xa), softmax_tasks(), prep[:cut])
        overlap(by_tile(xa, wk_p, k_s), value_tasks(v_s))
        carry_over(v_s, v_s)
        overlap(by_tile(xa, wv_p, v_s), logit_tasks(q_s, k_s), head)
        overlap(project(u - 1), norm_x(_clip(u + 1, 0, NU - 1)), prep[cut:])

    def hidden(u, w, cols):
        def store(r, c, v):
            n = v.shape[0]
            if c >= FH:
                z_s[r:r + n, c - FH:c - FH + 128] = _gelu(v)
            else:
                unit(z1_s, u, U // 2)[r // 2:(r + n) // 2, c:c + 128] = _pack(_gelu(v))
        return matmul(ha, w, None, D2, cols, store)

    def last_attention():
        main = hidden(0, wz2_p, Z2)
        regroup, factors = spatial_tasks(0, [0, 16])
        overlap(main, (softmax_tasks(), 0, 90), (value_tasks(v_s), 90, main[0]), regroup)
        overlap(project(NU - 1), prepare_bias() + factors + norm_h(1, q_s))

    def step_hidden(u):
        norm, factors = norm_z2(u - 1)
        cut = len(factors) * 3 // 8
        main = hidden(u - 1, wz1_p, Z1)
        last = main[0] - 49
        overlap(main, (norm + factors[:cut], 0, last + 21),
                *[(left_h(q_s, outer=[o]), last + 7 * j + 6, last + 7 * j + 13)
                  for j, o in enumerate(ORDER[:3])])
        main = hidden(u, wz2_p, Z2)
        overlap(main, (sum((left_h(q_s, outer=[o]) for o in ORDER[3:]), []), 0, 28),
                (norm_h(_clip(u + 1, 0, NU - 1), q_s), 28, main[0]),
                (factors[cut:] + prepare_wout(u - 1, NU - 1), 28, main[0]))

    def last_hidden():
        overlap(hidden(NU - 1, wz1_p, Z1), sum(norm_z2(NU - 1), []),
                spatial_tasks(0, [32, 48])[1])

    def step_output(u):
        bias, z1 = unit(bias_s, u), unit(z1_s, u, U // 2)

        def store(r, c, g):
            n = g.shape[0]
            z_s[r:r + n, c:c + 128] = _unpack(z1[r // 2:(r + n) // 2, c:c + 128]) * (
                g + bias[r:r + n, :])

        def left_y(**kw):
            return left_tasks(ya, F2, lambda r, c: z_s[r:r + 16, c:c + 128], [z_s], **kw)
        regroup, factors = spatial_tasks(_clip(u + 1, 0, NU - 1))
        overlap(matmul(sa, z2n_p, z2n_r, S2, F2, store), (regroup, 0, 49),
                *[(left_y(cols=[128 * j], rest=False), 49 * j + 49, 49 * j + 69)
                  for j in range(3)])
        _run(left_y(cols=[]))
        overlap(matmul(ya, wout_p, wout_r, F2, D2, add_into(u), 256), factors,
                at_dot(out_copy(u, 0).start, 36), at_dot(out_copy(u, 1).start, 43))
        out_copy(u, 2).start()

    start(*list(copies())[:-2])
    first_attention()
    wait("early")
    start("late0")
    pl.loop(2, NU)(step_attention)
    start("late1")
    wait("late0")
    last_attention()
    pl.loop(1, NU)(step_hidden)
    last_hidden()
    wait("late1")
    pl.loop(0, NU)(step_output)
    for u in range(NU):
        for part in range(3):
            out_copy(u, part).wait()


def _build():
    vm = pltpu.VMEM

    def right(ks, ns):
        return vm((7 ** ks.level, ks.width // 2, ns.width), u32)

    def left(ks):
        return vm((7 ** ks.level * U // ks.parts // 2, ks.width + ks.rest), u32)
    scratch = [
        vm((S + 16, D), bf16),
        vm((8, D + 16, D), bf16),
        vm((S,), bf16),
        *[right(D1, D1)] * 3, right(D2, D2), right(D2, Z1), right(D2, Z2),
        right(F2, D2), vm((14, F2.rest // 2, D2.width), u32),
        right(S2, F2), vm((21, S2.width // 2, F2.rest), u32),
        vm((S // 2, FH), u32),
        vm((S, 128), f32),
        left(D1), left(D1), left(D2), left(D2), left(S2), left(F2),
        *[vm((U + 8, D), f32)] * 2,
        *[vm((NT, HALO + U + 8, 128), f32)] * 3,
        vm((WIN, U + 8, 128), f32),
        *[vm((2, U + 8, 128), f32)] * 2,
        *[vm((U + 8, FH), f32)] * 2,
        vm((U // 2 + 8, S), u32),
        *[vm((3, U + 8, 128), f32)] * 2,
        *[vm((U, 128), f32)] * 2,
        vm((5 * U, 256), f32),
        pltpu.SemaphoreType.DMA((9 + 2 * PARTS,)),
        pltpu.SemaphoreType.DMA(()),
    ]
    hbm = pl.BlockSpec(memory_space=pl.ANY)
    return pl.pallas_call(
        _kernel,
        out_shape=jax.ShapeDtypeStruct((1, S, D), bf16),
        in_specs=[hbm] * 7,
        out_specs=hbm,
        scratch_shapes=scratch,
        compiler_params=pltpu.CompilerParams(
            vmem_limit_bytes=127 * 1024 * 1024,
            disable_bounds_checks=True, disable_semaphore_checks=True),
        name="fused_block",
    )


@jax.jit
def pallas_sequential_preLN__sliding_local_dilated__mixer_gmlp__prompt_kernel(
    A_x: jax.Array,
    A_wqkv: jax.Array,
    A_wo: jax.Array,
    B_x: jax.Array,
    B_w_in: jax.Array,
    B_w_sp: jax.Array,
    B_b_sp: jax.Array,
    B_w_out: jax.Array,
):
    del B_x
    return _build()(A_x, A_wqkv, A_wo, B_w_in, B_w_sp, B_b_sp, B_w_out)
```
